```python
import jax
import jax.numpy as jnp

def _softmax(x, axis=-1):
    return jax.nn.softmax(x, axis=axis)

def _gelu(x):
    return jax.nn.gelu(x, approximate=True)

def _silu(x):
    return jax.nn.silu(x)

def _sigmoid(x):
    return jax.nn.sigmoid(x)

def _layernorm(x, axis=-1, eps=1e-05):
    m = jnp.mean(x, axis=axis, keepdims=True)
    v = jnp.var(x, axis=axis, keepdims=True)
    return (x - m) / jnp.sqrt(v + eps)

def _scatter_add(tgt, idx, src, axis=0):
    return tgt.at[idx].add(src)

def _segment_sum(src, seg, n):
    return jax.ops.segment_sum(src, seg, n)

class _Rng:

    def __init__(self, key):
        self._k = key

    def _next(self):
        self._k, sub = jax.random.split(self._k)
        return sub

    def normal(self, shape):
        return jax.random.normal(self._next(), shape, dtype=jnp.bfloat16)

    def randint(self, lo, hi, shape):
        return jax.random.randint(self._next(), shape, lo, hi, dtype=jnp.int32)

    def uniform(self, shape, lo=0.0, hi=1.0):
        return jax.random.uniform(self._next(), shape, jnp.bfloat16, lo, hi)

    def permutation(self, n):
        return jax.random.permutation(self._next(), n)
kernel_name = 'interleave_layers__memory_aug_recurrent_mem_tr__glu_gated_glu__prompt'

def setup_inputs():
    _rng = _Rng(jax.random.key(int.from_bytes(__import__("os").urandom(4), "little")))
    _w = lambda a: (lambda t: t.astype(jnp.bfloat16) if jnp.issubdtype(t.dtype, jnp.floating) else t)(jnp.asarray(a))

    def _A_setup():
        B, S, Dm = (1, 2048, 1024)
        H, Dh = (32, 128)
        M, seg = (8, 32)
        seg = min(seg, S)
        S = S // seg * seg
        return {'x': _w((lambda *s: _rng.normal(s) * 0.05)(B, S, Dm)), 'mem0': _w((lambda *s: _rng.normal(s) * 0.05)(B, M, Dm)), 'Wq': _w((lambda *s: _rng.normal(s) * 0.05)(Dm, H, Dh) * Dm ** (-0.5)), 'Wk': _w((lambda *s: _rng.normal(s) * 0.05)(Dm, H, Dh) * Dm ** (-0.5)), 'Wv': _w((lambda *s: _rng.normal(s) * 0.05)(Dm, H, Dh) * Dm ** (-0.5)), 'Wo': _w((lambda *s: _rng.normal(s) * 0.05)(H, Dh, Dm) * (H * Dh) ** (-0.5)), 'seg_len': seg}
    _A_in = _A_setup()

    def _B_setup():
        B, S, D, F = (1, 2048, 1024, 3584)
        return {'x': _w((lambda *s: _rng.normal(s) * 0.05)(B, S, D)), 'w_gate': _w((lambda *s: _rng.normal(s) * 0.05)(D, F)), 'w_up': _w((lambda *s: _rng.normal(s) * 0.05)(D, F)), 'w_down': _w((lambda *s: _rng.normal(s) * 0.05)(F, D))}
    _B_in = _B_setup()
    return {'A_x': _A_in['x'], 'A_mem0': _A_in['mem0'], 'A_Wq': _A_in['Wq'], 'A_Wk': _A_in['Wk'], 'A_Wv': _A_in['Wv'], 'A_Wo': _A_in['Wo'], 'A_seg_len': _A_in['seg_len'], 'B_x': _B_in['x'], 'B_w_gate': _B_in['w_gate'], 'B_w_up': _B_in['w_up'], 'B_w_down': _B_in['w_down']}

def reference(A_x, A_mem0, A_Wq, A_Wk, A_Wv, A_Wo, A_seg_len, B_x, B_w_gate, B_w_up, B_w_down):

    def _A_ref(x, mem0, Wq, Wk, Wv, Wo, seg_len):
        B, S, Dm = x.shape
        H, Dh = (Wq.shape[1], Wq.shape[2])
        M = mem0.shape[1]
        scale = Dh ** (-0.5)
        n_seg = S // seg_len
        L = M + seg_len
        idx = jnp.arange(L)
        mask = (idx[:, None] < M) | (idx[:, None] >= idx[None, :])
        mem = mem0
        outs = []
        for s in range(n_seg):
            xs = x[:, s * seg_len:(s + 1) * seg_len, :].copy()
            h = jnp.concatenate([mem, xs], axis=1)
            q = jnp.einsum('btd,dhe->bhte', h, Wq)
            k = jnp.einsum('btd,dhe->bhte', h, Wk)
            v = jnp.einsum('btd,dhe->bhte', h, Wv)
            scores = jnp.einsum('bhqe,bhke->bhqk', q, k) * scale
            scores = jnp.where(mask[None, None], scores, -1000000000.0)
            p = _softmax(scores, axis=-1)
            o = jnp.einsum('bhqk,bhke->bhqe', p, v)
            o = jnp.einsum('bhte,hed->btd', o, Wo)
            mem = o[:, :M, :].copy()
            outs.append(o[:, M:, :])
        return jnp.concatenate(outs, axis=1)

    def _B_ref(x, w_gate, w_up, w_down):
        g = jnp.einsum('bsd,df->bsf', x, w_gate)
        u = jnp.einsum('bsd,df->bsf', x, w_up)
        h = _sigmoid(g) * u
        return jnp.einsum('bsf,fd->bsd', h, w_down)
    x = A_x
    x = x + _A_ref(_layernorm(x, axis=-1), A_mem0, A_Wq, A_Wk, A_Wv, A_Wo, A_seg_len)
    x = x + _B_ref(_layernorm(x, axis=-1), B_w_gate, B_w_up, B_w_down)
    x = x + _A_ref(_layernorm(x, axis=-1), A_mem0, A_Wq, A_Wk, A_Wv, A_Wo, A_seg_len)
    x = x + _B_ref(_layernorm(x, axis=-1), B_w_gate, B_w_up, B_w_down)
    return x
```

```python
import functools
import math

import jax
import jax.numpy as jnp
import jax.experimental.pallas as pl
import jax.experimental.pallas.tpu as pltpu

F32 = jnp.float32
BF16 = jnp.bfloat16
LN_EPS = 1e-5
MASK_VALUE = -1000000000.0

HEAD_GROUP = 4
F_CHUNK = 512
D_CHUNK = 128
STAGE_SLOTS = 3


def _layernorm(x):
    m = jnp.mean(x, axis=-1, keepdims=True)
    c = x - m
    v = jnp.mean(c * c, axis=-1, keepdims=True)
    return c * jax.lax.rsqrt(v + LN_EPS)


def _dot(a, b):
    return jnp.dot(a, b, preferred_element_type=F32)


def _kernel(x_hbm, mem0_ref, wq_hbm, wk_hbm, wv_hbm, wo_hbm, wg_hbm, wu_hbm, wd_hbm,
            out_hbm,
            x_vm, out_vm, stage, wq, wk, wv, wo, wg, wu, wd,
            h_ref, o_ref, ra_ref, rb_ref, xb_ref, hb_ref,
            stage_sem, w_sem, out_sem, *, seg, n_mem, n_heads, head_dim):
    S, D = x_vm.shape
    F = wg.shape[1]
    n_seg = S // seg
    M2 = 2 * n_mem
    RA = M2 + 2 * seg
    scale = head_dim ** -0.5

    n_chunk = D // D_CHUNK
    rows = D_CHUNK * n_heads
    qkv_hbm = (wq_hbm, wk_hbm, wv_hbm)

    def stage_copy(m, c, slot):
        src = qkv_hbm[m].at[pl.ds(pl.multiple_of(c * rows, rows), rows)]
        return pltpu.make_async_copy(src, stage.at[slot], stage_sem.at[slot])

    x_copy = pltpu.make_async_copy(x_hbm, x_vm, w_sem.at[0])
    wo_copy = pltpu.make_async_copy(wo_hbm, wo, w_sem.at[1])
    wg_copy = pltpu.make_async_copy(wg_hbm, wg, w_sem.at[2])
    wu_copy = pltpu.make_async_copy(wu_hbm, wu, w_sem.at[3])
    wd_copy = pltpu.make_async_copy(wd_hbm, wd, w_sem.at[4])

    for c in range(STAGE_SLOTS):
        stage_copy(0, c, c).start()

    o_ref[...] = jnp.zeros(o_ref.shape, o_ref.dtype)
    rb_ref[...] = jnp.zeros(rb_ref.shape, rb_ref.dtype)

    for m, dst in enumerate((wq, wk, wv)):
        def relayout(c, carry, m=m, dst=dst):
            slot = (m * n_chunk + c) % STAGE_SLOTS
            stage_copy(m, c, slot).wait()
            w = stage[slot].reshape(D_CHUNK, n_heads, head_dim)
            dst[pl.ds(pl.multiple_of(c * D_CHUNK, D_CHUNK), D_CHUNK), :] = (
                w.reshape(D_CHUNK, n_heads * head_dim))
            nxt = c + STAGE_SLOTS

            @pl.when(nxt < n_chunk)
            def _():
                stage_copy(m, nxt, slot).start()

            if m < 2:
                @pl.when(nxt >= n_chunk)
                def _():
                    stage_copy(m + 1, nxt - n_chunk, slot).start()
            else:
                @pl.when(nxt == n_chunk)
                def _():
                    x_copy.start()

                @pl.when(nxt == n_chunk + 1)
                def _():
                    wo_copy.start()
            return carry

        jax.lax.fori_loop(0, n_chunk, relayout, 0)

    def pass_and_pos(t):
        in_mem = t < M2
        p = jnp.where(in_mem, t // n_mem, (t - M2) // seg)
        pos = jnp.where(in_mem, t % n_mem, n_mem + (t - M2) % seg)
        return p, pos

    def attention_mask():
        qp, qpos = pass_and_pos(jax.lax.broadcasted_iota(jnp.int32, (RA, RA), 0))
        kp, kpos = pass_and_pos(jax.lax.broadcasted_iota(jnp.int32, (RA, RA), 1))
        same = qp == kp
        keep = same & ((qpos < n_mem) | (qpos >= kpos))
        fill = jnp.where(same, MASK_VALUE, -jnp.inf).astype(F32)
        return keep, fill

    def b_down():
        return rb_ref[...] + _dot(hb_ref[...], wd[...])

    def a_out():
        y = _dot(o_ref[...], wo[...])
        r = ra_ref[...] + y[M2:]
        rb_ref[...] = r
        xb_ref[...] = _layernorm(r).astype(BF16)
        return y[:M2]

    def a_in(mem, x1, x2):
        r = jnp.concatenate([x1, x2], axis=0)
        ra_ref[...] = r
        h_ref[pl.ds(0, M2), :] = mem.astype(BF16)
        h_ref[pl.ds(M2, 2 * seg), :] = _layernorm(r).astype(BF16)

    def a_attention():
        keep, fill = attention_mask()
        gw = HEAD_GROUP * head_dim

        def project(g):
            cols = pl.ds(g * gw, gw)
            h = h_ref[...]
            return tuple(_dot(h, w[:, cols]).astype(BF16) for w in (wq, wk, wv))

        def attend(g, q, k, v):
            for j in range(HEAD_GROUP):
                sl = slice(j * head_dim, (j + 1) * head_dim)
                s = jax.lax.dot_general(q[:, sl], k[:, sl], (((1,), (1,)), ((), ())),
                                        preferred_element_type=F32)
                s = jnp.where(keep, s * scale, fill)
                p = jnp.exp(s - jnp.max(s, axis=-1, keepdims=True))
                inv = 1.0 / jnp.sum(p, axis=-1, keepdims=True)
                o = _dot(p.astype(BF16), v[:, sl]) * inv
                o_ref[:, pl.ds(g * gw + j * head_dim, head_dim)] = o.astype(BF16)

        n_groups = n_heads // HEAD_GROUP
        cur = project(0)
        for g in range(n_groups):
            nxt = project(g + 1) if g + 1 < n_groups else None
            attend(g, *cur)
            cur = nxt

    def b_gate_up():
        for c in range(F // F_CHUNK):
            cols = pl.ds(c * F_CHUNK, F_CHUNK)
            xb = xb_ref[...]
            g = _dot(xb, wg[:, cols])
            u = _dot(xb, wu[:, cols])
            hb_ref[:, cols] = (jax.nn.sigmoid(g) * u).astype(BF16)

    def x_segment(i):
        return x_vm[pl.ds(pl.multiple_of(i * seg, seg), seg), :].astype(F32)

    def out_copy(i):
        rows_i = pl.ds(pl.multiple_of(i * seg, seg), seg)
        return pltpu.make_async_copy(out_vm.at[rows_i], out_hbm.at[rows_i], out_sem)

    def store_out(i, y):
        out_vm[pl.ds(pl.multiple_of(i * seg, seg), seg), :] = y.astype(out_vm.dtype)

    mem0 = mem0_ref[...].astype(F32)
    zeros = jnp.zeros((seg, D), F32)

    x_copy.wait()
    wg_copy.start()
    a_in(jnp.concatenate([mem0, mem0], axis=0), x_segment(0), zeros)
    a_attention()

    wo_copy.wait()
    wu_copy.start()
    mem = a_out()
    a_in(mem, x_segment(1), zeros)
    a_attention()
    wg_copy.wait()
    wd_copy.start()
    wu_copy.wait()
    b_gate_up()
    wd_copy.wait()

    def step(i, carry):
        @pl.when(i > 4)
        def _():
            out_copy(i - 5).start()

        yb = b_down()
        store_out(jnp.maximum(i - 4, 0), yb[seg:])
        mem = a_out()
        mem2 = jnp.where(i == 2, mem0, mem[n_mem:])
        a_in(jnp.concatenate([mem[:n_mem], mem2], axis=0),
             x_segment(jnp.minimum(i, n_seg - 1)), yb[:seg])
        a_attention()
        b_gate_up()
        return carry

    jax.lax.fori_loop(2, n_seg + 2, step, 0)

    out_copy(n_seg - 3).start()
    store_out(n_seg - 2, b_down()[seg:])
    out_copy(n_seg - 2).start()
    a_out()
    b_gate_up()
    store_out(n_seg - 1, b_down()[seg:])
    out_copy(n_seg - 1).start()
    pltpu.make_async_copy(out_vm, out_hbm, out_sem).wait()


@functools.partial(jax.jit, static_argnames=("A_seg_len",))
def pallas_interleave_layers__memory_aug_recurrent_mem_tr__glu_gated_glu__prompt_kernel(
    A_x: jax.Array,
    A_mem0: jax.Array,
    A_Wq: jax.Array,
    A_Wk: jax.Array,
    A_Wv: jax.Array,
    A_Wo: jax.Array,
    A_seg_len: int,
    B_x: jax.Array,
    B_w_gate: jax.Array,
    B_w_up: jax.Array,
    B_w_down: jax.Array,
):
    del B_x
    B, S, D = A_x.shape
    _, H, Dh = A_Wq.shape
    M = A_mem0.shape[1]
    F = B_w_gate.shape[1]
    seg = int(A_seg_len)
    assert B == 1 and S % seg == 0 and S // seg >= 4
    RA = 2 * (M + seg)

    hbm = pl.BlockSpec(memory_space=pl.ANY)
    out = pl.pallas_call(
        functools.partial(_kernel, seg=seg, n_mem=M, n_heads=H, head_dim=Dh),
        out_shape=jax.ShapeDtypeStruct((S, D), A_x.dtype),
        in_specs=[hbm, pl.BlockSpec(memory_space=pltpu.VMEM)] + [hbm] * 7,
        out_specs=hbm,
        scratch_shapes=[
            pltpu.VMEM((S, D), A_x.dtype),
            pltpu.VMEM((S, D), A_x.dtype),
            pltpu.VMEM((STAGE_SLOTS, D_CHUNK * H, Dh), BF16),
            pltpu.VMEM((D, H * Dh), BF16),
            pltpu.VMEM((D, H * Dh), BF16),
            pltpu.VMEM((D, H * Dh), BF16),
            pltpu.VMEM((H * Dh, D), BF16),
            pltpu.VMEM((D, F), BF16),
            pltpu.VMEM((D, F), BF16),
            pltpu.VMEM((F, D), BF16),
            pltpu.VMEM((RA, D), BF16),
            pltpu.VMEM((RA, H * Dh), BF16),
            pltpu.VMEM((2 * seg, D), F32),
            pltpu.VMEM((2 * seg, D), F32),
            pltpu.VMEM((2 * seg, D), BF16),
            pltpu.VMEM((2 * seg, F), BF16),
            pltpu.SemaphoreType.DMA((STAGE_SLOTS,)),
            pltpu.SemaphoreType.DMA((5,)),
            pltpu.SemaphoreType.DMA(()),
        ],
        compiler_params=pltpu.CompilerParams(vmem_limit_bytes=110 * 2**20),
    )(
        A_x.reshape(S, D),
        A_mem0.reshape(M, D),
        A_Wq.reshape(D * H, Dh),
        A_Wk.reshape(D * H, Dh),
        A_Wv.reshape(D * H, Dh),
        A_Wo.reshape(H * Dh, D),
        B_w_gate,
        B_w_up,
        B_w_down,
    )
    return out.reshape(B, S, D)
```

```python
import functools
import itertools

import jax
import jax.numpy as jnp
import jax.experimental.pallas as pl
import jax.experimental.pallas.tpu as pltpu

F32 = jnp.float32
BF16 = jnp.bfloat16
U32 = jnp.uint32
LANES = 128
LN_EPS = 1e-5
MASK_VALUE = -1000000000.0

OFFSETS = (-1.375, -0.375, 0.375, 1.375)
GROUP = 4
STAGE_SLOTS = 3
STAGE_ROWS = 128


def _layernorm(x):
    m = jnp.mean(x, axis=-1, keepdims=True)
    c = x - m
    v = jnp.mean(c * c, axis=-1, keepdims=True)
    return c * jax.lax.rsqrt(v + LN_EPS)


def _split(x, n):
    w = x.shape[1] // n
    return [x[:, i * w:(i + 1) * w] for i in range(n)]


def _pairs(n):
    return list(itertools.combinations(range(n), 2))


def _row_operands(h1, h2):
    t, n = OFFSETS, len(OFFSETS)
    h1, h2 = _split(h1, n), _split(h2, n)
    b = [h2[i] - t[i] * h1[i] for i in range(n)]
    ops = h1 + b
    for i, j in _pairs(n):
        g1, g2 = h1[i] + h1[j], h2[i] + h2[j]
        ops += [b[i] + b[j], g2 - t[i] * g1, g2 - t[j] * g1]
    return ops


def _weight_operands(w):
    n = len(OFFSETS)
    add = lambda xs: functools.reduce(lambda a, b: a + b, xs)
    ops = [add(w[i]) for i in range(n)]
    ops += [w[i][i] - add([w[j][i] for j in range(n) if j != i]) for i in range(n)]
    for i, j in _pairs(n):
        ops += [w[i][j] + w[j][i], w[j][i], w[i][j]]
    return [pltpu.bitcast(op.astype(BF16), U32) for op in ops]


def _paired_matmul(product):
    t, n = OFFSETS, len(OFFSETS)
    y1 = [product(i) for i in range(n)]
    y2 = [product(n + i) for i in range(n)]
    for k, (i, j) in enumerate(_pairs(n)):
        s, ti, tj = (product(2 * n + 3 * k + c) for c in range(3))
        u = ti + tj - s
        if t[j] - t[i] != 1:
            u = u * (1.0 / (t[j] - t[i]))
        y1[i], y1[j] = y1[i] + u, y1[j] - u
        y2[i], y2[j] = y2[i] + ti, y2[j] + tj
    y2 = [y2[i] + t[i] * y1[i] for i in range(n)]
    return jnp.concatenate(y1, axis=1), jnp.concatenate(y2, axis=1)


def _project(rows_ref, w_ref, cols=slice(None)):
    def product(r):
        w = pltpu.bitcast(w_ref[r, :, cols], BF16)
        return jax.lax.dot_general(rows_ref[r], w, (((1,), (0,)), ((), ())),
                                   preferred_element_type=F32)
    return _paired_matmul(product)


def _store_rows(ref, h1, h2, cols=slice(None)):
    for r, op in enumerate(_row_operands(h1, h2)):
        ref[r, :, cols] = op.astype(ref.dtype)


def _kernel(x_hbm, mem0_ref, wq_hbm, wk_hbm, wv_hbm, wo_hbm, wg_hbm, wu_hbm, wd_hbm,
            out_hbm,
            x_vm, out_vm, wq, wk, wv, wo, wg, wu, wd,
            h_ref, o_ref, ra_ref, rb_ref, xb_ref, hb_ref,
            stage_sem, x_sem, out_sem, *, seg, n_mem, n_heads):
    S, D = x_vm.shape
    F = wg_hbm.shape[2]
    n_seg = S // seg
    L = n_mem + seg
    n = len(OFFSETS)
    gw = GROUP * LANES
    bw = gw // n
    scale = LANES ** -0.5

    def stream(jobs, stage):
        starts = [sum(j[0] for j in jobs[:m]) for m in range(len(jobs))]

        def copy(m, c, slot):
            return pltpu.make_async_copy(jobs[m][1](c), stage.at[slot], stage_sem.at[slot])

        for c in range(STAGE_SLOTS):
            copy(0, c, c).start()
        for m, (count, _, consume) in enumerate(jobs):
            def body(c, carry, m=m, count=count, consume=consume):
                slot = (starts[m] + c) % STAGE_SLOTS
                copy(m, c, slot).wait()
                consume(c, stage.at[slot])
                nxt = c + STAGE_SLOTS

                @pl.when(nxt < count)
                def _():
                    copy(m, nxt, slot).start()

                if m + 1 < len(jobs):
                    @pl.when(nxt >= count)
                    def _():
                        copy(m + 1, nxt - count, slot).start()
                return carry

            jax.lax.fori_loop(0, count, body, 0)

    kr = STAGE_ROWS // n

    def wide_job(src, dst, per_row, load):
        def consume(c, staged):
            blocks = [load(staged, i).astype(F32) for i in range(n)]
            rows = pl.ds(pl.multiple_of(c * (kr // 2), kr // 2), kr // 2)
            for g in range(blocks[0].shape[1] // gw):
                w = [_split(blk[:, g * gw:(g + 1) * gw], n) for blk in blocks]
                for r, op in enumerate(_weight_operands(w)):
                    dst[r, rows, pl.ds(g * bw, bw)] = op
        step = kr * per_row
        return (D // STAGE_ROWS,
                lambda c: src.at[:, pl.ds(pl.multiple_of(c * step, step), step), :],
                consume)

    def tall_job(src, dst):
        def consume(c, staged):
            w = [_split(staged[pl.ds(i * bw, bw), :].astype(F32), n) for i in range(n)]
            rows = pl.ds(pl.multiple_of(c * (bw // 2), bw // 2), bw // 2)
            for r, op in enumerate(_weight_operands(w)):
                dst[r, rows, :] = op
        return (src.shape[0] // gw,
                lambda c: src.at[pl.ds(pl.multiple_of(c * gw, gw), gw), :],
                consume)

    def load_heads(staged, i):
        return staged[i].reshape(kr, n_heads, LANES).reshape(kr, n_heads * LANES)

    x_copy = pltpu.make_async_copy(x_hbm, x_vm, x_sem)
    x_copy.start()
    o_ref[...] = jnp.zeros(o_ref.shape, o_ref.dtype)
    rb_ref[...] = jnp.zeros(rb_ref.shape, rb_ref.dtype)
    pl.run_scoped(
        functools.partial(stream, [wide_job(s, d, n_heads, load_heads) for s, d in
                                   ((wq_hbm, wq), (wk_hbm, wk), (wv_hbm, wv))]),
        pltpu.VMEM((STAGE_SLOTS, n, kr * n_heads, LANES), BF16))
    pl.run_scoped(
        functools.partial(stream, [tall_job(wo_hbm, wo), tall_job(wd_hbm, wd)]),
        pltpu.VMEM((STAGE_SLOTS, gw, D), BF16))
    pl.run_scoped(
        functools.partial(stream, [wide_job(s, d, 1, lambda staged, i: staged[i]) for s, d in
                                   ((wg_hbm, wg), (wu_hbm, wu))]),
        pltpu.VMEM((STAGE_SLOTS, n, kr, F), BF16))

    def attention_mask():
        q = jax.lax.broadcasted_iota(jnp.int32, (2 * L, 2 * L), 0)
        k = jax.lax.broadcasted_iota(jnp.int32, (2 * L, 2 * L), 1)
        same = (q >= L) == (k >= L)
        keep = same & ((jnp.where(q >= L, q - L, q) < n_mem) | (q >= k))
        fill = jnp.where(same, MASK_VALUE, -jnp.inf).astype(F32)
        return keep, fill

    def b_down():
        y1, y2 = _project(hb_ref, wd)
        return rb_ref[0] + y1, rb_ref[1] + y2

    def a_out():
        y1, y2 = _project(o_ref, wo)
        r1, r2 = ra_ref[0] + y1[n_mem:], ra_ref[1] + y2[n_mem:]
        rb_ref[0], rb_ref[1] = r1, r2
        _store_rows(xb_ref, _layernorm(r1), _layernorm(r2))
        return y1[:n_mem], y2[:n_mem]

    def a_in(mem1, x1, mem2, x2):
        ra_ref[0], ra_ref[1] = x1, x2
        _store_rows(h_ref, jnp.concatenate([mem1, _layernorm(x1)], axis=0),
                    jnp.concatenate([mem2, _layernorm(x2)], axis=0))

    def qkv(g):
        return tuple(
            jnp.concatenate(_project(h_ref, w, pl.ds(g * bw, bw)), axis=0).astype(BF16)
            for w in (wq, wk, wv))

    def attend(g, q, k, v):
        keep, fill = attention_mask()
        heads = []
        for qh, kh, vh in zip(*(_split(a, GROUP) for a in (q, k, v))):
            s = jax.lax.dot_general(qh, kh, (((1,), (1,)), ((), ())),
                                    preferred_element_type=F32)
            s = jnp.where(keep, s * scale, fill)
            p = jnp.exp(s - jnp.max(s, axis=-1, keepdims=True))
            inv = 1.0 / jnp.sum(p, axis=-1, keepdims=True)
            heads.append(jnp.dot(p.astype(BF16), vh, preferred_element_type=F32) * inv)
        o = jnp.concatenate(heads, axis=1)
        _store_rows(o_ref, o[:L], o[L:], pl.ds(g * bw, bw))

    def gate_up(c):
        cols = pl.ds(c * bw, bw)
        g1, g2 = _project(xb_ref, wg, cols)
        u1, u2 = _project(xb_ref, wu, cols)
        _store_rows(hb_ref, jax.nn.sigmoid(g1) * u1, jax.nn.sigmoid(g2) * u2, cols)

    def run(attention, glu):
        pending = None
        for g in range(n_heads // GROUP if attention else 0):
            cur = (g,) + qkv(g)
            if pending:
                attend(*pending)
            pending = cur
        for c in range(F // gw if glu else 0):
            gate_up(c)
            if pending:
                attend(*pending)
                pending = None
        if pending:
            attend(*pending)

    def segment(i):
        return pl.ds(pl.multiple_of(i * seg, seg), seg)

    def out_copy(i):
        return pltpu.make_async_copy(out_vm.at[segment(i)], out_hbm.at[segment(i)], out_sem)

    def store_out(i, y):
        out_vm[segment(i), :] = y.astype(out_vm.dtype)

    mem0 = mem0_ref[...].astype(F32)
    zeros = jnp.zeros((seg, D), F32)

    x_copy.wait()
    a_in(mem0, x_vm[segment(0), :].astype(F32), mem0, zeros)
    run(True, False)
    mem1, mem2 = a_out()
    a_in(mem1, x_vm[segment(1), :].astype(F32), mem2, zeros)
    run(True, True)

    def step(i, carry):
        @pl.when(i > 4)
        def _():
            out_copy(i - 5).start()

        x2, y = b_down()
        store_out(jnp.maximum(i - 4, 0), y)
        mem1, mem2 = a_out()
        x1 = x_vm[segment(jnp.minimum(i, n_seg - 1)), :].astype(F32)
        a_in(mem1, x1, jnp.where(i == 2, mem0, mem2), x2)
        run(True, True)
        return carry

    jax.lax.fori_loop(2, n_seg + 2, step, 0)

    out_copy(n_seg - 3).start()
    store_out(n_seg - 2, b_down()[1])
    out_copy(n_seg - 2).start()
    a_out()
    run(False, True)
    store_out(n_seg - 1, b_down()[1])
    out_copy(n_seg - 1).start()
    pltpu.make_async_copy(out_vm, out_hbm, out_sem).wait()


@functools.partial(jax.jit, static_argnames=("A_seg_len",))
def pallas_interleave_layers__memory_aug_recurrent_mem_tr__glu_gated_glu__prompt_kernel(
    A_x: jax.Array,
    A_mem0: jax.Array,
    A_Wq: jax.Array,
    A_Wk: jax.Array,
    A_Wv: jax.Array,
    A_Wo: jax.Array,
    A_seg_len: int,
    B_x: jax.Array,
    B_w_gate: jax.Array,
    B_w_up: jax.Array,
    B_w_down: jax.Array,
):
    del B_x
    B, S, D = A_x.shape
    _, H, Dh = A_Wq.shape
    M = A_mem0.shape[1]
    F = B_w_gate.shape[1]
    seg = int(A_seg_len)
    assert B == 1 and Dh == LANES and S % seg == 0 and S // seg >= 4
    n = len(OFFSETS)
    R = (3 * n * n + n) // 2
    L = M + seg

    def packed(k, cols):
        return pltpu.VMEM((R, k // n // 2, cols // n), U32)

    hbm = pl.BlockSpec(memory_space=pl.ANY)
    out = pl.pallas_call(
        functools.partial(_kernel, seg=seg, n_mem=M, n_heads=H),
        out_shape=jax.ShapeDtypeStruct((S, D), A_x.dtype),
        in_specs=[hbm, pl.BlockSpec(memory_space=pltpu.VMEM)] + [hbm] * 7,
        out_specs=hbm,
        scratch_shapes=[
            pltpu.VMEM((S, D), A_x.dtype),
            pltpu.VMEM((S, D), A_x.dtype),
            packed(D, H * Dh),
            packed(D, H * Dh),
            packed(D, H * Dh),
            packed(H * Dh, D),
            packed(D, F),
            packed(D, F),
            packed(F, D),
            pltpu.VMEM((R, L, D // n), F32),
            pltpu.VMEM((R, L, H * Dh // n), F32),
            pltpu.VMEM((2, seg, D), F32),
            pltpu.VMEM((2, seg, D), F32),
            pltpu.VMEM((R, seg, D // n), BF16),
            pltpu.VMEM((R, seg, F // n), BF16),
            pltpu.SemaphoreType.DMA((STAGE_SLOTS,)),
            pltpu.SemaphoreType.DMA(()),
            pltpu.SemaphoreType.DMA(()),
        ],
        compiler_params=pltpu.CompilerParams(vmem_limit_bytes=120 * 2**20),
    )(
        A_x.reshape(S, D),
        A_mem0.reshape(M, D),
        A_Wq.reshape(n, D // n * H, Dh),
        A_Wk.reshape(n, D // n * H, Dh),
        A_Wv.reshape(n, D // n * H, Dh),
        A_Wo.reshape(H * Dh, D),
        B_w_gate.reshape(n, D // n, F),
        B_w_up.reshape(n, D // n, F),
        B_w_down,
    )
    return out.reshape(B, S, D)
```

```python
import functools

import jax
import jax.numpy as jnp
import jax.experimental.pallas as pl
import jax.experimental.pallas.tpu as pltpu

F32 = jnp.float32
BF16 = jnp.bfloat16
U32 = jnp.uint32
LANES = 128
LN_EPS = 1e-5
MASK_VALUE = -1000000000.0

OFFSETS = (-1.375, -0.375, 0.375, 1.375)
GROUP = 4
QKV_SLOTS, TALL_SLOTS, WIDE_SLOTS = 3, 6, 7
ROWS = 16
B_DTYPE = F32
FLAGS = None
ORDER = 'mxDahasasasasasasasbsbbbbbbW'
STAGE_ROWS = 128


def _layernorm(x):
    m = jnp.mean(x, axis=-1, keepdims=True)
    c = x - m
    v = jnp.mean(c * c, axis=-1, keepdims=True)
    return c * jax.lax.rsqrt(v + LN_EPS)


def _sigmoid(x):
    return 0.5 * jnp.tanh(0.5 * x) + 0.5


def _reciprocal(x):
    r = pl.reciprocal(x, approx=True)
    return r * (2.0 - x * r)


def _split(x, n):
    w = x.shape[1] // n
    return [x[:, i * w:(i + 1) * w] for i in range(n)]


def _pairs(n):
    return [(i, j) for j in range(n) for i in range(j)]


def _row_operands(h1, h2):
    t, n = OFFSETS, len(OFFSETS)
    if h1 is None:
        ops = [None] * n + list(h2)
        for i, j in _pairs(n):
            g2 = h2[i] + h2[j]
            ops += [None, g2, g2]
        return ops
    b = [h2[i] - t[i] * h1[i] for i in range(n)]
    ops = list(h1) + b
    for i, j in _pairs(n):
        s, d = b[i] + b[j], t[j] - t[i]
        ops += [s, s + d * h1[j], s - d * h1[i]]
    return ops


def _weight_operands(w):
    n = len(OFFSETS)
    add = lambda xs: functools.reduce(lambda a, b: a + b, xs)
    ops = [add(w[i]) for i in range(n)]
    ops += [w[i][i] - add([w[j][i] for j in range(n) if j != i]) for i in range(n)]
    for i, j in _pairs(n):
        ops += [w[i][j] + w[j][i], w[j][i], w[i][j]]
    return [pltpu.bitcast(op.astype(BF16), U32) for op in ops]


def _paired_matmul(product, both):
    t, n = OFFSETS, len(OFFSETS)
    y1, y2 = [None] * n, [None] * n
    acc = lambda a, b: b if a is None else a + b
    todo = [n - 1] * n
    for k, (i, j) in enumerate(_pairs(n)):
        ti, tj = product(2 * n + 3 * k + 1), product(2 * n + 3 * k + 2)
        y2[i], y2[j] = acc(y2[i], ti), acc(y2[j], tj)
        if both:
            u = (ti + tj - product(2 * n + 3 * k)) * (1.0 / (t[j] - t[i]))
            y1[i], y1[j] = acc(y1[i], u), (-u if y1[j] is None else y1[j] - u)
        for m in (i, j):
            todo[m] -= 1
            if todo[m] == 0:
                y2[m] = y2[m] + product(n + m)
                if both:
                    y1[m] = y1[m] + product(m)
                    y2[m] = y2[m] + t[m] * y1[m]
    return (y1 if both else None), y2


def _project(rows_ref, w_ref, both, cols=slice(None)):
    def product(r):
        w = pltpu.bitcast(w_ref[r, :, cols], BF16)
        return jax.lax.dot_general(rows_ref[r], w, (((1,), (0,)), ((), ())),
                                   preferred_element_type=F32)
    return _paired_matmul(product, both)


def _store_rows(ref, h1, h2, rows=slice(None), cols=slice(None)):
    for r, op in enumerate(_row_operands(h1, h2)):
        if op is not None:
            ref[r, rows, cols] = op.astype(ref.dtype)


def _kernel(x_hbm, mem0_ref, wq_hbm, wk_hbm, wv_hbm, wo_hbm, wg_hbm, wu_hbm, wd_hbm,
            out_hbm,
            x_vm, out_vm, wq, wk, wv, wo, wg, wu, wd,
            h_ref, o_ref, xb_ref, hb_ref, mem_ref, ra_ref, rn_ref, rb_ref, x2_ref, fill_ref,
            x_sem, out_sem, *, seg, n_mem, n_heads):
    S, D = x_vm.shape
    F = wg_hbm.shape[2]
    n_seg = S // seg
    L = n_mem + seg
    n = len(OFFSETS)
    gw = GROUP * LANES
    bw = gw // n
    n_a, n_b = n_heads // GROUP, F // gw
    scale = LANES ** -0.5

    class Stream:
        def __init__(self, jobs, stage, sems):
            self.jobs, self.stage, self.sems = jobs, stage, sems
            self.slots = stage.shape[0]

        def copy(self, m, c, slot):
            return pltpu.make_async_copy(self.jobs[m][1](c), self.stage.at[slot],
                                         self.sems.at[slot])

        def start(self, first=0, last=None):
            for c in range(first, self.slots if last is None else last):
                self.copy(0, c, c).start()

        def drain(self, m, refill=None):
            count, _, consume = self.jobs[m]
            first = sum(j[0] for j in self.jobs[:m])

            def body(c, carry):
                slot = (first + c) % self.slots
                self.copy(m, c, slot).wait()
                consume(c, self.stage.at[slot])
                nxt = c + self.slots
                if self.slots < count:
                    pl.when(nxt < count)(lambda: self.copy(m, nxt, slot).start())
                if m + 1 < len(self.jobs):
                    pl.when(nxt >= count)(lambda: self.copy(m + 1, nxt - count, slot).start())
                elif refill:
                    for k in range(self.slots):
                        pl.when(nxt == count + k)(functools.partial(refill, k))
                return carry

            jax.lax.fori_loop(0, count, body, 0)

    kr = STAGE_ROWS // n

    def wide_job(src, dst, per_row, load):
        def consume(c, staged):
            blocks = [load(staged, i).astype(F32) for i in range(n)]
            rows = pl.ds(pl.multiple_of(c * (kr // 2), kr // 2), kr // 2)
            for g in range(blocks[0].shape[1] // gw):
                w = [_split(blk[:, g * gw:(g + 1) * gw], n) for blk in blocks]
                for r, op in enumerate(_weight_operands(w)):
                    dst[r, rows, pl.ds(g * bw, bw)] = op
        step = kr * per_row
        return (D // STAGE_ROWS,
                lambda c: src.at[:, pl.ds(pl.multiple_of(c * step, step), step), :],
                consume)

    def tall_job(src, dst):
        def consume(c, staged):
            w = [_split(staged[pl.ds(i * bw, bw), :].astype(F32), n) for i in range(n)]
            rows = pl.ds(pl.multiple_of(c * (bw // 2), bw // 2), bw // 2)
            for r, op in enumerate(_weight_operands(w)):
                dst[r, rows, :] = op
        return (src.shape[0] // gw,
                lambda c: src.at[pl.ds(pl.multiple_of(c * gw, gw), gw), :],
                consume)

    def load_heads(staged, i):
        return staged[i].reshape(kr, n_heads, LANES).reshape(kr, n_heads * LANES)

    qi = jax.lax.broadcasted_iota(jnp.int32, fill_ref.shape, 0)
    ki = jax.lax.broadcasted_iota(jnp.int32, fill_ref.shape, 1)
    q_pass = jnp.where(qi >= L, 1, 0)
    q_pos = qi - L * q_pass
    same = (q_pass == (ki & 1)) & (ki < 2 * L)
    visible = (q_pos < n_mem) | (q_pos >= (ki >> 1))
    fill_ref[...] = jnp.where(same, jnp.where(visible, 0.0, MASK_VALUE), -jnp.inf)

    BOTH, FIRST, SECOND = (0, 1), (0,), (1,)
    join = lambda blocks: jnp.concatenate(blocks, axis=1)

    def store_rows(ref, h, **where):
        _store_rows(ref, h[0] if len(h) == 2 else None, h[-1], **where)

    def project(rows_ref, w_ref, live, cols=slice(None)):
        return _project(rows_ref, w_ref, len(live) == 2, cols)[-len(live):]

    def segment(i, start=0, size=seg):
        return pl.ds(pl.multiple_of(i * seg + start, size), size)

    def segments_in(i, live):
        for r in range(0, seg, ROWS):
            x = [x2_ref[pl.ds(r, ROWS), :] if p else x_vm[segment(i, r, ROWS), :].astype(F32)
                 for p in live]
            for p, xp in zip(live, x):
                ra_ref[p, pl.ds(r, ROWS), :] = xp
            store_rows(h_ref, [_split(_layernorm(xp), n) for xp in x],
                       rows=pl.ds(n_mem + r, ROWS))

    def memories_in(live):
        store_rows(h_ref, [_split(mem_ref[p], n) for p in live], rows=pl.ds(0, n_mem))

    def interleave(a, b):
        words = pltpu.pack_elementwise([a, b], packed_dtype=BF16)
        pad = jnp.zeros((LANES // 2 - L, LANES), words.dtype)
        return pltpu.bitcast(jnp.concatenate([words, pad], axis=0), BF16)

    def qkv(cols, live):
        out = []
        for w in (wk, wv, wq):
            y = project(h_ref, w, live, cols)
            heads = zip(*([h for blk in yp for h in _split(blk, bw // LANES)] for yp in y))
            out.append([jnp.concatenate(h, axis=0) if w is wq else interleave(h[0], h[-1])
                        for h in heads])
        return out

    def attend(cols, live, k, v, q):
        o = []
        for qh, kh, vh in zip(q, k, v):
            s = jax.lax.dot_general(qh, kh, (((1,), (1,)), ((), ())),
                                    preferred_element_type=F32)
            fill = fill_ref[pl.ds(0, len(live) * L), :]
            s = jnp.where(fill == 0.0, s * scale, fill)
            p = jnp.exp(s - jnp.max(s, axis=-1, keepdims=True))
            p = p * _reciprocal(jnp.sum(p, axis=-1, keepdims=True))
            o.append(jax.lax.dot_general(p, vh, (((1,), (0,)), ((), ())),
                                         preferred_element_type=F32))
        per = GROUP // n
        o = [join(o[i * per:(i + 1) * per]) for i in range(n)]
        store_rows(o_ref, [[a[p * L:(p + 1) * L] for a in o] for p in range(len(live))],
                   cols=cols)

    def attention_out(live):
        for p, y in zip(live, project(o_ref, wo, live)):
            y = join(y)
            mem_ref[p] = y[:n_mem]
            rn_ref[p] = ra_ref[p] + y[n_mem:]

    def hand_over(live):
        for r in range(0, seg, ROWS):
            x = [rn_ref[p, pl.ds(r, ROWS), :] for p in live]
            for p, xp in zip(live, x):
                rb_ref[p, pl.ds(r, ROWS), :] = xp
            store_rows(xb_ref, [_split(_layernorm(xp), n) for xp in x], rows=pl.ds(r, ROWS))

    def gate_up(cols, live):
        g, u = project(xb_ref, wg, live, cols), project(xb_ref, wu, live, cols)
        h = [[_sigmoid(a) * b for a, b in zip(gp, up)] for gp, up in zip(g, u)]
        zero = [jnp.zeros_like(a) for a in h[0]]
        _store_rows(hb_ref, h[0] if 0 in live else zero, h[-1] if 1 in live else zero, cols=cols)

    def glu_out(done):
        y1, y2 = project(hb_ref, wd, BOTH)
        x2_ref[...] = rb_ref[0] + join(y1)
        out_vm[segment(done), :] = (rb_ref[1] + join(y2)).astype(out_vm.dtype)

    def chunk(c):
        return pl.ds(c * bw if isinstance(c, int) else pl.multiple_of(c * bw, bw), bw)

    def attention_loop(i, live):
        segments_in(i, live)
        memories_in(live)

        def body(g, carry):
            first = qkv(chunk(2 * g), live)
            second = qkv(chunk(2 * g + 1), live)
            attend(chunk(2 * g), live, *first)
            attend(chunk(2 * g + 1), live, *second)
            return carry
        jax.lax.fori_loop(0, n_a // 2, body, 0)

    def glu_loop(live):
        hand_over(live)

        def body(c, carry):
            gate_up(chunk(c), live)
            return carry
        jax.lax.fori_loop(0, n_b, body, 0)

    def out_copy(i):
        return pltpu.make_async_copy(out_vm.at[segment(i)], out_hbm.at[segment(i)], out_sem)

    head = pl.ds(0, 4 * seg)
    tail = pl.ds(4 * seg, S - 4 * seg)
    x_head = pltpu.make_async_copy(x_hbm.at[head], x_vm.at[head], x_sem.at[0])
    x_tail = pltpu.make_async_copy(x_hbm.at[tail], x_vm.at[tail], x_sem.at[1])

    def fill(tall_stage, tall_sems, wide_stage, wide_sems):
        tall = Stream([tall_job(wo_hbm, wo)], tall_stage, tall_sems)
        down = Stream([tall_job(wd_hbm, wd)], tall_stage, tall_sems)
        wide = Stream([wide_job(s, d, 1, lambda staged, i: staged[i])
                       for s, d in ((wg_hbm, wg), (wu_hbm, wu))], wide_stage, wide_sems)

        def refill(stream, slots):
            return lambda k: stream.start(k * stream.slots // slots,
                                          (k + 1) * stream.slots // slots)

        def load_qkv(stage, sems):
            qkv_stream = Stream([wide_job(s, d, n_heads, load_heads) for s, d in
                                 ((wq_hbm, wq), (wk_hbm, wk), (wv_hbm, wv))], stage, sems)
            qkv_stream.start()
            x_head.start()
            for m in range(3):
                qkv_stream.drain(m, refill(tall, qkv_stream.slots))

        pl.run_scoped(load_qkv, pltpu.VMEM((QKV_SLOTS, n, kr * n_heads, LANES), BF16),
                      pltpu.SemaphoreType.DMA((QKV_SLOTS,)))
        mem_ref[0] = mem_ref[1] = mem0_ref[...].astype(F32)
        rn_ref[1] = rb_ref[1] = jnp.zeros((seg, D), F32)
        x_head.wait()

        def step(i, carry):
            attention_loop(i, FIRST)
            pl.when(i == 0)(lambda: tall.drain(0, refill(wide, tall.slots)))

            @pl.when(i == 1)
            def _():
                wide.drain(0)
                wide.drain(1, refill(down, wide.slots))

            @pl.when(i == 2)
            def _():
                down.drain(0, lambda k: x_tail.start() if k == 0 else None)
                glu_out(0)

            pl.when(i > 0)(lambda: glu_loop(FIRST))
            attention_out(FIRST)
            return carry

        jax.lax.fori_loop(0, 3, step, 0)

    pl.run_scoped(fill, pltpu.VMEM((TALL_SLOTS, gw, D), BF16),
                  pltpu.SemaphoreType.DMA((TALL_SLOTS,)),
                  pltpu.VMEM((WIDE_SLOTS, n, kr, F), BF16),
                  pltpu.SemaphoreType.DMA((WIDE_SLOTS,)))

    def step(i, carry):
        pl.when(i == 4)(x_tail.wait)
        pl.when(i > 5)(lambda: out_copy(i - 6).start())
        pending, g, c = [], 0, 0
        for what in ORDER:
            if what == 'x':
                segments_in(jnp.minimum(i, n_seg - 1), BOTH)
            elif what == 'm':
                memories_in(BOTH)
            elif what == 'D':
                glu_out(jnp.maximum(i - 5, 0))
            elif what == 'h':
                hand_over(BOTH)
            elif what == 'a':
                pending.append((chunk(g), BOTH, *qkv(chunk(g), BOTH)))
                g += 1
            elif what == 's':
                attend(*pending.pop(0))
            elif what == 'b':
                gate_up(chunk(c), BOTH)
                c += 1
            elif what == 'W':
                attention_out(BOTH)
        assert (g, c, pending) == (n_a, n_b, [])
        return carry

    jax.lax.fori_loop(3, n_seg + 1, step, 0)

    def drain_step(i, carry):
        out_copy(i - 6).start()
        pl.when(i < n_seg + 3)(lambda: attention_loop(i, SECOND))
        glu_out(i - 5)
        pl.when(i < n_seg + 4)(lambda: glu_loop(SECOND))
        pl.when(i < n_seg + 3)(lambda: attention_out(SECOND))
        return carry

    jax.lax.fori_loop(n_seg + 1, n_seg + 5, drain_step, 0)
    out_copy(n_seg - 1).start()
    pltpu.make_async_copy(out_vm, out_hbm, out_sem).wait()


@functools.partial(jax.jit, static_argnames=("A_seg_len",))
def pallas_interleave_layers__memory_aug_recurrent_mem_tr__glu_gated_glu__prompt_kernel(
    A_x: jax.Array,
    A_mem0: jax.Array,
    A_Wq: jax.Array,
    A_Wk: jax.Array,
    A_Wv: jax.Array,
    A_Wo: jax.Array,
    A_seg_len: int,
    B_x: jax.Array,
    B_w_gate: jax.Array,
    B_w_up: jax.Array,
    B_w_down: jax.Array,
):
    del B_x
    B, S, D = A_x.shape
    _, H, Dh = A_Wq.shape
    M = A_mem0.shape[1]
    F = B_w_gate.shape[1]
    seg = int(A_seg_len)
    assert B == 1 and Dh == LANES and S % seg == 0 and S // seg >= 8
    n = len(OFFSETS)
    R = (3 * n * n + n) // 2
    L = M + seg

    def packed(k, cols):
        return pltpu.VMEM((R, k // n // 2, cols // n), U32)

    hbm = pl.BlockSpec(memory_space=pl.ANY)
    out = pl.pallas_call(
        functools.partial(_kernel, seg=seg, n_mem=M, n_heads=H),
        out_shape=jax.ShapeDtypeStruct((S, D), A_x.dtype),
        in_specs=[hbm, pl.BlockSpec(memory_space=pltpu.VMEM)] + [hbm] * 7,
        out_specs=hbm,
        scratch_shapes=[
            pltpu.VMEM((S, D), A_x.dtype),
            pltpu.VMEM((S, D), A_x.dtype),
            packed(D, H * Dh),
            packed(D, H * Dh),
            packed(D, H * Dh),
            packed(H * Dh, D),
            packed(D, F),
            packed(D, F),
            packed(F, D),
            pltpu.VMEM((R, L, D // n), F32),
            pltpu.VMEM((R, L, H * Dh // n), F32),
            pltpu.VMEM((R, seg, D // n), B_DTYPE),
            pltpu.VMEM((R, seg, F // n), B_DTYPE),
            pltpu.VMEM((2, M, D), F32),
            pltpu.VMEM((2, seg, D), F32),
            pltpu.VMEM((2, seg, D), F32),
            pltpu.VMEM((2, seg, D), F32),
            pltpu.VMEM((seg, D), F32),
            pltpu.VMEM((2 * L, LANES), F32),
            pltpu.SemaphoreType.DMA((2,)),
            pltpu.SemaphoreType.DMA(()),
        ],
        compiler_params=pltpu.CompilerParams(vmem_limit_bytes=124 * 2**20, flags=FLAGS),
    )(
        A_x.reshape(S, D),
        A_mem0.reshape(M, D),
        A_Wq.reshape(n, D // n * H, Dh),
        A_Wk.reshape(n, D // n * H, Dh),
        A_Wv.reshape(n, D // n * H, Dh),
        A_Wo.reshape(H * Dh, D),
        B_w_gate.reshape(n, D // n, F),
        B_w_up.reshape(n, D // n, F),
        B_w_down,
    )
    return out.reshape(B, S, D)
```

```python
import functools

import jax
import jax.numpy as jnp
import jax.experimental.pallas as pl
import jax.experimental.pallas.tpu as pltpu

F32 = jnp.float32
BF16 = jnp.bfloat16
U32 = jnp.uint32
LANES = 128
LN_EPS = 1e-5
MASK_VALUE = -1000000000.0

OFFSETS = (-1.375, -0.375, 0.375, 1.375)
GROUP = 4
QKV_SLOTS, TALL_SLOTS, WIDE_SLOTS = 3, 6, 7
ROWS = 16
B_DTYPE = F32
FLAGS = None
ORDER = 'mxD' + 'qkvS' + 'qPkvS' * 7 + 'DPh' + 'guG' * 7 + 'WW'
STAGE_ROWS = 128


def _layernorm(x):
    m = jnp.mean(x, axis=-1, keepdims=True)
    c = x - m
    v = jnp.mean(c * c, axis=-1, keepdims=True)
    return c * jax.lax.rsqrt(v + LN_EPS)


def _sigmoid(x):
    return 0.5 * jnp.tanh(0.5 * x) + 0.5


def _reciprocal(x):
    r = pl.reciprocal(x, approx=True)
    return r * (2.0 - x * r)


def _split(x, n):
    w = x.shape[1] // n
    return [x[:, i * w:(i + 1) * w] for i in range(n)]


def _pairs(n):
    return [(i, j) for j in range(n) for i in range(j)]


def _row_operands(h1, h2):
    t, n = OFFSETS, len(OFFSETS)
    if h1 is None:
        ops = [None] * n + list(h2)
        for i, j in _pairs(n):
            g2 = h2[i] + h2[j]
            ops += [None, g2, g2]
        return ops
    b = [h2[i] - t[i] * h1[i] for i in range(n)]
    ops = list(h1) + b
    for i, j in _pairs(n):
        s, d = b[i] + b[j], t[j] - t[i]
        ops += [s, s + d * h1[j], s - d * h1[i]]
    return ops


def _weight_operands(w):
    n = len(OFFSETS)
    add = lambda xs: functools.reduce(lambda a, b: a + b, xs)
    ops = [add(w[i]) for i in range(n)]
    ops += [w[i][i] - add([w[j][i] for j in range(n) if j != i]) for i in range(n)]
    for i, j in _pairs(n):
        ops += [w[i][j] + w[j][i], w[j][i], w[i][j]]
    return [pltpu.bitcast(op.astype(BF16), U32) for op in ops]


def _paired_matmul(product, both):
    t, n = OFFSETS, len(OFFSETS)
    y1, y2 = [None] * n, [None] * n
    acc = lambda a, b: b if a is None else a + b
    todo = [n - 1] * n
    for k, (i, j) in enumerate(_pairs(n)):
        ti, tj = product(2 * n + 3 * k + 1), product(2 * n + 3 * k + 2)
        y2[i], y2[j] = acc(y2[i], ti), acc(y2[j], tj)
        if both:
            u = (ti + tj - product(2 * n + 3 * k)) * (1.0 / (t[j] - t[i]))
            y1[i], y1[j] = acc(y1[i], u), (-u if y1[j] is None else y1[j] - u)
        for m in (i, j):
            todo[m] -= 1
            if todo[m] == 0:
                y2[m] = y2[m] + product(n + m)
                if both:
                    y1[m] = y1[m] + product(m)
                    y2[m] = y2[m] + t[m] * y1[m]
    return (y1 if both else None), y2


def _project(rows_ref, w_ref, both, cols=slice(None)):
    def product(r):
        w = pltpu.bitcast(w_ref[r, :, cols], BF16)
        return jax.lax.dot_general(rows_ref[r], w, (((1,), (0,)), ((), ())),
                                   preferred_element_type=F32)
    return _paired_matmul(product, both)


def _store_rows(ref, h1, h2, rows=slice(None), cols=slice(None)):
    for r, op in enumerate(_row_operands(h1, h2)):
        if op is not None:
            ref[r, rows, cols] = op.astype(ref.dtype)


def _kernel(x_hbm, mem0_ref, wq_hbm, wk_hbm, wv_hbm, wo_hbm, wg_hbm, wu_hbm, wd_hbm,
            out_hbm,
            x_vm, out_vm, wq, wk, wv, wo, wg, wu, wd,
            h_ref, o_ref, xb_ref, hb_ref, mem_ref, ra_ref, rn_ref, rb_ref, x2_ref, fill_ref,
            x_sem, out_sem, *, seg, n_mem, n_heads):
    S, D = x_vm.shape
    F = wg_hbm.shape[2]
    n_seg = S // seg
    L = n_mem + seg
    n = len(OFFSETS)
    gw = GROUP * LANES
    bw = gw // n
    n_a, n_b = n_heads // GROUP, F // gw
    scale = LANES ** -0.5

    class Stream:
        def __init__(self, jobs, stage, sems):
            self.jobs, self.stage, self.sems = jobs, stage, sems
            self.slots = stage.shape[0]

        def copy(self, m, c, slot):
            return pltpu.make_async_copy(self.jobs[m][1](c), self.stage.at[slot],
                                         self.sems.at[slot])

        def start(self, first=0, last=None):
            for c in range(first, self.slots if last is None else last):
                self.copy(0, c, c).start()

        def drain(self, m, refill=None):
            count, _, consume = self.jobs[m]
            first = sum(j[0] for j in self.jobs[:m])

            def body(c, carry):
                slot = (first + c) % self.slots
                self.copy(m, c, slot).wait()
                consume(c, self.stage.at[slot])
                nxt = c + self.slots
                if self.slots < count:
                    pl.when(nxt < count)(lambda: self.copy(m, nxt, slot).start())
                if m + 1 < len(self.jobs):
                    pl.when(nxt >= count)(lambda: self.copy(m + 1, nxt - count, slot).start())
                elif refill:
                    for k in range(self.slots):
                        pl.when(nxt == count + k)(functools.partial(refill, k))
                return carry

            jax.lax.fori_loop(0, count, body, 0)

    kr = STAGE_ROWS // n

    def wide_job(src, dst, per_row, load):
        def consume(c, staged):
            blocks = [load(staged, i).astype(F32) for i in range(n)]
            rows = pl.ds(pl.multiple_of(c * (kr // 2), kr // 2), kr // 2)
            for g in range(blocks[0].shape[1] // gw):
                w = [_split(blk[:, g * gw:(g + 1) * gw], n) for blk in blocks]
                for r, op in enumerate(_weight_operands(w)):
                    dst[r, rows, pl.ds(g * bw, bw)] = op
        step = kr * per_row
        return (D // STAGE_ROWS,
                lambda c: src.at[:, pl.ds(pl.multiple_of(c * step, step), step), :],
                consume)

    def tall_job(src, dst):
        def consume(c, staged):
            rows = pl.ds(pl.multiple_of(c * (bw // 2), bw // 2), bw // 2)
            for g in range(D // gw):
                w = [_split(staged[pl.ds(i * bw, bw), pl.ds(g * gw, gw)].astype(F32), n)
                     for i in range(n)]
                for r, op in enumerate(_weight_operands(w)):
                    dst[r, rows, pl.ds(g * bw, bw)] = op
        return (src.shape[0] // gw,
                lambda c: src.at[pl.ds(pl.multiple_of(c * gw, gw), gw), :],
                consume)

    def load_heads(staged, i):
        return staged[i].reshape(kr, n_heads, LANES).reshape(kr, n_heads * LANES)

    qi = jax.lax.broadcasted_iota(jnp.int32, fill_ref.shape, 0)
    ki = jax.lax.broadcasted_iota(jnp.int32, fill_ref.shape, 1)
    q_pass = jnp.where(qi >= L, 1, 0)
    q_pos = qi - L * q_pass
    same = (q_pass == (ki & 1)) & (ki < 2 * L)
    visible = (q_pos < n_mem) | (q_pos >= (ki >> 1))
    fill_ref[...] = jnp.where(same, jnp.where(visible, 0.0, MASK_VALUE), -jnp.inf)

    BOTH, FIRST, SECOND = (0, 1), (0,), (1,)
    join = lambda blocks: jnp.concatenate(blocks, axis=1)

    def store_rows(ref, h, **where):
        _store_rows(ref, h[0] if len(h) == 2 else None, h[-1], **where)

    def project(rows_ref, w_ref, live, cols=slice(None)):
        return _project(rows_ref, w_ref, len(live) == 2, cols)[-len(live):]

    def segment(i, start=0, size=seg):
        return pl.ds(pl.multiple_of(i * seg + start, size), size)

    def segments_in(i, live):
        for r in range(0, seg, ROWS):
            x = [x2_ref[pl.ds(r, ROWS), :] if p else x_vm[segment(i, r, ROWS), :].astype(F32)
                 for p in live]
            for p, xp in zip(live, x):
                ra_ref[p, pl.ds(r, ROWS), :] = xp
            store_rows(h_ref, [_split(_layernorm(xp), n) for xp in x],
                       rows=pl.ds(n_mem + r, ROWS))

    def memories_in(live):
        store_rows(h_ref, [_split(mem_ref[p], n) for p in live], rows=pl.ds(0, n_mem))

    def interleave(a, b):
        words = pltpu.pack_elementwise([a, b], packed_dtype=BF16)
        pad = jnp.zeros((LANES // 2 - L, LANES), words.dtype)
        return pltpu.bitcast(jnp.concatenate([words, pad], axis=0), BF16)

    def heads_of(w, cols, live):
        y = project(h_ref, w, live, cols)
        heads = zip(*([h for blk in yp for h in _split(blk, bw // LANES)] for yp in y))
        return [jnp.concatenate(h, axis=0) if w is wq else interleave(h[0], h[-1])
                for h in heads]

    def softmax(q, k):
        out = []
        for qh, kh in zip(q, k):
            s = jax.lax.dot_general(qh, kh, (((1,), (1,)), ((), ())),
                                    preferred_element_type=F32)
            fill = fill_ref[pl.ds(0, s.shape[0]), :]
            s = jnp.where(fill == 0.0, s * scale, fill)
            p = jnp.exp(s - jnp.max(s, axis=-1, keepdims=True))
            out.append(p * _reciprocal(jnp.sum(p, axis=-1, keepdims=True)))
        return out

    def mix(cols, p, v):
        o = [jax.lax.dot_general(ph, vh, (((1,), (0,)), ((), ())), preferred_element_type=F32)
             for ph, vh in zip(p, v)]
        per = GROUP // n
        o = [join(o[i * per:(i + 1) * per]) for i in range(n)]
        store_rows(o_ref, [[a[r:r + L] for a in o] for r in range(0, o[0].shape[0], L)],
                   cols=cols)

    def chunk(c):
        return pl.ds(c * bw if isinstance(c, int) else pl.multiple_of(c * bw, bw), bw)

    def attention_out(c, live):
        for p, y in zip(live, project(o_ref, wo, live, chunk(c))):
            y, cols = join(y), pl.ds(c * gw, gw)
            mem_ref[p, :, cols] = y[:n_mem]
            rn_ref[p, :, cols] = ra_ref[p, :, cols] + y[n_mem:]

    def hand_over(live):
        for r in range(0, seg, ROWS):
            x = [rn_ref[p, pl.ds(r, ROWS), :] for p in live]
            for p, xp in zip(live, x):
                rb_ref[p, pl.ds(r, ROWS), :] = xp
            store_rows(xb_ref, [_split(_layernorm(xp), n) for xp in x], rows=pl.ds(r, ROWS))

    def gate(cols, g, u, live):
        h = [[_sigmoid(a) * b for a, b in zip(gp, up)] for gp, up in zip(g, u)]
        zero = [jnp.zeros_like(a) for a in h[0]]
        _store_rows(hb_ref, h[0] if 0 in live else zero, h[-1] if 1 in live else zero, cols=cols)

    def glu_out(c, done):
        y1, y2 = project(hb_ref, wd, BOTH, chunk(c))
        cols = pl.ds(c * gw, gw)
        x2_ref[:, cols] = rb_ref[0, :, cols] + join(y1)
        out_vm[segment(done), cols] = (rb_ref[1, :, cols] + join(y2)).astype(out_vm.dtype)

    def each_d(fn, *args):
        for c in range(D // gw):
            fn(c, *args)

    def attention_loop(i, live):
        segments_in(i, live)
        memories_in(live)

        def body(g, carry):
            c0, c1 = chunk(2 * g), chunk(2 * g + 1)
            q0, k0, q1 = heads_of(wq, c0, live), heads_of(wk, c0, live), heads_of(wq, c1, live)
            p0, k1, v0 = softmax(q0, k0), heads_of(wk, c1, live), heads_of(wv, c0, live)
            p1, v1 = softmax(q1, k1), heads_of(wv, c1, live)
            mix(c0, p0, v0)
            mix(c1, p1, v1)
            return carry
        jax.lax.fori_loop(0, n_a // 2, body, 0)

    def glu_loop(live):
        hand_over(live)

        def body(c, carry):
            gate(chunk(c), project(xb_ref, wg, live, chunk(c)),
                 project(xb_ref, wu, live, chunk(c)), live)
            return carry
        jax.lax.fori_loop(0, n_b, body, 0)

    def out_copy(i):
        return pltpu.make_async_copy(out_vm.at[segment(i)], out_hbm.at[segment(i)], out_sem)

    head = pl.ds(0, 4 * seg)
    tail = pl.ds(4 * seg, S - 4 * seg)
    x_head = pltpu.make_async_copy(x_hbm.at[head], x_vm.at[head], x_sem.at[0])
    x_tail = pltpu.make_async_copy(x_hbm.at[tail], x_vm.at[tail], x_sem.at[1])

    def fill(tall_stage, tall_sems, wide_stage, wide_sems):
        tall = Stream([tall_job(wo_hbm, wo)], tall_stage, tall_sems)
        down = Stream([tall_job(wd_hbm, wd)], tall_stage, tall_sems)
        wide = Stream([wide_job(s, d, 1, lambda staged, i: staged[i])
                       for s, d in ((wg_hbm, wg), (wu_hbm, wu))], wide_stage, wide_sems)

        def refill(stream, slots):
            return lambda k: stream.start(k * stream.slots // slots,
                                          (k + 1) * stream.slots // slots)

        def load_qkv(stage, sems):
            qkv_stream = Stream([wide_job(s, d, n_heads, load_heads) for s, d in
                                 ((wq_hbm, wq), (wk_hbm, wk), (wv_hbm, wv))], stage, sems)
            qkv_stream.start()
            x_head.start()
            for m in range(3):
                qkv_stream.drain(m, refill(tall, qkv_stream.slots))

        pl.run_scoped(load_qkv, pltpu.VMEM((QKV_SLOTS, n, kr * n_heads, LANES), BF16),
                      pltpu.SemaphoreType.DMA((QKV_SLOTS,)))
        mem_ref[0] = mem_ref[1] = mem0_ref[...].astype(F32)
        rn_ref[1] = rb_ref[1] = jnp.zeros((seg, D), F32)
        x_head.wait()

        def step(i, carry):
            attention_loop(i, FIRST)
            pl.when(i == 0)(lambda: tall.drain(0, refill(wide, tall.slots)))

            @pl.when(i == 1)
            def _():
                wide.drain(0)
                wide.drain(1, refill(down, wide.slots))

            @pl.when(i == 2)
            def _():
                down.drain(0, lambda k: x_tail.start() if k == 0 else None)
                each_d(glu_out, 0)

            pl.when(i > 0)(lambda: glu_loop(FIRST))
            each_d(attention_out, FIRST)
            return carry

        jax.lax.fori_loop(0, 3, step, 0)

    pl.run_scoped(fill, pltpu.VMEM((TALL_SLOTS, gw, D), BF16),
                  pltpu.SemaphoreType.DMA((TALL_SLOTS,)),
                  pltpu.VMEM((WIDE_SLOTS, n, kr, F), BF16),
                  pltpu.SemaphoreType.DMA((WIDE_SLOTS,)))

    def step(i, carry):
        pl.when(i == 4)(x_tail.wait)
        pl.when(i > 5)(lambda: out_copy(i - 6).start())
        val = {what: [] for what in ORDER}
        for what in ORDER:
            c = len(val[what])
            val[what].append({
                'x': lambda: segments_in(jnp.minimum(i, n_seg - 1), BOTH),
                'm': lambda: memories_in(BOTH),
                'q': lambda: heads_of(wq, chunk(c), BOTH),
                'k': lambda: heads_of(wk, chunk(c), BOTH),
                'v': lambda: heads_of(wv, chunk(c), BOTH),
                'S': lambda: softmax(val['q'][c], val['k'][c]),
                'P': lambda: mix(chunk(c), val['S'][c], val['v'][c]),
                'W': lambda: attention_out(c, BOTH),
                'h': lambda: hand_over(BOTH),
                'g': lambda: project(xb_ref, wg, BOTH, chunk(c)),
                'u': lambda: project(xb_ref, wu, BOTH, chunk(c)),
                'G': lambda: gate(chunk(c), val['g'][c], val['u'][c], BOTH),
                'D': lambda: glu_out(c, jnp.maximum(i - 5, 0)),
            }[what]())
        assert [len(val[w]) for w in 'PGWDxmh'] == [n_a, n_b, D // gw, D // gw, 1, 1, 1]
        return carry

    jax.lax.fori_loop(3, n_seg + 1, step, 0)

    def drain_step(i, carry):
        out_copy(i - 6).start()
        pl.when(i < n_seg + 3)(lambda: attention_loop(i, SECOND))
        each_d(glu_out, i - 5)
        pl.when(i < n_seg + 4)(lambda: glu_loop(SECOND))
        pl.when(i < n_seg + 3)(lambda: each_d(attention_out, SECOND))
        return carry

    jax.lax.fori_loop(n_seg + 1, n_seg + 5, drain_step, 0)
    out_copy(n_seg - 1).start()
    pltpu.make_async_copy(out_vm, out_hbm, out_sem).wait()


@functools.partial(jax.jit, static_argnames=("A_seg_len",))
def pallas_interleave_layers__memory_aug_recurrent_mem_tr__glu_gated_glu__prompt_kernel(
    A_x: jax.Array,
    A_mem0: jax.Array,
    A_Wq: jax.Array,
    A_Wk: jax.Array,
    A_Wv: jax.Array,
    A_Wo: jax.Array,
    A_seg_len: int,
    B_x: jax.Array,
    B_w_gate: jax.Array,
    B_w_up: jax.Array,
    B_w_down: jax.Array,
):
    del B_x
    B, S, D = A_x.shape
    _, H, Dh = A_Wq.shape
    M = A_mem0.shape[1]
    F = B_w_gate.shape[1]
    seg = int(A_seg_len)
    assert B == 1 and Dh == LANES and S % seg == 0 and S // seg >= 8
    n = len(OFFSETS)
    R = (3 * n * n + n) // 2
    L = M + seg

    def packed(k, cols):
        return pltpu.VMEM((R, k // n // 2, cols // n), U32)

    hbm = pl.BlockSpec(memory_space=pl.ANY)
    out = pl.pallas_call(
        functools.partial(_kernel, seg=seg, n_mem=M, n_heads=H),
        out_shape=jax.ShapeDtypeStruct((S, D), A_x.dtype),
        in_specs=[hbm, pl.BlockSpec(memory_space=pltpu.VMEM)] + [hbm] * 7,
        out_specs=hbm,
        scratch_shapes=[
            pltpu.VMEM((S, D), A_x.dtype),
            pltpu.VMEM((S, D), A_x.dtype),
            packed(D, H * Dh),
            packed(D, H * Dh),
            packed(D, H * Dh),
            packed(H * Dh, D),
            packed(D, F),
            packed(D, F),
            packed(F, D),
            pltpu.VMEM((R, L, D // n), F32),
            pltpu.VMEM((R, L, H * Dh // n), F32),
            pltpu.VMEM((R, seg, D // n), B_DTYPE),
            pltpu.VMEM((R, seg, F // n), B_DTYPE),
            pltpu.VMEM((2, M, D), F32),
            pltpu.VMEM((2, seg, D), F32),
            pltpu.VMEM((2, seg, D), F32),
            pltpu.VMEM((2, seg, D), F32),
            pltpu.VMEM((seg, D), F32),
            pltpu.VMEM((2 * L, LANES), F32),
            pltpu.SemaphoreType.DMA((2,)),
            pltpu.SemaphoreType.DMA(()),
        ],
        compiler_params=pltpu.CompilerParams(vmem_limit_bytes=124 * 2**20, flags=FLAGS),
    )(
        A_x.reshape(S, D),
        A_mem0.reshape(M, D),
        A_Wq.reshape(n, D // n * H, Dh),
        A_Wk.reshape(n, D // n * H, Dh),
        A_Wv.reshape(n, D // n * H, Dh),
        A_Wo.reshape(H * Dh, D),
        B_w_gate.reshape(n, D // n, F),
        B_w_up.reshape(n, D // n, F),
        B_w_down,
    )
    return out.reshape(B, S, D)
```

```python
import functools

import jax
import jax.numpy as jnp
import jax.experimental.pallas as pl
import jax.experimental.pallas.tpu as pltpu

F32 = jnp.float32
BF16 = jnp.bfloat16
WORD = jnp.uint32
LANES = 128
LN_EPS = 1e-5
MASK_VALUE = -1000000000.0

OFFSETS = (-1.375, -0.375, 0.375, 1.375)
GROUP = 4
QKV_SLOTS, TALL_SLOTS, WIDE_SLOTS = 3, 6, 7
ROWS = 16
B_DTYPE = F32
FLAGS = None
ORDER = 'mxD' + 'qkvS' + 'qPkvS' * 7 + 'DPh' + 'guG' * 7 + 'WW'
STAGE_ROWS = 128
LONE_ATTENTION = 'mxqkvS' + 'qPkvS' * 6 + 'qkPSvP'


def _layernorm(x):
    m = jnp.mean(x, axis=-1, keepdims=True)
    c = x - m
    v = jnp.mean(c * c, axis=-1, keepdims=True)
    return c * jax.lax.rsqrt(v + LN_EPS)


def _sigmoid(x):
    return 0.5 * jnp.tanh(0.5 * x) + 0.5


def _reciprocal(x):
    r = pl.reciprocal(x, approx=True)
    return r * (2.0 - x * r)


def _split(x, n):
    w = x.shape[1] // n
    return [x[:, i * w:(i + 1) * w] for i in range(n)]


def _pairs(n):
    return [(i, j) for j in range(n) for i in range(j)]


def _row_operands(h1, h2):
    t, n = OFFSETS, len(OFFSETS)
    if h1 is None:
        ops = [None] * n + list(h2)
        for i, j in _pairs(n):
            g2 = h2[i] + h2[j]
            ops += [None, g2, g2]
        return ops
    b = [h2[i] - t[i] * h1[i] for i in range(n)]
    ops = list(h1) + b
    for i, j in _pairs(n):
        s, d = b[i] + b[j], t[j] - t[i]
        ops += [s, s + d * h1[j], s - d * h1[i]]
    return ops


def _weight_operands(w):
    n = len(OFFSETS)
    add = lambda xs: functools.reduce(lambda a, b: a + b, xs)
    sums = []
    for half in range(2):
        f = [[pltpu.unpack_elementwise(blk, index=half, packed_dtype=BF16, unpacked_dtype=F32)
              for blk in row] for row in w]
        sums.append([add(f[i]) for i in range(n)]
                    + [f[i][i] - add([f[j][i] for j in range(n) if j != i]) for i in range(n)]
                    + [f[i][j] + f[j][i] for i, j in _pairs(n)])
    sums = [pltpu.pack_elementwise(list(s), packed_dtype=BF16) for s in zip(*sums)]
    ops = sums[:2 * n]
    for s, (i, j) in zip(sums[2 * n:], _pairs(n)):
        ops += [s, w[j][i], w[i][j]]
    return ops


def _paired_matmul(product, both):
    t, n = OFFSETS, len(OFFSETS)
    y1, y2 = [None] * n, [None] * n
    acc = lambda a, b: b if a is None else a + b
    todo = [n - 1] * n
    for k, (i, j) in enumerate(_pairs(n)):
        ti, tj = product(2 * n + 3 * k + 1), product(2 * n + 3 * k + 2)
        y2[i], y2[j] = acc(y2[i], ti), acc(y2[j], tj)
        if both:
            u = (ti + tj - product(2 * n + 3 * k)) * (1.0 / (t[j] - t[i]))
            y1[i], y1[j] = acc(y1[i], u), (-u if y1[j] is None else y1[j] - u)
        for m in (i, j):
            todo[m] -= 1
            if todo[m] == 0:
                y2[m] = y2[m] + product(n + m)
                if both:
                    y1[m] = y1[m] + product(m)
                    y2[m] = y2[m] + t[m] * y1[m]
    return (y1 if both else None), y2


def _project(rows_ref, w_ref, both, cols=slice(None)):
    def product(r):
        w = pltpu.bitcast(w_ref[r, :, cols], BF16)
        return jax.lax.dot_general(rows_ref[r], w, (((1,), (0,)), ((), ())),
                                   preferred_element_type=F32)
    return _paired_matmul(product, both)


def _store_rows(ref, h1, h2, rows=slice(None), cols=slice(None)):
    for r, op in enumerate(_row_operands(h1, h2)):
        if op is not None:
            ref[r, rows, cols] = op.astype(ref.dtype)


def _kernel(x_hbm, mem0_hbm, wq_hbm, wk_hbm, wv_hbm, wo_hbm, wg_hbm, wu_hbm, wd_hbm,
            out_hbm,
            x_vm, out_vm, wq, wk, wv, wo, wg, wu, wd,
            h_ref, o_ref, xb_ref, hb_ref, mem_ref, ra_ref, rn_ref, rb_ref, x2_ref, fill_ref,
            mem0_vm, qkv_stage, tall_stage, wide_stage,
            qkv_sems, tall_sems, wide_sems, x_sem, out_sem, *, seg, n_mem, n_heads):
    S, D = x_vm.shape
    F = wg_hbm.shape[2]
    n_seg = S // seg
    L = n_mem + seg
    n = len(OFFSETS)
    gw = GROUP * LANES
    bw = gw // n
    n_a, n_b = n_heads // GROUP, F // gw
    scale = LANES ** -0.5

    class Stream:
        def __init__(self, jobs, stage, sems):
            self.jobs, self.stage, self.sems = jobs, stage, sems
            self.slots = stage.shape[0]

        def copy(self, m, c, slot):
            return pltpu.make_async_copy(self.jobs[m][1](c), self.stage.at[slot],
                                         self.sems.at[slot])

        def start(self, first=0, last=None):
            for c in range(first, self.slots if last is None else last):
                self.copy(0, c, c).start()

        def drain(self, m, refill=None):
            count, _, consume = self.jobs[m]
            first = sum(j[0] for j in self.jobs[:m])

            def body(c, carry):
                slot = (first + c) % self.slots
                self.copy(m, c, slot).wait()
                consume(c, self.stage.at[slot])
                nxt = c + self.slots
                if self.slots < count:
                    pl.when(nxt < count)(lambda: self.copy(m, nxt, slot).start())
                if m + 1 < len(self.jobs):
                    pl.when(nxt >= count)(lambda: self.copy(m + 1, nxt - count, slot).start())
                elif refill:
                    for k in range(self.slots):
                        pl.when(nxt == count + k)(functools.partial(refill, k))
                return carry

            jax.lax.fori_loop(0, count, body, 0)

    kr = STAGE_ROWS // n

    def wide_job(src, dst, per_row, load):
        def consume(c, staged):
            blocks = [pltpu.bitcast(load(staged, i), WORD) for i in range(n)]
            rows = pl.ds(pl.multiple_of(c * (kr // 2), kr // 2), kr // 2)
            for g in range(blocks[0].shape[1] // gw):
                w = [_split(blk[:, g * gw:(g + 1) * gw], n) for blk in blocks]
                for r, op in enumerate(_weight_operands(w)):
                    dst[r, rows, pl.ds(g * bw, bw)] = op
        step = kr * per_row
        return (D // STAGE_ROWS,
                lambda c: src.at[:, pl.ds(pl.multiple_of(c * step, step), step), :],
                consume)

    def tall_job(src, dst):
        def consume(c, staged):
            rows = pl.ds(pl.multiple_of(c * (bw // 2), bw // 2), bw // 2)
            for g in range(D // gw):
                w = [_split(pltpu.bitcast(staged[pl.ds(i * bw, bw), pl.ds(g * gw, gw)], WORD), n)
                     for i in range(n)]
                for r, op in enumerate(_weight_operands(w)):
                    dst[r, rows, pl.ds(g * bw, bw)] = op
        return (src.shape[0] // gw,
                lambda c: src.at[pl.ds(pl.multiple_of(c * gw, gw), gw), :],
                consume)

    def load_heads(staged, i):
        return staged[i].reshape(kr, n_heads, LANES).reshape(kr, n_heads * LANES)

    qi = jax.lax.broadcasted_iota(jnp.int32, fill_ref.shape, 0)
    ki = jax.lax.broadcasted_iota(jnp.int32, fill_ref.shape, 1)
    q_pass = jnp.where(qi >= L, 1, 0)
    q_pos = qi - L * q_pass
    same = (q_pass == (ki & 1)) & (ki < 2 * L)
    visible = (q_pos < n_mem) | (q_pos >= (ki >> 1))
    fill_ref[...] = jnp.where(same, jnp.where(visible, 0.0, MASK_VALUE), -jnp.inf)

    BOTH = (0, 1)
    join = lambda blocks: jnp.concatenate(blocks, axis=1)

    def store_rows(ref, h, **where):
        _store_rows(ref, h[0] if len(h) == 2 else None, h[-1], **where)

    def project(rows_ref, w_ref, live, cols=slice(None)):
        return _project(rows_ref, w_ref, len(live) == 2, cols)[-len(live):]

    def segment(i, start=0, size=seg):
        return pl.ds(pl.multiple_of(i * seg + start, size), size)

    def segments_in(i, live):
        for r in range(0, seg, ROWS):
            x = [x_vm[segment(jnp.minimum(i, n_seg - 1), r, ROWS), :].astype(F32),
                 x2_ref[pl.ds(r, ROWS), :]]
            if len(live) == 1:
                x = [jnp.where(live[0] == 0, *x)]
            for p, xp in zip(live, x):
                ra_ref[p, pl.ds(r, ROWS), :] = xp
            store_rows(h_ref, [_split(_layernorm(xp), n) for xp in x],
                       rows=pl.ds(n_mem + r, ROWS))

    def memories_in(live):
        store_rows(h_ref, [_split(mem_ref[p], n) for p in live], rows=pl.ds(0, n_mem))

    def interleave(a, b):
        words = pltpu.pack_elementwise([a, b], packed_dtype=BF16)
        pad = jnp.zeros((LANES // 2 - L, LANES), words.dtype)
        return pltpu.bitcast(jnp.concatenate([words, pad], axis=0), BF16)

    def heads_of(w, cols, live):
        y = project(h_ref, w, live, cols)
        heads = zip(*([h for blk in yp for h in _split(blk, bw // LANES)] for yp in y))
        return [jnp.concatenate(h, axis=0) if w is wq else interleave(h[0], h[-1])
                for h in heads]

    def softmax(q, k):
        out = []
        for qh, kh in zip(q, k):
            s = jax.lax.dot_general(qh, kh, (((1,), (1,)), ((), ())),
                                    preferred_element_type=F32)
            fill = fill_ref[pl.ds(0, s.shape[0]), :]
            s = jnp.where(fill == 0.0, s * scale, fill)
            p = jnp.exp(s - jnp.max(s, axis=-1, keepdims=True))
            out.append(p * _reciprocal(jnp.sum(p, axis=-1, keepdims=True)))
        return out

    def mix(cols, p, v):
        o = [jax.lax.dot_general(ph, vh, (((1,), (0,)), ((), ())), preferred_element_type=F32)
             for ph, vh in zip(p, v)]
        per = GROUP // n
        o = [join(o[i * per:(i + 1) * per]) for i in range(n)]
        store_rows(o_ref, [[a[r:r + L] for a in o] for r in range(0, o[0].shape[0], L)],
                   cols=cols)

    def chunk(c):
        return pl.ds(c * bw, bw)

    def attention_out(c, live):
        for p, y in zip(live, project(o_ref, wo, live, chunk(c))):
            y, cols = join(y), pl.ds(c * gw, gw)
            mem_ref[p, :, cols] = y[:n_mem]
            rn_ref[p, :, cols] = ra_ref[p, :, cols] + y[n_mem:]

    def hand_over(live):
        for r in range(0, seg, ROWS):
            x = [rn_ref[p, pl.ds(r, ROWS), :] for p in live]
            for p, xp in zip(live, x):
                rb_ref[p, pl.ds(r, ROWS), :] = xp
            store_rows(xb_ref, [_split(_layernorm(xp), n) for xp in x], rows=pl.ds(r, ROWS))

    def gate(cols, g, u, live):
        h = [[_sigmoid(a) * b for a, b in zip(gp, up)] for gp, up in zip(g, u)]
        if len(live) == 1:
            h = [[jnp.where(live[0] == p, a, 0.0) for a in h[0]] for p in BOTH]
        store_rows(hb_ref, h, cols=cols)

    def glu_out(c, i, live):
        cols = pl.ds(c * gw, gw)
        for p, y in zip(live, project(hb_ref, wd, live, chunk(c))):
            y = rb_ref[p, :, cols] + join(y)
            if p == 0:
                x2_ref[:, cols] = y
            else:
                out_vm[segment(jnp.maximum(i - 5, 0)), cols] = y.astype(out_vm.dtype)

    def run(order, i, live):
        val = {what: [] for what in order}
        for what in order:
            c = len(val[what])
            val[what].append({
                'x': lambda: segments_in(i, live),
                'm': lambda: memories_in(live),
                'q': lambda: heads_of(wq, chunk(c), live),
                'k': lambda: heads_of(wk, chunk(c), live),
                'v': lambda: heads_of(wv, chunk(c), live),
                'S': lambda: softmax(val['q'][c], val['k'][c]),
                'P': lambda: mix(chunk(c), val['S'][c], val['v'][c]),
                'W': lambda: attention_out(c, live),
                'h': lambda: hand_over(live),
                'g': lambda: project(xb_ref, wg, live, chunk(c)),
                'u': lambda: project(xb_ref, wu, live, chunk(c)),
                'G': lambda: gate(chunk(c), val['g'][c], val['u'][c], live),
                'D': lambda: glu_out(c, i, live),
            }[what]())

    def out_copy(i):
        return pltpu.make_async_copy(out_vm.at[segment(i)], out_hbm.at[segment(i)], out_sem)

    n_d = D // gw
    head = pl.ds(0, 4 * seg)
    tail = pl.ds(4 * seg, S - 4 * seg)
    x_head = pltpu.make_async_copy(x_hbm.at[head], x_vm.at[head], x_sem.at[0])
    x_tail = pltpu.make_async_copy(x_hbm.at[tail], x_vm.at[tail], x_sem.at[1])
    mem_copy = pltpu.make_async_copy(mem0_hbm, mem0_vm, x_sem.at[2])

    qkv = Stream([wide_job(s, d, n_heads, load_heads) for s, d in
                  ((wq_hbm, wq), (wk_hbm, wk), (wv_hbm, wv))], qkv_stage, qkv_sems)
    proj = Stream([tall_job(wo_hbm, wo)], tall_stage, tall_sems)
    wide = Stream([wide_job(s, d, 1, lambda staged, i: staged[i])
                   for s, d in ((wg_hbm, wg), (wu_hbm, wu))], wide_stage, wide_sems)
    down = Stream([tall_job(wd_hbm, wd)], tall_stage, tall_sems)

    def refill(stream, calls):
        return lambda k: stream.start(k * stream.slots // calls, (k + 1) * stream.slots // calls)

    qkv.start()
    x_head.start()
    mem_copy.start()
    for m in range(3):
        qkv.drain(m, refill(proj, qkv.slots))
    x_head.wait()
    mem_copy.wait()
    mem_ref[0] = mem_ref[1] = mem0_vm[...].astype(F32)
    x2_ref[...] = rn_ref[1] = rb_ref[1] = jnp.zeros((seg, D), F32)

    def full_step(i, carry):
        pl.when(i == 4)(x_tail.wait)
        pl.when(i > 5)(lambda: out_copy(i - 6).start())
        run(ORDER, i, BOTH)
        return carry

    def ragged_step(j, carry):
        lone = (jnp.where(j < 3, 0, 1),)
        i = jnp.where(j < 3, j, j - 3 + n_seg)
        phase = lambda cond, order, live: pl.when(cond)(lambda: run(order, i, live))
        pl.when(j >= 3)(lambda: out_copy(i - 6).start())
        phase(j < 6, LONE_ATTENTION, lone)
        pl.when(j == 0)(lambda: proj.drain(0, refill(wide, proj.slots)))

        @pl.when(j == 1)
        def _():
            wide.drain(0)
            wide.drain(1, refill(down, wide.slots))

        pl.when(j == 2)(lambda: down.drain(0, lambda k: x_tail.start() if k == 0 else None))
        phase((j >= 2) & (j < 5), 'D' * n_d, BOTH)
        phase(j >= 5, 'D' * n_d, (1,))
        phase(j == 3, 'h' + 'guG' * n_b, BOTH)
        phase((j > 0) & (j != 3) & (j < 7), 'h' + 'guG' * n_b, lone)
        phase(j < 6, 'W' * n_d, lone)

        @pl.when(j == 2)
        def _():
            jax.lax.fori_loop(3, n_seg, full_step, 0)
        return carry

    for order, letters in ((ORDER, 'PGWDxmh'), (LONE_ATTENTION, 'Pxm')):
        counts = dict(P=n_a, G=n_b, W=n_d, D=n_d, x=1, m=1, h=1)
        assert all(order.count(c) == counts[c] for c in letters)
    jax.lax.fori_loop(0, 8, ragged_step, 0)
    out_copy(n_seg - 1).start()
    pltpu.make_async_copy(out_vm, out_hbm, out_sem).wait()


@functools.partial(jax.jit, static_argnames=("A_seg_len",))
def pallas_interleave_layers__memory_aug_recurrent_mem_tr__glu_gated_glu__prompt_kernel(
    A_x: jax.Array,
    A_mem0: jax.Array,
    A_Wq: jax.Array,
    A_Wk: jax.Array,
    A_Wv: jax.Array,
    A_Wo: jax.Array,
    A_seg_len: int,
    B_x: jax.Array,
    B_w_gate: jax.Array,
    B_w_up: jax.Array,
    B_w_down: jax.Array,
):
    del B_x
    B, S, D = A_x.shape
    _, H, Dh = A_Wq.shape
    M = A_mem0.shape[1]
    F = B_w_gate.shape[1]
    seg = int(A_seg_len)
    assert B == 1 and Dh == LANES and S % seg == 0 and S // seg >= 8
    n = len(OFFSETS)
    R = (3 * n * n + n) // 2
    L = M + seg

    def packed(k, cols):
        return pltpu.VMEM((R, k // n // 2, cols // n), WORD)

    hbm = pl.BlockSpec(memory_space=pl.ANY)
    out = pl.pallas_call(
        functools.partial(_kernel, seg=seg, n_mem=M, n_heads=H),
        out_shape=jax.ShapeDtypeStruct((S, D), A_x.dtype),
        in_specs=[hbm] * 9,
        out_specs=hbm,
        scratch_shapes=[
            pltpu.VMEM((S, D), A_x.dtype),
            pltpu.VMEM((S, D), A_x.dtype),
            packed(D, H * Dh),
            packed(D, H * Dh),
            packed(D, H * Dh),
            packed(H * Dh, D),
            packed(D, F),
            packed(D, F),
            packed(F, D),
            pltpu.VMEM((R, L, D // n), F32),
            pltpu.VMEM((R, L, H * Dh // n), F32),
            pltpu.VMEM((R, seg, D // n), B_DTYPE),
            pltpu.VMEM((R, seg, F // n), B_DTYPE),
            pltpu.VMEM((2, M, D), F32),
            pltpu.VMEM((2, seg, D), F32),
            pltpu.VMEM((2, seg, D), F32),
            pltpu.VMEM((2, seg, D), F32),
            pltpu.VMEM((seg, D), F32),
            pltpu.VMEM((2 * L, LANES), F32),
            pltpu.VMEM((M, D), A_mem0.dtype),
            pltpu.VMEM((QKV_SLOTS, n, STAGE_ROWS // n * H, Dh), BF16),
            pltpu.VMEM((TALL_SLOTS, GROUP * LANES, D), BF16),
            pltpu.VMEM((WIDE_SLOTS, n, STAGE_ROWS // n, F), BF16),
            pltpu.SemaphoreType.DMA((QKV_SLOTS,)),
            pltpu.SemaphoreType.DMA((TALL_SLOTS,)),
            pltpu.SemaphoreType.DMA((WIDE_SLOTS,)),
            pltpu.SemaphoreType.DMA((3,)),
            pltpu.SemaphoreType.DMA(()),
        ],
        compiler_params=pltpu.CompilerParams(vmem_limit_bytes=124 * 2**20, flags=FLAGS),
    )(
        A_x.reshape(S, D),
        A_mem0.reshape(M, D),
        A_Wq.reshape(n, D // n * H, Dh),
        A_Wk.reshape(n, D // n * H, Dh),
        A_Wv.reshape(n, D // n * H, Dh),
        A_Wo.reshape(H * Dh, D),
        B_w_gate.reshape(n, D // n, F),
        B_w_up.reshape(n, D // n, F),
        B_w_down,
    )
    return out.reshape(B, S, D)
```

```python
import functools

import jax
import jax.numpy as jnp
import jax.experimental.pallas as pl
import jax.experimental.pallas.tpu as pltpu

F32 = jnp.float32
BF16 = jnp.bfloat16
WORD = jnp.uint32
LANES = 128
LN_EPS = 1e-5
MASK_VALUE = -1000000000.0

OFFSETS = (-1.5, -0.5, 0.5, 1.5)
GROUP = 4
QKV_SLOTS, TALL_SLOTS, WIDE_SLOTS = 3, 6, 7
ROWS = 16
B_DTYPE = F32
FLAGS = None
ORDER = None
STAGE_ROWS = 128


def _layernorm(x):
    m = jnp.mean(x, axis=-1, keepdims=True)
    c = x - m
    v = jnp.mean(c * c, axis=-1, keepdims=True)
    return c * jax.lax.rsqrt(v + LN_EPS)


def _sigmoid(x):
    return 0.5 * jnp.tanh(0.5 * x) + 0.5


def _reciprocal(x):
    r = pl.reciprocal(x, approx=True)
    return r * (2.0 - x * r)


def _times(c, x):
    return x if c == 1 else c * x


def _split(x, n):
    w = x.shape[1] // n
    return [x[:, i * w:(i + 1) * w] for i in range(n)]


def _pairs(n):
    return [(i, j) for j in range(n) for i in range(j)]


def _row_operands(h1, h2):
    t, n = OFFSETS, len(OFFSETS)
    if h1 is None:
        ops = [None] * n + list(h2)
        for i, j in _pairs(n):
            g2 = h2[i] + h2[j]
            ops += [None, g2, g2]
        return ops
    b = [h2[i] - t[i] * h1[i] for i in range(n)]
    ops = list(h1) + b
    for i, j in _pairs(n):
        s, d = b[i] + b[j], t[j] - t[i]
        ops += [s, s + _times(d, h1[j]), s - _times(d, h1[i])]
    return ops


def _pack_rows(even, odd):
    bits = lambda x: jax.lax.bitcast_convert_type(x.astype(BF16).astype(F32), WORD)
    return (bits(even) >> 16) | bits(odd)


def _weight_operands(w):
    n = len(OFFSETS)
    add = lambda xs: functools.reduce(lambda a, b: a + b, xs)
    sums = []
    for rows in (lambda x: x << 16, lambda x: x & WORD(0xFFFF0000)):
        f = [[jax.lax.bitcast_convert_type(rows(blk), F32) for blk in row] for row in w]
        sums.append([add(f[i]) for i in range(n)]
                    + [f[i][i] - add([f[j][i] for j in range(n) if j != i]) for i in range(n)]
                    + [f[i][j] + f[j][i] for i, j in _pairs(n)])
    sums = [_pack_rows(*s) for s in zip(*sums)]
    ops = sums[:2 * n]
    for s, (i, j) in zip(sums[2 * n:], _pairs(n)):
        ops += [s, w[j][i], w[i][j]]
    return ops


def _paired_matmul(product, both):
    t, n = OFFSETS, len(OFFSETS)
    y1, y2 = [None] * n, [None] * n
    acc = lambda a, b: b if a is None else a + b
    todo = [n - 1] * n
    for k, (i, j) in enumerate(_pairs(n)):
        ti, tj = product(2 * n + 3 * k + 1), product(2 * n + 3 * k + 2)
        y2[i], y2[j] = acc(y2[i], ti), acc(y2[j], tj)
        if both:
            u = _times(1.0 / (t[j] - t[i]), ti + tj - product(2 * n + 3 * k))
            y1[i], y1[j] = acc(y1[i], u), (-u if y1[j] is None else y1[j] - u)
        for m in (i, j):
            todo[m] -= 1
            if todo[m] == 0:
                y2[m] = y2[m] + product(n + m)
                if both:
                    y1[m] = y1[m] + product(m)
                    y2[m] = y2[m] + t[m] * y1[m]
    return (y1 if both else None), y2


def _project(rows_ref, w_ref, both, cols=slice(None)):
    def product(r):
        w = pltpu.bitcast(w_ref[r, :, cols], BF16)
        return jax.lax.dot_general(rows_ref[r], w, (((1,), (0,)), ((), ())),
                                   preferred_element_type=F32)
    return _paired_matmul(product, both)


def _store_rows(ref, h1, h2, rows=slice(None), cols=slice(None)):
    for r, op in enumerate(_row_operands(h1, h2)):
        if op is not None:
            ref[r, rows, cols] = op.astype(ref.dtype)


def _kernel(x_hbm, mem0_hbm, wq_hbm, wk_hbm, wv_hbm, wo_hbm, wg_hbm, wu_hbm, wd_hbm,
            out_hbm,
            x_vm, out_vm, wq, wk, wv, wo, wg, wu, wd,
            h_ref, o_ref, xb_ref, hb_ref, mem_ref, ra_ref, rb_ref, x2_ref, fill_ref,
            mem0_vm, qkv_stage, tall_stage, wide_stage,
            qkv_sems, tall_sems, wide_sems, x_sem, out_sem, *, seg, n_mem, n_heads):
    S, D = x_vm.shape
    F = wg_hbm.shape[2]
    n_seg = S // seg
    L = n_mem + seg
    n = len(OFFSETS)
    gw = GROUP * LANES
    bw = gw // n
    n_a, n_b = n_heads // GROUP, F // gw
    scale = LANES ** -0.5

    class Stream:
        def __init__(self, jobs, stage, sems):
            self.jobs, self.stage, self.sems = jobs, stage, sems
            self.slots = stage.shape[0]

        def copy(self, m, c, slot):
            return pltpu.make_async_copy(self.jobs[m][1](c), self.stage.at[slot],
                                         self.sems.at[slot])

        def start(self, first=0, last=None):
            for c in range(first, self.slots if last is None else last):
                self.copy(0, c, c).start()

        def drain(self, m, refill=None):
            count, _, consume = self.jobs[m]
            first = sum(j[0] for j in self.jobs[:m])

            def body(c, carry):
                slot = (first + c) % self.slots
                self.copy(m, c, slot).wait()
                consume(c, self.stage.at[slot])
                nxt = c + self.slots
                if self.slots < count:
                    pl.when(nxt < count)(lambda: self.copy(m, nxt, slot).start())
                if m + 1 < len(self.jobs):
                    pl.when(nxt >= count)(lambda: self.copy(m + 1, nxt - count, slot).start())
                elif refill:
                    for k in range(self.slots):
                        pl.when(nxt == count + k)(functools.partial(refill, k))
                return carry

            jax.lax.fori_loop(0, count, body, 0)

    kr = STAGE_ROWS // n

    def wide_job(src, dst, per_row, load):
        def consume(c, staged):
            blocks = [pltpu.bitcast(load(staged, i), WORD) for i in range(n)]
            rows = pl.ds(pl.multiple_of(c * (kr // 2), kr // 2), kr // 2)
            for g in range(blocks[0].shape[1] // gw):
                w = [_split(blk[:, g * gw:(g + 1) * gw], n) for blk in blocks]
                for r, op in enumerate(_weight_operands(w)):
                    dst[r, rows, pl.ds(g * bw, bw)] = op
        step = kr * per_row
        return (D // STAGE_ROWS,
                lambda c: src.at[:, pl.ds(pl.multiple_of(c * step, step), step), :],
                consume)

    def tall_job(src, dst):
        def consume(c, staged):
            rows = pl.ds(pl.multiple_of(c * (bw // 2), bw // 2), bw // 2)
            for g in range(D // gw):
                w = [_split(pltpu.bitcast(staged[pl.ds(i * bw, bw), pl.ds(g * gw, gw)], WORD), n)
                     for i in range(n)]
                for r, op in enumerate(_weight_operands(w)):
                    dst[r, rows, pl.ds(g * bw, bw)] = op
        return (src.shape[0] // gw,
                lambda c: src.at[pl.ds(pl.multiple_of(c * gw, gw), gw), :],
                consume)

    def load_heads(staged, i):
        return staged[i].reshape(kr, n_heads, LANES).reshape(kr, n_heads * LANES)

    qi = jax.lax.broadcasted_iota(jnp.int32, fill_ref.shape, 0)
    ki = jax.lax.broadcasted_iota(jnp.int32, fill_ref.shape, 1)
    same = ((qi >= L) == (ki >= L)) & (ki < 2 * L)
    visible = (jnp.where(qi >= L, qi - L, qi) < n_mem) | (qi >= ki)
    fill_ref[...] = jnp.where(same, jnp.where(visible, 0.0, MASK_VALUE), -jnp.inf)

    BOTH = (0, 1)
    join = lambda blocks: jnp.concatenate(blocks, axis=1)

    def store_rows(ref, h, **where):
        _store_rows(ref, h[0] if len(h) == 2 else None, h[-1], **where)

    def project(rows_ref, w_ref, live, cols=slice(None)):
        return _project(rows_ref, w_ref, len(live) == 2, cols)[-len(live):]

    def segment(i, start=0, size=seg):
        return pl.ds(pl.multiple_of(i * seg + start, size), size)

    def segments_in(i, live):
        for r in range(0, seg, ROWS):
            x = [x_vm[segment(jnp.minimum(i, n_seg - 1), r, ROWS), :].astype(F32),
                 x2_ref[pl.ds(r, ROWS), :]]
            if len(live) == 1:
                x = [jnp.where(live[0] == 0, *x)]
            for p, xp in zip(live, x):
                ra_ref[p, pl.ds(r, ROWS), :] = xp
            store_rows(h_ref, [_split(_layernorm(xp), n) for xp in x],
                       rows=pl.ds(n_mem + r, ROWS))

    def memories_in(live):
        store_rows(h_ref, [_split(mem_ref[p], n) for p in live], rows=pl.ds(0, n_mem))

    def heads_of(w, cols, live):
        y = project(h_ref, w, live, cols)
        heads = zip(*([h for blk in yp for h in _split(blk, bw // LANES)] for yp in y))
        pad = () if w is wq else (jnp.zeros((LANES - len(live) * L, LANES), F32),)
        return [jnp.concatenate(h + pad, axis=0) for h in heads]

    def softmax(q, k):
        out = []
        for qh, kh in zip(q, k):
            s = jax.lax.dot_general(qh, kh, (((1,), (1,)), ((), ())),
                                    preferred_element_type=F32)
            fill = fill_ref[pl.ds(0, s.shape[0]), :]
            s = jnp.where(fill == 0.0, s * scale, fill)
            p = jnp.exp(s - jnp.max(s, axis=-1, keepdims=True))
            out.append(p * _reciprocal(jnp.sum(p, axis=-1, keepdims=True)))
        return out

    def mix(cols, p, v):
        o = [jax.lax.dot_general(ph, vh, (((1,), (0,)), ((), ())), preferred_element_type=F32)
             for ph, vh in zip(p, v)]
        per = GROUP // n
        o = [join(o[i * per:(i + 1) * per]) for i in range(n)]
        store_rows(o_ref, [[a[r:r + L] for a in o] for r in range(0, o[0].shape[0], L)],
                   cols=cols)

    def chunk(c):
        return pl.ds(c * bw, bw)

    def attention_out(c, i, live):
        for p, y in zip(live, project(o_ref, wo, live, chunk(c))):
            y, cols = join(y), pl.ds(c * gw, gw)
            mem_ref[p, :, cols] = y[:n_mem]
            rb_ref[i & 1, p, :, cols] = ra_ref[p, :, cols] + y[n_mem:]

    def glu_in(i, live):
        for r in range(0, seg, ROWS):
            x = [rb_ref[(i + 1) & 1, p, pl.ds(r, ROWS), :] for p in live]
            store_rows(xb_ref, [_split(_layernorm(xp), n) for xp in x], rows=pl.ds(r, ROWS))

    def gate(cols, g, u, live):
        h = [[_sigmoid(a) * b for a, b in zip(gp, up)] for gp, up in zip(g, u)]
        if len(live) == 1:
            h = [[jnp.where(live[0] == p, a, 0.0) for a in h[0]] for p in BOTH]
        store_rows(hb_ref, h, cols=cols)

    def glu_out(c, i, live):
        cols = pl.ds(c * gw, gw)
        for p, y in zip(live, project(hb_ref, wd, live, chunk(c))):
            y = rb_ref[i & 1, p, :, cols] + join(y)
            if p == 0:
                x2_ref[:, cols] = y
            else:
                out_vm[segment(jnp.maximum(i - 5, 0)), cols] = y.astype(out_vm.dtype)

    def run(order, i, live):
        val = {what: [] for what in order}
        for what in order:
            c = len(val[what])
            val[what].append({
                'x': lambda: segments_in(i, live),
                'm': lambda: memories_in(live),
                'q': lambda: heads_of(wq, chunk(c), live),
                'k': lambda: heads_of(wk, chunk(c), live),
                'v': lambda: heads_of(wv, chunk(c), live),
                'S': lambda: softmax(val['q'][c], val['k'][c]),
                'P': lambda: mix(chunk(c), val['S'][c], val['v'][c]),
                'W': lambda: attention_out(c, i, live),
                'h': lambda: glu_in(i, live),
                'g': lambda: project(xb_ref, wg, live, chunk(c)),
                'u': lambda: project(xb_ref, wu, live, chunk(c)),
                'G': lambda: gate(chunk(c), val['g'][c], val['u'][c], live),
                'D': lambda: glu_out(c, i, live),
            }[what]())

    def out_copy(i):
        return pltpu.make_async_copy(out_vm.at[segment(i)], out_hbm.at[segment(i)], out_sem)

    n_d = D // gw
    head = pl.ds(0, 4 * seg)
    tail = pl.ds(4 * seg, S - 4 * seg)
    x_head = pltpu.make_async_copy(x_hbm.at[head], x_vm.at[head], x_sem.at[0])
    x_tail = pltpu.make_async_copy(x_hbm.at[tail], x_vm.at[tail], x_sem.at[1])
    mem_copy = pltpu.make_async_copy(mem0_hbm, mem0_vm, x_sem.at[2])

    qkv = Stream([wide_job(s, d, n_heads, load_heads) for s, d in
                  ((wq_hbm, wq), (wk_hbm, wk), (wv_hbm, wv))], qkv_stage, qkv_sems)
    proj = Stream([tall_job(wo_hbm, wo)], tall_stage, tall_sems)
    wide = Stream([wide_job(s, d, 1, lambda staged, i: staged[i])
                   for s, d in ((wg_hbm, wg), (wu_hbm, wu))], wide_stage, wide_sems)
    down = Stream([tall_job(wd_hbm, wd)], tall_stage, tall_sems)

    def refill(stream, calls):
        return lambda k: stream.start(k * stream.slots // calls, (k + 1) * stream.slots // calls)

    qkv.start()
    x_head.start()
    mem_copy.start()
    for m in range(3):
        qkv.drain(m, refill(proj, qkv.slots))
    x_head.wait()
    mem_copy.wait()
    mem_ref[0] = mem_ref[1] = mem0_vm[...].astype(F32)
    x2_ref[...] = rb_ref[0, 1] = rb_ref[1, 1] = jnp.zeros((seg, D), F32)

    attention = 'qkvS' + 'qPkvS' * (n_a - 1)
    glu = 'guG' * n_b

    def full_step(i, carry):
        pl.when(i == 4)(x_tail.wait)
        pl.when(i > 5)(lambda: out_copy(i - 6).start())
        run(ORDER or 'mxD' + attention + 'D' * (n_d - 1) + 'Ph' + glu + 'W' * n_d, i, BOTH)
        return carry

    def ragged_step(j, carry):
        lone = (jnp.where(j < 4, 0, 1),)
        i = jnp.where(j < 4, jnp.minimum(j, 2), j - 4 + n_seg)
        phase = lambda cond, order, live: pl.when(cond)(lambda: run(order, i, live))
        attends = (j != 3) & (j < 7)
        pl.when(j >= 4)(lambda: out_copy(i - 6).start())
        phase(attends, 'mx' + attention[:-5] + 'qkPSvP', lone)
        pl.when(j == 0)(lambda: proj.drain(0, refill(wide, proj.slots)))
        pl.when(j == 1)(lambda: wide.drain(0))

        pl.when(j == 2)(lambda: wide.drain(1, lambda k: down.start() if k == 0 else None))
        pl.when(j == 3)(lambda: down.drain(0, lambda k: x_tail.start() if k == 0 else None))
        phase((j >= 3) & (j < 6), 'D' * n_d, BOTH)
        phase(j >= 6, 'D' * n_d, (1,))
        phase(j == 4, 'h' + glu, BOTH)
        pl.when((j > 1) & (j != 4) & (j < 8))(
            lambda: run('h' + glu, jnp.where(j == 2, 1, i), lone))
        phase((j != 2) & (j < 7), 'W' * n_d, lone)

        @pl.when(j == 3)
        def _():
            jax.lax.fori_loop(3, n_seg, full_step, 0)
        return carry

    jax.lax.fori_loop(0, 9, ragged_step, 0)
    out_copy(n_seg - 1).start()
    pltpu.make_async_copy(out_vm, out_hbm, out_sem).wait()


@functools.partial(jax.jit, static_argnames=("A_seg_len",))
def pallas_interleave_layers__memory_aug_recurrent_mem_tr__glu_gated_glu__prompt_kernel(
    A_x: jax.Array,
    A_mem0: jax.Array,
    A_Wq: jax.Array,
    A_Wk: jax.Array,
    A_Wv: jax.Array,
    A_Wo: jax.Array,
    A_seg_len: int,
    B_x: jax.Array,
    B_w_gate: jax.Array,
    B_w_up: jax.Array,
    B_w_down: jax.Array,
):
    del B_x
    B, S, D = A_x.shape
    _, H, Dh = A_Wq.shape
    M = A_mem0.shape[1]
    F = B_w_gate.shape[1]
    seg = int(A_seg_len)
    assert B == 1 and Dh == LANES and S % seg == 0 and S // seg >= 8
    n = len(OFFSETS)
    R = (3 * n * n + n) // 2
    L = M + seg

    def packed(k, cols):
        return pltpu.VMEM((R, k // n // 2, cols // n), WORD)

    hbm = pl.BlockSpec(memory_space=pl.ANY)
    out = pl.pallas_call(
        functools.partial(_kernel, seg=seg, n_mem=M, n_heads=H),
        out_shape=jax.ShapeDtypeStruct((S, D), A_x.dtype),
        in_specs=[hbm] * 9,
        out_specs=hbm,
        scratch_shapes=[
            pltpu.VMEM((S, D), A_x.dtype),
            pltpu.VMEM((S, D), A_x.dtype),
            packed(D, H * Dh),
            packed(D, H * Dh),
            packed(D, H * Dh),
            packed(H * Dh, D),
            packed(D, F),
            packed(D, F),
            packed(F, D),
            pltpu.VMEM((R, L, D // n), F32),
            pltpu.VMEM((R, L, H * Dh // n), F32),
            pltpu.VMEM((R, seg, D // n), B_DTYPE),
            pltpu.VMEM((R, seg, F // n), B_DTYPE),
            pltpu.VMEM((2, M, D), F32),
            pltpu.VMEM((2, seg, D), F32),
            pltpu.VMEM((2, 2, seg, D), F32),
            pltpu.VMEM((seg, D), F32),
            pltpu.VMEM((2 * L, LANES), F32),
            pltpu.VMEM((M, D), A_mem0.dtype),
            pltpu.VMEM((QKV_SLOTS, n, STAGE_ROWS // n * H, Dh), BF16),
            pltpu.VMEM((TALL_SLOTS, GROUP * LANES, D), BF16),
            pltpu.VMEM((WIDE_SLOTS, n, STAGE_ROWS // n, F), BF16),
            pltpu.SemaphoreType.DMA((QKV_SLOTS,)),
            pltpu.SemaphoreType.DMA((TALL_SLOTS,)),
            pltpu.SemaphoreType.DMA((WIDE_SLOTS,)),
            pltpu.SemaphoreType.DMA((3,)),
            pltpu.SemaphoreType.DMA(()),
        ],
        compiler_params=pltpu.CompilerParams(vmem_limit_bytes=124 * 2**20, flags=FLAGS),
    )(
        A_x.reshape(S, D),
        A_mem0.reshape(M, D),
        A_Wq.reshape(n, D // n * H, Dh),
        A_Wk.reshape(n, D // n * H, Dh),
        A_Wv.reshape(n, D // n * H, Dh),
        A_Wo.reshape(H * Dh, D),
        B_w_gate.reshape(n, D // n, F),
        B_w_up.reshape(n, D // n, F),
        B_w_down,
    )
    return out.reshape(B, S, D)
```

```python
import functools

import jax
import jax.numpy as jnp
import jax.experimental.pallas as pl
import jax.experimental.pallas.tpu as pltpu

F32 = jnp.float32
BF16 = jnp.bfloat16
WORD = jnp.uint32
LANES = 128
LN_EPS = 1e-5
MASK_VALUE = -1000000000.0

OFFSETS = (-1.5, -0.5, 0.5, 1.5)
GROUP = 4
QKV_SLOTS, TALL_SLOTS, WIDE_SLOTS = 3, 6, 7
ROWS = 16
NH, NO, NX, NB = 0, 8, 8, 8
FLAGS = None
ORDER = None
PAD, HALF = '', ''
STAGE_ROWS = 128


def _layernorm(x):
    m = jnp.mean(x, axis=-1, keepdims=True)
    c = x - m
    v = jnp.mean(c * c, axis=-1, keepdims=True)
    return c * jax.lax.rsqrt(v + LN_EPS)


def _sigmoid(x):
    return 0.5 * jnp.tanh(0.5 * x) + 0.5


def _reciprocal(x):
    r = pl.reciprocal(x, approx=True)
    return r * (2.0 - x * r)


def _times(c, x):
    return x if c == 1 else c * x


def _split(x, n):
    w = x.shape[1] // n
    return [x[:, i * w:(i + 1) * w] for i in range(n)]


def _pairs(n):
    return [(i, j) for j in range(n) for i in range(j)]


def _row_operand(r, base, both):
    t, n = OFFSETS, len(OFFSETS)
    if r < 2 * n:
        return base(r)
    (i, j), kind = _pairs(n)[(r - 2 * n) // 3], (r - 2 * n) % 3
    s = base(n + i) + base(n + j)
    if kind == 0 or not both:
        return s
    d = t[j] - t[i]
    return s + _times(d, base(j)) if kind == 1 else s - _times(d, base(i))


def _pack_rows(even, odd):
    bits = lambda x: jax.lax.bitcast_convert_type(x.astype(BF16).astype(F32), WORD)
    return (bits(even) >> 16) | bits(odd)


def _weight_operands(w):
    n = len(OFFSETS)
    add = lambda xs: functools.reduce(lambda a, b: a + b, xs)
    sums = []
    for rows in (lambda x: x << 16, lambda x: x & WORD(0xFFFF0000)):
        f = [[jax.lax.bitcast_convert_type(rows(blk), F32) for blk in row] for row in w]
        sums.append([add(f[i]) for i in range(n)]
                    + [f[i][i] - add([f[j][i] for j in range(n) if j != i]) for i in range(n)]
                    + [f[i][j] + f[j][i] for i, j in _pairs(n)])
    sums = [_pack_rows(*s) for s in zip(*sums)]
    ops = sums[:2 * n]
    for s, (i, j) in zip(sums[2 * n:], _pairs(n)):
        ops += [s, w[j][i], w[i][j]]
    return ops


def _paired_matmul(product, both):
    t, n = OFFSETS, len(OFFSETS)
    y1, y2 = [None] * n, [None] * n
    acc = lambda a, b: b if a is None else a + b
    todo = [n - 1] * n
    for k, (i, j) in enumerate(_pairs(n)):
        ti, tj = product(2 * n + 3 * k + 1), product(2 * n + 3 * k + 2)
        y2[i], y2[j] = acc(y2[i], ti), acc(y2[j], tj)
        if both:
            u = _times(1.0 / (t[j] - t[i]), ti + tj - product(2 * n + 3 * k))
            y1[i], y1[j] = acc(y1[i], u), (-u if y1[j] is None else y1[j] - u)
        for m in (i, j):
            todo[m] -= 1
            if todo[m] == 0:
                y2[m] = y2[m] + product(n + m)
                if both:
                    y1[m] = y1[m] + product(m)
                    y2[m] = y2[m] + t[m] * y1[m]
    return (y1 if both else None), y2


def _project(rows_ref, w_ref, both, cols):
    def product(r):
        rows = (rows_ref[r] if r < rows_ref.shape[0]
                else _row_operand(r, lambda m: rows_ref[m], both))
        w = pltpu.bitcast(w_ref[r, :, cols], BF16)
        return jax.lax.dot_general(rows, w, (((1,), (0,)), ((), ())),
                                   preferred_element_type=F32)
    return _paired_matmul(product, both)


def _store_rows(ref, h, rows=slice(None), cols=slice(None)):
    n, both = len(OFFSETS), len(h) == 2
    base = ((list(h[0]) + [b - t * a for t, a, b in zip(OFFSETS, *h)]) if both
            else [None] * n + list(h[0]))
    for r in range(ref.shape[0]):
        if both or (r >= n and (r < 2 * n or (r - 2 * n) % 3)):
            ref[r, rows, cols] = _row_operand(r, base.__getitem__, both)


def _kernel(x_hbm, mem0_hbm, wq_hbm, wk_hbm, wv_hbm, wo_hbm, wg_hbm, wu_hbm, wd_hbm,
            out_hbm,
            x_vm, out_vm, wq, wk, wv, wo, wg, wu, wd,
            h_ref, o_ref, xb_ref, hb_ref, mem_ref, ra_ref, rb_ref, x2_ref, fill_ref,
            mem0_vm, qkv_stage, tall_stage, wide_stage,
            qkv_sems, tall_sems, wide_sems, x_sem, out_sem, *, seg, n_mem, n_heads):
    S, D = x_vm.shape
    F = wg_hbm.shape[2]
    n_seg = S // seg
    L = n_mem + seg
    n = len(OFFSETS)
    gw = GROUP * LANES
    bw = gw // n
    n_a, n_b = n_heads // GROUP, F // gw
    scale = LANES ** -0.5

    class Stream:
        def __init__(self, jobs, stage, sems):
            self.jobs, self.stage, self.sems = jobs, stage, sems
            self.slots = stage.shape[0]

        def copy(self, m, c, slot):
            return pltpu.make_async_copy(self.jobs[m][1](c), self.stage.at[slot],
                                         self.sems.at[slot])

        def start(self, first=0, last=None):
            for c in range(first, self.slots if last is None else last):
                self.copy(0, c, c).start()

        def drain(self, m, refill=None):
            count, _, consume = self.jobs[m]
            first = sum(j[0] for j in self.jobs[:m])

            def body(c, carry):
                slot = (first + c) % self.slots
                self.copy(m, c, slot).wait()
                consume(c, self.stage.at[slot])
                nxt = c + self.slots
                if self.slots < count:
                    pl.when(nxt < count)(lambda: self.copy(m, nxt, slot).start())
                if m + 1 < len(self.jobs):
                    pl.when(nxt >= count)(lambda: self.copy(m + 1, nxt - count, slot).start())
                elif refill:
                    for k in range(self.slots):
                        pl.when(nxt == count + k)(functools.partial(refill, k))
                return carry

            jax.lax.fori_loop(0, count, body, 0)

    kr = STAGE_ROWS // n

    def wide_job(src, dst, per_row, load):
        def consume(c, staged):
            blocks = [pltpu.bitcast(load(staged, i), WORD) for i in range(n)]
            rows = pl.ds(pl.multiple_of(c * (kr // 2), kr // 2), kr // 2)
            for g in range(blocks[0].shape[1] // gw):
                w = [_split(blk[:, g * gw:(g + 1) * gw], n) for blk in blocks]
                for r, op in enumerate(_weight_operands(w)):
                    dst[r, rows, pl.ds(g * bw, bw)] = op
        step = kr * per_row
        return (D // STAGE_ROWS,
                lambda c: src.at[:, pl.ds(pl.multiple_of(c * step, step), step), :],
                consume)

    def tall_job(src, dst):
        def consume(c, staged):
            rows = pl.ds(pl.multiple_of(c * (bw // 2), bw // 2), bw // 2)
            for g in range(D // gw):
                w = [_split(pltpu.bitcast(staged[pl.ds(i * bw, bw), pl.ds(g * gw, gw)], WORD), n)
                     for i in range(n)]
                for r, op in enumerate(_weight_operands(w)):
                    dst[r, rows, pl.ds(g * bw, bw)] = op
        return (src.shape[0] // gw,
                lambda c: src.at[pl.ds(pl.multiple_of(c * gw, gw), gw), :],
                consume)

    def load_heads(staged, i):
        return staged[i].reshape(kr, n_heads, LANES).reshape(kr, n_heads * LANES)

    qi = jax.lax.broadcasted_iota(jnp.int32, fill_ref.shape, 0)
    ki = jax.lax.broadcasted_iota(jnp.int32, fill_ref.shape, 1)
    same = ((qi >= L) == (ki >= L)) & (ki < 2 * L)
    visible = (jnp.where(qi >= L, qi - L, qi) < n_mem) | (qi >= ki)
    fill_ref[...] = jnp.where(same, jnp.where(visible, 0.0, MASK_VALUE), -jnp.inf)

    BOTH = (0, 1)
    join = lambda blocks: jnp.concatenate(blocks, axis=1)

    def project(rows_ref, w_ref, live, cols):
        return _project(rows_ref, w_ref, len(live) == 2, cols)[-len(live):]

    def segment(i, start=0, size=seg):
        return pl.ds(pl.multiple_of(i * seg + start, size), size)

    def segments_in(i, live):
        for r in range(0, seg, ROWS):
            x = [x_vm[segment(jnp.minimum(i, n_seg - 1), r, ROWS), :].astype(F32),
                 x2_ref[pl.ds(r, ROWS), :]]
            if len(live) == 1:
                x = [jnp.where(live[0] == 0, *x)]
            for p, xp in zip(live, x):
                ra_ref[p, pl.ds(r, ROWS), :] = xp
            _store_rows(h_ref, [_split(_layernorm(xp), n) for xp in x],
                       rows=pl.ds(n_mem + r, ROWS))

    def memories_in(live):
        _store_rows(h_ref, [_split(mem_ref[p], n) for p in live], rows=pl.ds(0, n_mem))

    def heads_of(w, cols, live):
        y = project(h_ref, w, live, cols)
        heads = zip(*([h for blk in yp for h in _split(blk, bw // LANES)] for yp in y))
        name = 'q' if w is wq else 'k' if w is wk else 'v'
        pad = (jnp.zeros((LANES - len(live) * L, LANES), F32),) if name in PAD else ()
        return [jnp.concatenate(h + pad, axis=0).astype(BF16 if name in HALF else F32)
                for h in heads]

    def softmax(q, k):
        out = []
        for qh, kh in zip(q, k):
            s = jax.lax.dot_general(qh, kh, (((1,), (1,)), ((), ())),
                                    preferred_element_type=F32)
            fill = fill_ref[pl.ds(0, s.shape[0]), pl.ds(0, s.shape[1])]
            s = jnp.where(fill == 0.0, s * scale, fill)
            p = jnp.exp(s - jnp.max(s, axis=-1, keepdims=True))
            out.append(p * _reciprocal(jnp.sum(p, axis=-1, keepdims=True)))
        return out

    def mix(cols, p, v):
        if p[0].shape[1] < v[0].shape[0]:
            p = [join([ph, jnp.zeros((ph.shape[0], LANES - ph.shape[1]), F32)]) for ph in p]
        p = [ph[:, :v[0].shape[0]] for ph in p]
        o = [jax.lax.dot_general(ph, vh, (((1,), (0,)), ((), ())), preferred_element_type=F32)
             for ph, vh in zip(p, v)]
        per = GROUP // n
        o = [join(o[i * per:(i + 1) * per]) for i in range(n)]
        _store_rows(o_ref, [[a[r:r + L] for a in o] for r in range(0, o[0].shape[0], L)],
                   cols=cols)

    def chunk(c):
        return pl.ds(c * bw, bw)

    def attention_out(c, i, live):
        for p, y in zip(live, project(o_ref, wo, live, chunk(c))):
            y, cols = join(y), pl.ds(c * gw, gw)
            mem_ref[p, :, cols] = y[:n_mem]
            rb_ref[i & 1, p, :, cols] = ra_ref[p, :, cols] + y[n_mem:]

    def glu_in(i, live):
        for r in range(0, seg, ROWS):
            x = [rb_ref[(i + 1) & 1, p, pl.ds(r, ROWS), :] for p in live]
            _store_rows(xb_ref, [_split(_layernorm(xp), n) for xp in x], rows=pl.ds(r, ROWS))

    def gate(cols, g, u, live):
        h = [[_sigmoid(a) * b for a, b in zip(gp, up)] for gp, up in zip(g, u)]
        if len(live) == 1:
            h = [[jnp.where(live[0] == p, a, 0.0) for a in h[0]] for p in BOTH]
        _store_rows(hb_ref, h, cols=cols)

    def glu_out(c, i, live):
        cols = pl.ds(c * gw, gw)
        for p, y in zip(live, project(hb_ref, wd, live, chunk(c))):
            y = rb_ref[i & 1, p, :, cols] + join(y)
            if p == 0:
                x2_ref[:, cols] = y
            else:
                out_vm[segment(jnp.maximum(i - 5, 0)), cols] = y.astype(out_vm.dtype)

    def run(order, i, live):
        val = {what: [] for what in order}
        for what in order:
            c = len(val[what])
            val[what].append({
                'x': lambda: segments_in(i, live),
                'm': lambda: memories_in(live),
                'q': lambda: heads_of(wq, chunk(c), live),
                'k': lambda: heads_of(wk, chunk(c), live),
                'v': lambda: heads_of(wv, chunk(c), live),
                'S': lambda: softmax(val['q'][c], val['k'][c]),
                'P': lambda: mix(chunk(c), val['S'][c], val['v'][c]),
                'W': lambda: attention_out(c, i, live),
                'h': lambda: glu_in(i, live),
                'g': lambda: project(xb_ref, wg, live, chunk(c)),
                'u': lambda: project(xb_ref, wu, live, chunk(c)),
                'G': lambda: gate(chunk(c), val['g'][c], val['u'][c], live),
                'D': lambda: glu_out(c, i, live),
            }[what]())

    def out_copy(i):
        return pltpu.make_async_copy(out_vm.at[segment(i)], out_hbm.at[segment(i)], out_sem)

    n_d = D // gw
    head = pl.ds(0, 4 * seg)
    tail = pl.ds(4 * seg, S - 4 * seg)
    x_head = pltpu.make_async_copy(x_hbm.at[head], x_vm.at[head], x_sem.at[0])
    x_tail = pltpu.make_async_copy(x_hbm.at[tail], x_vm.at[tail], x_sem.at[1])
    mem_copy = pltpu.make_async_copy(mem0_hbm, mem0_vm, x_sem.at[2])

    qkv = Stream([wide_job(s, d, n_heads, load_heads) for s, d in
                  ((wq_hbm, wq), (wk_hbm, wk), (wv_hbm, wv))], qkv_stage, qkv_sems)
    proj = Stream([tall_job(wo_hbm, wo)], tall_stage, tall_sems)
    wide = Stream([wide_job(s, d, 1, lambda staged, i: staged[i])
                   for s, d in ((wg_hbm, wg), (wu_hbm, wu))], wide_stage, wide_sems)
    down = Stream([tall_job(wd_hbm, wd)], tall_stage, tall_sems)

    def refill(stream, calls):
        return lambda k: stream.start(k * stream.slots // calls, (k + 1) * stream.slots // calls)

    qkv.start()
    x_head.start()
    mem_copy.start()
    for m in range(3):
        qkv.drain(m, refill(proj, qkv.slots))
    x_head.wait()
    mem_copy.wait()
    mem_ref[0] = mem_ref[1] = mem0_vm[...].astype(F32)
    x2_ref[...] = rb_ref[0, 1] = rb_ref[1, 1] = jnp.zeros((seg, D), F32)

    attention = 'qkvS' + 'qPkvS' * (n_a - 1)
    glu = 'guG' * n_b

    def full_step(i, carry):
        pl.when(i == 4)(x_tail.wait)
        pl.when(i > 5)(lambda: out_copy(i - 6).start())
        run(ORDER or 'mxD' + attention + 'D' * (n_d - 1) + 'Ph' + glu + 'W' * n_d, i, BOTH)
        return carry

    def ragged_step(j, carry):
        lone = (jnp.where(j < 4, 0, 1),)
        i = jnp.where(j < 4, jnp.minimum(j, 2), j - 4 + n_seg)
        phase = lambda cond, order, live: pl.when(cond)(lambda: run(order, i, live))
        attends = (j != 3) & (j < 7)
        pl.when(j >= 4)(lambda: out_copy(i - 6).start())
        phase(attends, 'mx' + attention[:-5] + 'qkPSvP', lone)
        pl.when(j == 0)(lambda: proj.drain(0, refill(wide, proj.slots)))
        pl.when(j == 1)(lambda: wide.drain(0))

        pl.when(j == 2)(lambda: wide.drain(1, lambda k: down.start() if k == 0 else None))
        pl.when(j == 3)(lambda: down.drain(0, lambda k: x_tail.start() if k == 0 else None))
        phase((j >= 3) & (j < 6), 'D' * n_d, BOTH)
        phase(j >= 6, 'D' * n_d, (1,))
        phase(j == 4, 'h' + glu, BOTH)
        pl.when((j > 1) & (j != 4) & (j < 8))(
            lambda: run('h' + glu, jnp.where(j == 2, 1, i), lone))
        phase((j != 2) & (j < 7), 'W' * n_d, lone)

        @pl.when(j == 3)
        def _():
            jax.lax.fori_loop(3, n_seg, full_step, 0)
        return carry

    jax.lax.fori_loop(0, 9, ragged_step, 0)
    out_copy(n_seg - 1).start()
    pltpu.make_async_copy(out_vm, out_hbm, out_sem).wait()


@functools.partial(jax.jit, static_argnames=("A_seg_len",))
def pallas_interleave_layers__memory_aug_recurrent_mem_tr__glu_gated_glu__prompt_kernel(
    A_x: jax.Array,
    A_mem0: jax.Array,
    A_Wq: jax.Array,
    A_Wk: jax.Array,
    A_Wv: jax.Array,
    A_Wo: jax.Array,
    A_seg_len: int,
    B_x: jax.Array,
    B_w_gate: jax.Array,
    B_w_up: jax.Array,
    B_w_down: jax.Array,
):
    del B_x
    B, S, D = A_x.shape
    _, H, Dh = A_Wq.shape
    M = A_mem0.shape[1]
    F = B_w_gate.shape[1]
    seg = int(A_seg_len)
    assert B == 1 and Dh == LANES and S % seg == 0 and S // seg >= 8
    n = len(OFFSETS)
    R = (3 * n * n + n) // 2
    L = M + seg

    def packed(k, cols):
        return pltpu.VMEM((R, k // n // 2, cols // n), WORD)

    hbm = pl.BlockSpec(memory_space=pl.ANY)
    out = pl.pallas_call(
        functools.partial(_kernel, seg=seg, n_mem=M, n_heads=H),
        out_shape=jax.ShapeDtypeStruct((S, D), A_x.dtype),
        in_specs=[hbm] * 9,
        out_specs=hbm,
        scratch_shapes=[
            pltpu.VMEM((S, D), A_x.dtype),
            pltpu.VMEM((S, D), A_x.dtype),
            packed(D, H * Dh),
            packed(D, H * Dh),
            packed(D, H * Dh),
            packed(H * Dh, D),
            packed(D, F),
            packed(D, F),
            packed(F, D),
            pltpu.VMEM((NH or R, L, D // n), F32),
            pltpu.VMEM((NO or R, L, H * Dh // n), F32),
            pltpu.VMEM((NX or R, seg, D // n), F32),
            pltpu.VMEM((NB or R, seg, F // n), F32),
            pltpu.VMEM((2, M, D), F32),
            pltpu.VMEM((2, seg, D), F32),
            pltpu.VMEM((2, 2, seg, D), F32),
            pltpu.VMEM((seg, D), F32),
            pltpu.VMEM((2 * L, LANES), F32),
            pltpu.VMEM((M, D), A_mem0.dtype),
            pltpu.VMEM((QKV_SLOTS, n, STAGE_ROWS // n * H, Dh), BF16),
            pltpu.VMEM((TALL_SLOTS, GROUP * LANES, D), BF16),
            pltpu.VMEM((WIDE_SLOTS, n, STAGE_ROWS // n, F), BF16),
            pltpu.SemaphoreType.DMA((QKV_SLOTS,)),
            pltpu.SemaphoreType.DMA((TALL_SLOTS,)),
            pltpu.SemaphoreType.DMA((WIDE_SLOTS,)),
            pltpu.SemaphoreType.DMA((3,)),
            pltpu.SemaphoreType.DMA(()),
        ],
        compiler_params=pltpu.CompilerParams(vmem_limit_bytes=124 * 2**20, flags=FLAGS),
    )(
        A_x.reshape(S, D),
        A_mem0.reshape(M, D),
        A_Wq.reshape(n, D // n * H, Dh),
        A_Wk.reshape(n, D // n * H, Dh),
        A_Wv.reshape(n, D // n * H, Dh),
        A_Wo.reshape(H * Dh, D),
        B_w_gate.reshape(n, D // n, F),
        B_w_up.reshape(n, D // n, F),
        B_w_down,
    )
    return out.reshape(B, S, D)
```

```python
import functools

import jax
import jax.numpy as jnp
import jax.experimental.pallas as pl
import jax.experimental.pallas.tpu as pltpu

F32 = jnp.float32
BF16 = jnp.bfloat16
WORD = jnp.uint32
LANES = 128
PACK = 16
LN_EPS = 1e-5
MASK_VALUE = -1000000000.0

OFFSETS = (-1.5, -0.5, 0.5, 1.5)
GROUP = 4
QKV_SLOTS, TALL_SLOTS, WIDE_SLOTS = 3, 6, 7
ROWS = 16
NH, NO, NX, NB = 0, 8, 8, 8
FLAGS = None
ORDER = None
PAD, HALF = 'kv', 'kv'
STAGE_ROWS = 128


def _layernorm(x):
    m = jnp.mean(x, axis=-1, keepdims=True)
    c = x - m
    v = jnp.mean(c * c, axis=-1, keepdims=True)
    return c * jax.lax.rsqrt(v + LN_EPS)


def _sigmoid(x):
    return 0.5 * jnp.tanh(0.5 * x) + 0.5


def _reciprocal(x):
    r = pl.reciprocal(x, approx=True)
    return r * (2.0 - x * r)


def _times(c, x):
    return x if c == 1 else c * x


def _split(x, n):
    w = x.shape[1] // n
    return [x[:, i * w:(i + 1) * w] for i in range(n)]


def _pairs(n):
    return [(i, j) for j in range(n) for i in range(j)]


def _row_operand(r, base, both):
    t, n = OFFSETS, len(OFFSETS)
    if r < 2 * n:
        return base(r)
    (i, j), kind = _pairs(n)[(r - 2 * n) // 3], (r - 2 * n) % 3
    s = base(n + i) + base(n + j)
    if kind == 0 or not both:
        return s
    d = t[j] - t[i]
    return s + _times(d, base(j)) if kind == 1 else s - _times(d, base(i))


def _pack_rows(even, odd):
    bits = lambda x: jax.lax.bitcast_convert_type(x.astype(BF16).astype(F32), WORD)
    return (bits(even) >> 16) | bits(odd)


def _weight_operands(w):
    n = len(OFFSETS)
    add = lambda xs: functools.reduce(lambda a, b: a + b, xs)
    sums = []
    for rows in (lambda x: x << 16, lambda x: x & WORD(0xFFFF0000)):
        f = [[jax.lax.bitcast_convert_type(rows(blk), F32) for blk in row] for row in w]
        sums.append([add(f[i]) for i in range(n)]
                    + [f[i][i] - add([f[j][i] for j in range(n) if j != i]) for i in range(n)]
                    + [f[i][j] + f[j][i] for i, j in _pairs(n)])
    sums = [_pack_rows(*s) for s in zip(*sums)]
    ops = sums[:2 * n]
    for s, (i, j) in zip(sums[2 * n:], _pairs(n)):
        ops += [s, w[j][i], w[i][j]]
    return ops


def _paired_matmul(product, both):
    t, n = OFFSETS, len(OFFSETS)
    y1, y2 = [None] * n, [None] * n
    acc = lambda a, b: b if a is None else a + b
    todo = [n - 1] * n
    for k, (i, j) in enumerate(_pairs(n)):
        ti, tj = product(2 * n + 3 * k + 1), product(2 * n + 3 * k + 2)
        y2[i], y2[j] = acc(y2[i], ti), acc(y2[j], tj)
        if both:
            u = _times(1.0 / (t[j] - t[i]), ti + tj - product(2 * n + 3 * k))
            y1[i], y1[j] = acc(y1[i], u), (-u if y1[j] is None else y1[j] - u)
        for m in (i, j):
            todo[m] -= 1
            if todo[m] == 0:
                y2[m] = y2[m] + product(n + m)
                if both:
                    y1[m] = y1[m] + product(m)
                    y2[m] = y2[m] + t[m] * y1[m]
    return (y1 if both else None), y2


def _project(rows_ref, w_ref, both, cols):
    def product(r):
        rows = (rows_ref[r] if r < rows_ref.shape[0]
                else _row_operand(r, lambda m: rows_ref[m], both))
        w = pltpu.bitcast(w_ref[r, :, cols], BF16)
        return jax.lax.dot_general(rows, w, (((1,), (0,)), ((), ())),
                                   preferred_element_type=F32)
    return _paired_matmul(product, both)


def _store_rows(ref, h, rows=slice(None), cols=slice(None)):
    n, both = len(OFFSETS), len(h) == 2
    base = ((list(h[0]) + [b - t * a for t, a, b in zip(OFFSETS, *h)]) if both
            else [None] * n + list(h[0]))
    for r in range(ref.shape[0]):
        if both or (r >= n and (r < 2 * n or (r - 2 * n) % 3)):
            ref[r, rows, cols] = _row_operand(r, base.__getitem__, both)


def _kernel(x_hbm, mem0_hbm, wq_hbm, wk_hbm, wv_hbm, wo_hbm, wg_hbm, wu_hbm, wd_hbm,
            out_hbm,
            x_vm, out_vm, wq, wk, wv, wo, wg, wu, wd,
            h_ref, o_ref, xb_ref, hb_ref, mem_ref, ra_ref, rb_ref, x2_ref, fill_ref,
            mem0_vm, qkv_stage, tall_stage, wide_stage,
            qkv_sems, tall_sems, wide_sems, x_sem, out_sem, *, seg, n_mem, n_heads):
    S, D = x_vm.shape
    F = wg_hbm.shape[2]
    n_seg = S // seg
    L = n_mem + seg
    n = len(OFFSETS)
    gw = GROUP * LANES
    bw = gw // n
    n_a, n_b = n_heads // GROUP, F // gw
    scale = LANES ** -0.5

    class Stream:
        def __init__(self, jobs, stage, sems):
            self.jobs, self.stage, self.sems = jobs, stage, sems
            self.slots = stage.shape[0]

        def copy(self, m, c, slot):
            return pltpu.make_async_copy(self.jobs[m][1](c), self.stage.at[slot],
                                         self.sems.at[slot])

        def start(self, first=0, last=None):
            for c in range(first, self.slots if last is None else last):
                self.copy(0, c, c).start()

        def drain(self, m, refill=None):
            count, _, consume = self.jobs[m]
            first = sum(j[0] for j in self.jobs[:m])

            def body(c, carry):
                slot = (first + c) % self.slots
                self.copy(m, c, slot).wait()
                consume(c, self.stage.at[slot])
                nxt = c + self.slots
                if self.slots < count:
                    pl.when(nxt < count)(lambda: self.copy(m, nxt, slot).start())
                if m + 1 < len(self.jobs):
                    pl.when(nxt >= count)(lambda: self.copy(m + 1, nxt - count, slot).start())
                elif refill:
                    for k in range(self.slots):
                        pl.when(nxt == count + k)(functools.partial(refill, k))
                return carry

            jax.lax.fori_loop(0, count, body, 0)

    kr = STAGE_ROWS // n

    def put(dst, row, g, blocks):
        rows = pl.ds(pl.multiple_of(row // 2, PACK // 2), PACK // 2)
        w = [_split(pltpu.bitcast(blk, WORD), n) for blk in blocks]
        for r, op in enumerate(_weight_operands(w)):
            dst[r, rows, pl.ds(g * bw, bw)] = op

    def head_job(src, dst):
        def consume(c, staged):
            for r in range(0, kr, PACK):
                blocks = [staged[i, pl.ds(r * n_heads, PACK * n_heads), :]
                          .reshape(PACK, n_heads, LANES).reshape(PACK, n_heads * LANES)
                          for i in range(n)]
                for g in range(n_a):
                    put(dst, c * kr + r, g, [blk[:, g * gw:(g + 1) * gw] for blk in blocks])
        step = kr * n_heads
        return (D // STAGE_ROWS,
                lambda c: src.at[:, pl.ds(pl.multiple_of(c * step, step), step), :], consume)

    def wide_job(src, dst):
        def consume(c, staged):
            for r in range(0, kr, PACK):
                for g in range(n_b):
                    put(dst, c * kr + r, g,
                        [staged[i, pl.ds(r, PACK), pl.ds(g * gw, gw)] for i in range(n)])
        return (D // STAGE_ROWS,
                lambda c: src.at[:, pl.ds(pl.multiple_of(c * kr, kr), kr), :], consume)

    def tall_job(src, dst):
        def consume(c, staged):
            for r in range(0, bw, PACK):
                for g in range(D // gw):
                    put(dst, c * bw + r, g,
                        [staged[pl.ds(i * bw + r, PACK), pl.ds(g * gw, gw)] for i in range(n)])
        return (src.shape[0] // gw,
                lambda c: src.at[pl.ds(pl.multiple_of(c * gw, gw), gw), :], consume)

    qi = jax.lax.broadcasted_iota(jnp.int32, fill_ref.shape, 0)
    ki = jax.lax.broadcasted_iota(jnp.int32, fill_ref.shape, 1)
    same = ((qi >= L) == (ki >= L)) & (ki < 2 * L)
    visible = (jnp.where(qi >= L, qi - L, qi) < n_mem) | (qi >= ki)
    fill_ref[...] = jnp.where(same, jnp.where(visible, 0.0, MASK_VALUE), -jnp.inf)

    BOTH = (0, 1)
    join = lambda blocks: jnp.concatenate(blocks, axis=1)

    def project(rows_ref, w_ref, live, cols):
        return _project(rows_ref, w_ref, len(live) == 2, cols)[-len(live):]

    def segment(i, start=0, size=seg):
        return pl.ds(pl.multiple_of(i * seg + start, size), size)

    def segments_in(i, live):
        for r in range(0, seg, ROWS):
            x = [x_vm[segment(jnp.minimum(i, n_seg - 1), r, ROWS), :].astype(F32),
                 x2_ref[pl.ds(r, ROWS), :]]
            if len(live) == 1:
                x = [jnp.where(live[0] == 0, *x)]
            for p, xp in zip(live, x):
                ra_ref[p, pl.ds(r, ROWS), :] = xp
            _store_rows(h_ref, [_split(_layernorm(xp), n) for xp in x],
                       rows=pl.ds(n_mem + r, ROWS))

    def memories_in(live):
        _store_rows(h_ref, [_split(mem_ref[p], n) for p in live], rows=pl.ds(0, n_mem))

    def heads_of(w, cols, live):
        y = project(h_ref, w, live, cols)
        heads = zip(*([h for blk in yp for h in _split(blk, bw // LANES)] for yp in y))
        name = 'q' if w is wq else 'k' if w is wk else 'v'
        pad = (jnp.zeros((LANES - len(live) * L, LANES), F32),) if name in PAD else ()
        return [jnp.concatenate(h + pad, axis=0).astype(BF16 if name in HALF else F32)
                for h in heads]

    def softmax(q, k):
        out = []
        for qh, kh in zip(q, k):
            s = jax.lax.dot_general(qh, kh, (((1,), (1,)), ((), ())),
                                    preferred_element_type=F32)
            fill = fill_ref[pl.ds(0, s.shape[0]), pl.ds(0, s.shape[1])]
            s = jnp.where(fill == 0.0, s * scale, fill)
            p = jnp.exp(s - jnp.max(s, axis=-1, keepdims=True))
            out.append(p * _reciprocal(jnp.sum(p, axis=-1, keepdims=True)))
        return out

    def mix(cols, p, v):
        if p[0].shape[1] < v[0].shape[0]:
            p = [join([ph, jnp.zeros((ph.shape[0], LANES - ph.shape[1]), F32)]) for ph in p]
        p = [ph[:, :v[0].shape[0]] for ph in p]
        o = [jax.lax.dot_general(ph, vh, (((1,), (0,)), ((), ())), preferred_element_type=F32)
             for ph, vh in zip(p, v)]
        per = GROUP // n
        o = [join(o[i * per:(i + 1) * per]) for i in range(n)]
        _store_rows(o_ref, [[a[r:r + L] for a in o] for r in range(0, o[0].shape[0], L)],
                   cols=cols)

    def chunk(c):
        return pl.ds(c * bw, bw)

    def attention_out(c, i, live):
        for p, y in zip(live, project(o_ref, wo, live, chunk(c))):
            y, cols = join(y), pl.ds(c * gw, gw)
            mem_ref[p, :, cols] = y[:n_mem]
            rb_ref[i & 3, p, :, cols] = ra_ref[p, :, cols] + y[n_mem:]

    def glu_in(i, live):
        for r in range(0, seg, ROWS):
            x = [rb_ref[(i + 3) & 3, p, pl.ds(r, ROWS), :] for p in live]
            _store_rows(xb_ref, [_split(_layernorm(xp), n) for xp in x], rows=pl.ds(r, ROWS))

    def gate(cols, g, u, live):
        h = [[_sigmoid(a) * b for a, b in zip(gp, up)] for gp, up in zip(g, u)]
        if len(live) == 1:
            h = [[jnp.where(live[0] == p, a, 0.0) for a in h[0]] for p in BOTH]
        _store_rows(hb_ref, h, cols=cols)

    def glu_out(c, i, live):
        cols = pl.ds(c * gw, gw)
        for p, y in zip(live, project(hb_ref, wd, live, chunk(c))):
            y = rb_ref[(i + 2) & 3, p, :, cols] + join(y)
            if p == 0:
                x2_ref[:, cols] = y
            else:
                out_vm[segment(jnp.maximum(i - 5, 0)), cols] = y.astype(out_vm.dtype)

    def run(order, i, live):
        val = {what: [] for what in order}
        for what in order:
            c = len(val[what])
            val[what].append({
                'x': lambda: segments_in(i, live),
                'm': lambda: memories_in(live),
                'q': lambda: heads_of(wq, chunk(c), live),
                'k': lambda: heads_of(wk, chunk(c), live),
                'v': lambda: heads_of(wv, chunk(c), live),
                'S': lambda: softmax(val['q'][c], val['k'][c]),
                'P': lambda: mix(chunk(c), val['S'][c], val['v'][c]),
                'W': lambda: attention_out(c, i, live),
                'h': lambda: glu_in(i, live),
                'g': lambda: project(xb_ref, wg, live, chunk(c)),
                'u': lambda: project(xb_ref, wu, live, chunk(c)),
                'G': lambda: gate(chunk(c), val['g'][c], val['u'][c], live),
                'D': lambda: glu_out(c, i, live),
            }[what]())

    def out_copy(i):
        return pltpu.make_async_copy(out_vm.at[segment(i)], out_hbm.at[segment(i)], out_sem)

    n_d = D // gw
    head = pl.ds(0, 4 * seg)
    tail = pl.ds(4 * seg, S - 4 * seg)
    x_head = pltpu.make_async_copy(x_hbm.at[head], x_vm.at[head], x_sem.at[0])
    x_tail = pltpu.make_async_copy(x_hbm.at[tail], x_vm.at[tail], x_sem.at[1])
    mem_copy = pltpu.make_async_copy(mem0_hbm, mem0_vm, x_sem.at[2])

    qkv = Stream([head_job(s, d) for s, d in
                  ((wq_hbm, wq), (wk_hbm, wk), (wv_hbm, wv))], qkv_stage, qkv_sems)
    proj = Stream([tall_job(wo_hbm, wo)], tall_stage, tall_sems)
    wide = Stream([wide_job(s, d)
                   for s, d in ((wg_hbm, wg), (wu_hbm, wu))], wide_stage, wide_sems)
    down = Stream([tall_job(wd_hbm, wd)], tall_stage, tall_sems)

    def refill(stream, calls):
        return lambda k: stream.start(k * stream.slots // calls, (k + 1) * stream.slots // calls)

    qkv.start()
    x_head.start()
    mem_copy.start()
    for m in range(3):
        qkv.drain(m, refill(proj, qkv.slots))
    x_head.wait()
    mem_copy.wait()
    mem_ref[0] = mem_ref[1] = mem0_vm[...].astype(F32)
    x2_ref[...] = rb_ref[0, 1] = rb_ref[1, 1] = rb_ref[2, 1] = jnp.zeros((seg, D), F32)

    attention = 'qkvS' + 'qPkvS' * (n_a - 1)
    glu = 'guG' * n_b

    def full_step(i, carry):
        run(ORDER or 'mxD' + attention + 'D' * (n_d - 1) + 'Ph' + glu + 'W' * n_d, i, BOTH)
        return carry

    def ragged_step(j, carry):
        lone = (jnp.where(j < 4, 0, 1),)
        i = jnp.where(j < 4, jnp.minimum(j, 2), j - 4 + n_seg)
        phase = lambda cond, order, live: pl.when(cond)(lambda: run(order, i, live))
        attends = (j != 3) & (j < 7)
        pl.when(j >= 4)(lambda: out_copy(i - 6).start())
        phase(attends, 'mx' + attention[:-5] + 'qkPSvP', lone)
        pl.when(j == 0)(lambda: proj.drain(0, refill(wide, proj.slots)))
        pl.when(j == 1)(lambda: wide.drain(0))

        pl.when(j == 2)(lambda: wide.drain(1, lambda k: down.start() if k == 0 else None))
        pl.when(j == 3)(lambda: down.drain(0, lambda k: x_tail.start() if k == 0 else None))
        phase((j >= 3) & (j < 6), 'D' * n_d, BOTH)
        phase(j >= 6, 'D' * n_d, (1,))
        phase(j == 4, 'h' + glu, BOTH)
        pl.when((j > 1) & (j != 4) & (j < 8))(
            lambda: run('h' + glu, jnp.where(j == 2, 1, i), lone))
        phase(attends, 'W' * n_d, lone)

        @pl.when(j == 3)
        def _():
            x_tail.wait()
            jax.lax.fori_loop(3, n_seg, full_step, 0)
            done = pl.ds(0, (n_seg - 6) * seg)
            pltpu.make_async_copy(out_vm.at[done], out_hbm.at[done], out_sem).start()
        return carry

    jax.lax.fori_loop(0, 9, ragged_step, 0)
    out_copy(n_seg - 1).start()
    pltpu.make_async_copy(out_vm, out_hbm, out_sem).wait()


@functools.partial(jax.jit, static_argnames=("A_seg_len",))
def pallas_interleave_layers__memory_aug_recurrent_mem_tr__glu_gated_glu__prompt_kernel(
    A_x: jax.Array,
    A_mem0: jax.Array,
    A_Wq: jax.Array,
    A_Wk: jax.Array,
    A_Wv: jax.Array,
    A_Wo: jax.Array,
    A_seg_len: int,
    B_x: jax.Array,
    B_w_gate: jax.Array,
    B_w_up: jax.Array,
    B_w_down: jax.Array,
):
    del B_x
    B, S, D = A_x.shape
    _, H, Dh = A_Wq.shape
    M = A_mem0.shape[1]
    F = B_w_gate.shape[1]
    seg = int(A_seg_len)
    assert B == 1 and Dh == LANES and S % seg == 0 and S // seg >= 8
    n = len(OFFSETS)
    R = (3 * n * n + n) // 2
    L = M + seg

    def packed(k, cols):
        return pltpu.VMEM((R, k // n // 2, cols // n), WORD)

    hbm = pl.BlockSpec(memory_space=pl.ANY)
    out = pl.pallas_call(
        functools.partial(_kernel, seg=seg, n_mem=M, n_heads=H),
        out_shape=jax.ShapeDtypeStruct((S, D), A_x.dtype),
        in_specs=[hbm] * 9,
        out_specs=hbm,
        scratch_shapes=[
            pltpu.VMEM((S, D), A_x.dtype),
            pltpu.VMEM((S, D), A_x.dtype),
            packed(D, H * Dh),
            packed(D, H * Dh),
            packed(D, H * Dh),
            packed(H * Dh, D),
            packed(D, F),
            packed(D, F),
            packed(F, D),
            pltpu.VMEM((NH or R, L, D // n), F32),
            pltpu.VMEM((NO or R, L, H * Dh // n), F32),
            pltpu.VMEM((NX or R, seg, D // n), F32),
            pltpu.VMEM((NB or R, seg, F // n), F32),
            pltpu.VMEM((2, M, D), F32),
            pltpu.VMEM((2, seg, D), F32),
            pltpu.VMEM((4, 2, seg, D), F32),
            pltpu.VMEM((seg, D), F32),
            pltpu.VMEM((2 * L, LANES), F32),
            pltpu.VMEM((M, D), A_mem0.dtype),
            pltpu.VMEM((QKV_SLOTS, n, STAGE_ROWS // n * H, Dh), BF16),
            pltpu.VMEM((TALL_SLOTS, GROUP * LANES, D), BF16),
            pltpu.VMEM((WIDE_SLOTS, n, STAGE_ROWS // n, F), BF16),
            pltpu.SemaphoreType.DMA((QKV_SLOTS,)),
            pltpu.SemaphoreType.DMA((TALL_SLOTS,)),
            pltpu.SemaphoreType.DMA((WIDE_SLOTS,)),
            pltpu.SemaphoreType.DMA((3,)),
            pltpu.SemaphoreType.DMA(()),
        ],
        compiler_params=pltpu.CompilerParams(vmem_limit_bytes=124 * 2**20, flags=FLAGS),
    )(
        A_x.reshape(S, D),
        A_mem0.reshape(M, D),
        A_Wq.reshape(n, D // n * H, Dh),
        A_Wk.reshape(n, D // n * H, Dh),
        A_Wv.reshape(n, D // n * H, Dh),
        A_Wo.reshape(H * Dh, D),
        B_w_gate.reshape(n, D // n, F),
        B_w_up.reshape(n, D // n, F),
        B_w_down,
    )
    return out.reshape(B, S, D)
```

```python
import functools

import jax
import jax.numpy as jnp
import jax.experimental.pallas as pl
import jax.experimental.pallas.tpu as pltpu

F32 = jnp.float32
BF16 = jnp.bfloat16
WORD = jnp.uint32
LANES = 128
PACK = 16
LN_EPS = 1e-5
MASK_VALUE = -1000000000.0

OFFSETS = (-1.5, -0.5, 0.5, 1.5)
GROUP = 4
QKV_SLOTS, TALL_SLOTS, WIDE_SLOTS = 3, 6, 7
ROWS = 16
ORDER = None
LONE = None
STAGE_ROWS = 128


def _layernorm(x):
    m = jnp.mean(x, axis=-1, keepdims=True)
    c = x - m
    v = jnp.mean(c * c, axis=-1, keepdims=True)
    return c * jax.lax.rsqrt(v + LN_EPS)


def _sigmoid(x):
    return 0.5 * jnp.tanh(0.5 * x) + 0.5


def _reciprocal(x):
    r = pl.reciprocal(x, approx=True)
    return r * (2.0 - x * r)


def _times(c, x):
    return x if c == 1 else c * x


def _split(x, n):
    w = x.shape[1] // n
    return [x[:, i * w:(i + 1) * w] for i in range(n)]


def _pairs(n):
    return [(i, j) for j in range(n) for i in range(j)]


def _row_operand(r, base, both):
    t, n = OFFSETS, len(OFFSETS)
    if r < 2 * n:
        return base(r)
    (i, j), kind = _pairs(n)[(r - 2 * n) // 3], (r - 2 * n) % 3
    s = base(n + i) + base(n + j)
    if kind == 0 or not both:
        return s
    d = t[j] - t[i]
    return s + _times(d, base(j)) if kind == 1 else s - _times(d, base(i))


def _pack_rows(even, odd):
    bits = lambda x: jax.lax.bitcast_convert_type(x.astype(BF16).astype(F32), WORD)
    return (bits(even) >> 16) | bits(odd)


def _weight_operands(w):
    n = len(OFFSETS)
    add = lambda xs: functools.reduce(lambda a, b: a + b, xs)
    sums = []
    for rows in (lambda x: x << 16, lambda x: x & WORD(0xFFFF0000)):
        f = [[jax.lax.bitcast_convert_type(rows(blk), F32) for blk in row] for row in w]
        sums.append([add(f[i]) for i in range(n)]
                    + [f[i][i] - add([f[j][i] for j in range(n) if j != i]) for i in range(n)]
                    + [f[i][j] + f[j][i] for i, j in _pairs(n)])
    sums = [_pack_rows(*s) for s in zip(*sums)]
    ops = sums[:2 * n]
    for s, (i, j) in zip(sums[2 * n:], _pairs(n)):
        ops += [s, w[j][i], w[i][j]]
    return ops


def _paired_matmul(product, both):
    t, n = OFFSETS, len(OFFSETS)
    y1, y2 = [None] * n, [None] * n
    acc = lambda a, b: b if a is None else a + b
    todo = [n - 1] * n
    for k, (i, j) in enumerate(_pairs(n)):
        ti, tj = product(2 * n + 3 * k + 1), product(2 * n + 3 * k + 2)
        y2[i], y2[j] = acc(y2[i], ti), acc(y2[j], tj)
        if both:
            u = _times(1.0 / (t[j] - t[i]), ti + tj - product(2 * n + 3 * k))
            y1[i], y1[j] = acc(y1[i], u), (-u if y1[j] is None else y1[j] - u)
        for m in (i, j):
            todo[m] -= 1
            if todo[m] == 0:
                y2[m] = y2[m] + product(n + m)
                if both:
                    y1[m] = y1[m] + product(m)
                    y2[m] = y2[m] + t[m] * y1[m]
    return (y1 if both else None), y2


def _project(rows_ref, w_ref, both, cols):
    def product(r):
        rows = (rows_ref[r] if r < rows_ref.shape[0]
                else _row_operand(r, lambda m: rows_ref[m], both))
        w = pltpu.bitcast(w_ref[r, :, cols], BF16)
        return jax.lax.dot_general(rows, w, (((1,), (0,)), ((), ())),
                                   preferred_element_type=F32)
    return _paired_matmul(product, both)


def _store_rows(ref, h, rows=slice(None), cols=slice(None)):
    n, both = len(OFFSETS), len(h) == 2
    base = ((list(h[0]) + [b - t * a for t, a, b in zip(OFFSETS, *h)]) if both
            else [None] * n + list(h[0]))
    for r in range(ref.shape[0]):
        if both or (r >= n and (r < 2 * n or (r - 2 * n) % 3)):
            ref[r, rows, cols] = _row_operand(r, base.__getitem__, both)


def _kernel(x_hbm, mem0_hbm, wq_hbm, wk_hbm, wv_hbm, wo_hbm, wg_hbm, wu_hbm, wd_hbm,
            out_hbm,
            x_vm, out_vm, wq, wk, wv, wo, wg, wu, wd,
            h_ref, o_ref, xb_ref, hb_ref, mem_ref, ra_ref, rb_ref, x2_ref, fill_ref,
            mem0_vm, qkv_stage, tall_stage, wide_stage,
            qkv_sems, tall_sems, wide_sems, x_sem, out_sem, *, seg, n_mem, n_heads):
    S, D = x_vm.shape
    F = wg_hbm.shape[2]
    n_seg = S // seg
    L = n_mem + seg
    n = len(OFFSETS)
    gw = GROUP * LANES
    bw = gw // n
    n_a, n_b = n_heads // GROUP, F // gw
    scale = LANES ** -0.5

    class Stream:
        def __init__(self, jobs, stage, sems):
            self.jobs, self.stage, self.sems = jobs, stage, sems
            self.slots = stage.shape[0]

        def copy(self, m, c, slot):
            return pltpu.make_async_copy(self.jobs[m][1](c), self.stage.at[slot],
                                         self.sems.at[slot])

        def start(self, first=0, last=None):
            for c in range(first, self.slots if last is None else last):
                self.copy(0, c, c).start()

        def drain(self, m, refill=None):
            count, _, consume = self.jobs[m]
            first = sum(j[0] for j in self.jobs[:m])

            def body(c, carry):
                slot = (first + c) % self.slots
                self.copy(m, c, slot).wait()
                consume(c, self.stage.at[slot])
                nxt = c + self.slots
                if self.slots < count:
                    pl.when(nxt < count)(lambda: self.copy(m, nxt, slot).start())
                if m + 1 < len(self.jobs):
                    pl.when(nxt >= count)(lambda: self.copy(m + 1, nxt - count, slot).start())
                elif refill:
                    for k in range(self.slots):
                        pl.when(nxt == count + k)(functools.partial(refill, k))
                return carry

            jax.lax.fori_loop(0, count, body, 0)

    kr = STAGE_ROWS // n

    def put(dst, row, g, blocks):
        rows = pl.ds(pl.multiple_of(row // 2, PACK // 2), PACK // 2)
        w = [_split(pltpu.bitcast(blk, WORD), n) for blk in blocks]
        for r, op in enumerate(_weight_operands(w)):
            dst[r, rows, pl.ds(g * bw, bw)] = op

    def head_job(src, dst):
        def consume(c, staged):
            for r in range(0, kr, PACK):
                blocks = [staged[i, pl.ds(r * n_heads, PACK * n_heads), :]
                          .reshape(PACK, n_heads, LANES).reshape(PACK, n_heads * LANES)
                          for i in range(n)]
                for g in range(n_a):
                    put(dst, c * kr + r, g, [blk[:, g * gw:(g + 1) * gw] for blk in blocks])
        step = kr * n_heads
        return (D // STAGE_ROWS,
                lambda c: src.at[:, pl.ds(pl.multiple_of(c * step, step), step), :], consume)

    def wide_job(src, dst):
        def consume(c, staged):
            for r in range(0, kr, PACK):
                for g in range(n_b):
                    put(dst, c * kr + r, g,
                        [staged[i, pl.ds(r, PACK), pl.ds(g * gw, gw)] for i in range(n)])
        return (D // STAGE_ROWS,
                lambda c: src.at[:, pl.ds(pl.multiple_of(c * kr, kr), kr), :], consume)

    def tall_job(src, dst):
        def consume(c, staged):
            for r in range(0, bw, PACK):
                for g in range(D // gw):
                    put(dst, c * bw + r, g,
                        [staged[pl.ds(i * bw + r, PACK), pl.ds(g * gw, gw)] for i in range(n)])
        return (src.shape[0] // gw,
                lambda c: src.at[pl.ds(pl.multiple_of(c * gw, gw), gw), :], consume)

    qi = jax.lax.broadcasted_iota(jnp.int32, fill_ref.shape, 0)
    ki = jax.lax.broadcasted_iota(jnp.int32, fill_ref.shape, 1)
    same = ((qi >= L) == (ki >= L)) & (ki < 2 * L)
    visible = (jnp.where(qi >= L, qi - L, qi) < n_mem) | (qi >= ki)
    fill_ref[...] = jnp.where(same, jnp.where(visible, 0.0, MASK_VALUE), -jnp.inf)

    BOTH = (0, 1)
    join = lambda blocks: jnp.concatenate(blocks, axis=1)

    def project(rows_ref, w_ref, live, cols):
        return _project(rows_ref, w_ref, len(live) == 2, cols)[-len(live):]

    def segment(i, start=0, size=seg):
        return pl.ds(pl.multiple_of(i * seg + start, size), size)

    def segments_in(i, live):
        for r in range(0, seg, ROWS):
            x = [x_vm[segment(jnp.minimum(i, n_seg - 1), r, ROWS), :].astype(F32),
                 x2_ref[pl.ds(r, ROWS), :]]
            if len(live) == 1:
                x = [jnp.where(live[0] == 0, *x)]
            for p, xp in zip(live, x):
                ra_ref[p, pl.ds(r, ROWS), :] = xp
            _store_rows(h_ref, [_split(_layernorm(xp), n) for xp in x],
                       rows=pl.ds(n_mem + r, ROWS))

    def memories_in(live):
        _store_rows(h_ref, [_split(mem_ref[p], n) for p in live], rows=pl.ds(0, n_mem))

    def heads_of(w, cols, live):
        y = project(h_ref, w, live, cols)
        heads = zip(*([h for blk in yp for h in _split(blk, bw // LANES)] for yp in y))
        if w is wq:
            return [jnp.concatenate(h, axis=0) for h in heads]
        pad = (jnp.zeros((LANES - len(live) * L, LANES), F32),)
        return [jnp.concatenate(h + pad, axis=0).astype(BF16) for h in heads]

    def softmax(q, k):
        out = []
        for qh, kh in zip(q, k):
            s = jax.lax.dot_general(qh, kh, (((1,), (1,)), ((), ())),
                                    preferred_element_type=F32)
            fill = fill_ref[pl.ds(0, s.shape[0]), :]
            s = jnp.where(fill == 0.0, s * scale, fill)
            p = jnp.exp(s - jnp.max(s, axis=-1, keepdims=True))
            out.append(p * _reciprocal(jnp.sum(p, axis=-1, keepdims=True)))
        return out

    def mix(cols, p, v):
        o = [jax.lax.dot_general(ph, vh, (((1,), (0,)), ((), ())), preferred_element_type=F32)
             for ph, vh in zip(p, v)]
        per = GROUP // n
        o = [join(o[i * per:(i + 1) * per]) for i in range(n)]
        _store_rows(o_ref, [[a[r:r + L] for a in o] for r in range(0, o[0].shape[0], L)],
                   cols=cols)

    def chunk(c):
        return pl.ds(c * bw, bw)

    def attention_out(c, i, live):
        for p, y in zip(live, project(o_ref, wo, live, chunk(c))):
            y, cols = join(y), pl.ds(c * gw, gw)
            mem_ref[p, :, cols] = y[:n_mem]
            rb_ref[i & 3, p, :, cols] = ra_ref[p, :, cols] + y[n_mem:]

    def glu_in(i, live):
        for r in range(0, seg, ROWS):
            x = [rb_ref[(i + 3) & 3, p, pl.ds(r, ROWS), :] for p in live]
            _store_rows(xb_ref, [_split(_layernorm(xp), n) for xp in x], rows=pl.ds(r, ROWS))

    def gate(cols, g, u, live):
        h = [[_sigmoid(a) * b for a, b in zip(gp, up)] for gp, up in zip(g, u)]
        if len(live) == 1:
            h = [[jnp.where(live[0] == p, a, 0.0) for a in h[0]] for p in BOTH]
        _store_rows(hb_ref, h, cols=cols)

    def glu_out(c, i, live):
        cols = pl.ds(c * gw, gw)
        for p, y in zip(live, project(hb_ref, wd, live, chunk(c))):
            y = rb_ref[(i + 2) & 3, p, :, cols] + join(y)
            if p == 0:
                x2_ref[:, cols] = y
            else:
                out_vm[segment(jnp.maximum(i - 5, 0)), cols] = y.astype(out_vm.dtype)

    def run(order, i, live):
        val = {what: [] for what in order}
        for what in order:
            c = len(val[what])
            val[what].append({
                'x': lambda: segments_in(i, live),
                'm': lambda: memories_in(live),
                'q': lambda: heads_of(wq, chunk(c), live),
                'k': lambda: heads_of(wk, chunk(c), live),
                'v': lambda: heads_of(wv, chunk(c), live),
                'S': lambda: softmax(val['q'][c], val['k'][c]),
                'P': lambda: mix(chunk(c), val['S'][c], val['v'][c]),
                'W': lambda: attention_out(c, i, live),
                'h': lambda: glu_in(i, live),
                'g': lambda: project(xb_ref, wg, live, chunk(c)),
                'u': lambda: project(xb_ref, wu, live, chunk(c)),
                'G': lambda: gate(chunk(c), val['g'][c], val['u'][c], live),
                'D': lambda: glu_out(c, i, live),
            }[what]())

    def out_copy(i):
        return pltpu.make_async_copy(out_vm.at[segment(i)], out_hbm.at[segment(i)], out_sem)

    n_d = D // gw
    head = pl.ds(0, 4 * seg)
    tail = pl.ds(4 * seg, S - 4 * seg)
    x_head = pltpu.make_async_copy(x_hbm.at[head], x_vm.at[head], x_sem.at[0])
    x_tail = pltpu.make_async_copy(x_hbm.at[tail], x_vm.at[tail], x_sem.at[1])
    mem_copy = pltpu.make_async_copy(mem0_hbm, mem0_vm, x_sem.at[2])

    qkv = Stream([head_job(s, d) for s, d in
                  ((wq_hbm, wq), (wk_hbm, wk), (wv_hbm, wv))], qkv_stage, qkv_sems)
    proj = Stream([tall_job(wo_hbm, wo)], tall_stage, tall_sems)
    wide = Stream([wide_job(s, d)
                   for s, d in ((wg_hbm, wg), (wu_hbm, wu))], wide_stage, wide_sems)
    down = Stream([tall_job(wd_hbm, wd)], tall_stage, tall_sems)

    def refill(stream, calls):
        return lambda k: stream.start(k * stream.slots // calls, (k + 1) * stream.slots // calls)

    qkv.start()
    x_head.start()
    mem_copy.start()
    for m in range(3):
        qkv.drain(m, refill(proj, qkv.slots))
    x_head.wait()
    mem_copy.wait()
    mem_ref[0] = mem_ref[1] = mem0_vm[...].astype(F32)
    x2_ref[...] = rb_ref[0, 1] = rb_ref[1, 1] = rb_ref[2, 1] = jnp.zeros((seg, D), F32)

    attention = 'qkvS' + 'qkvPS' * (n_a - 1)
    glu = 'guG' * n_b

    def full_step(i, carry):
        run(ORDER or 'mxD' + attention + 'D' * (n_d - 1) + 'Ph' + glu + 'W' * n_d, i, BOTH)
        return carry

    def ragged_step(j, carry):
        lone = (jnp.where(j < 4, 0, 1),)
        i = jnp.where(j < 4, jnp.minimum(j, 2), j - 4 + n_seg)
        phase = lambda cond, order, live: pl.when(cond)(lambda: run(order, i, live))
        attends = (j != 3) & (j < 7)
        pl.when(j >= 4)(lambda: out_copy(i - 6).start())
        phase(attends, LONE or 'mx' + attention[:-5] + 'qkPSvP', lone)
        pl.when(j == 0)(lambda: proj.drain(0, refill(wide, proj.slots)))
        pl.when(j == 1)(lambda: wide.drain(0))

        pl.when(j == 2)(lambda: wide.drain(1, lambda k: down.start() if k == 0 else None))
        pl.when(j == 3)(lambda: down.drain(0, lambda k: x_tail.start() if k == 0 else None))
        phase((j >= 3) & (j < 6), 'D' * n_d, BOTH)
        phase(j >= 6, 'D' * n_d, (1,))
        phase(j == 4, 'h' + glu, BOTH)
        pl.when((j > 1) & (j != 4) & (j < 8))(
            lambda: run('h' + glu, jnp.where(j == 2, 1, i), lone))
        phase(attends, 'W' * n_d, lone)

        @pl.when(j == 3)
        def _():
            x_tail.wait()
            jax.lax.fori_loop(3, n_seg, full_step, 0)
            done = pl.ds(0, (n_seg - 6) * seg)
            pltpu.make_async_copy(out_vm.at[done], out_hbm.at[done], out_sem).start()
        return carry

    jax.lax.fori_loop(0, 9, ragged_step, 0)
    out_copy(n_seg - 1).start()
    pltpu.make_async_copy(out_vm, out_hbm, out_sem).wait()


@functools.partial(jax.jit, static_argnames=("A_seg_len",))
def pallas_interleave_layers__memory_aug_recurrent_mem_tr__glu_gated_glu__prompt_kernel(
    A_x: jax.Array,
    A_mem0: jax.Array,
    A_Wq: jax.Array,
    A_Wk: jax.Array,
    A_Wv: jax.Array,
    A_Wo: jax.Array,
    A_seg_len: int,
    B_x: jax.Array,
    B_w_gate: jax.Array,
    B_w_up: jax.Array,
    B_w_down: jax.Array,
):
    del B_x
    B, S, D = A_x.shape
    _, H, Dh = A_Wq.shape
    M = A_mem0.shape[1]
    F = B_w_gate.shape[1]
    seg = int(A_seg_len)
    assert B == 1 and Dh == LANES and S % seg == 0 and S // seg >= 8
    n = len(OFFSETS)
    R = (3 * n * n + n) // 2
    L = M + seg

    def packed(k, cols):
        return pltpu.VMEM((R, k // n // 2, cols // n), WORD)

    hbm = pl.BlockSpec(memory_space=pl.ANY)
    out = pl.pallas_call(
        functools.partial(_kernel, seg=seg, n_mem=M, n_heads=H),
        out_shape=jax.ShapeDtypeStruct((S, D), A_x.dtype),
        in_specs=[hbm] * 9,
        out_specs=hbm,
        scratch_shapes=[
            pltpu.VMEM((S, D), A_x.dtype),
            pltpu.VMEM((S, D), A_x.dtype),
            packed(D, H * Dh),
            packed(D, H * Dh),
            packed(D, H * Dh),
            packed(H * Dh, D),
            packed(D, F),
            packed(D, F),
            packed(F, D),
            pltpu.VMEM((R, L, D // n), F32),
            pltpu.VMEM((2 * n, L, H * Dh // n), F32),
            pltpu.VMEM((2 * n, seg, D // n), F32),
            pltpu.VMEM((2 * n, seg, F // n), F32),
            pltpu.VMEM((2, M, D), F32),
            pltpu.VMEM((2, seg, D), F32),
            pltpu.VMEM((4, 2, seg, D), F32),
            pltpu.VMEM((seg, D), F32),
            pltpu.VMEM((2 * L, LANES), F32),
            pltpu.VMEM((M, D), A_mem0.dtype),
            pltpu.VMEM((QKV_SLOTS, n, STAGE_ROWS // n * H, Dh), BF16),
            pltpu.VMEM((TALL_SLOTS, GROUP * LANES, D), BF16),
            pltpu.VMEM((WIDE_SLOTS, n, STAGE_ROWS // n, F), BF16),
            pltpu.SemaphoreType.DMA((QKV_SLOTS,)),
            pltpu.SemaphoreType.DMA((TALL_SLOTS,)),
            pltpu.SemaphoreType.DMA((WIDE_SLOTS,)),
            pltpu.SemaphoreType.DMA((3,)),
            pltpu.SemaphoreType.DMA(()),
        ],
        compiler_params=pltpu.CompilerParams(vmem_limit_bytes=124 * 2**20),
    )(
        A_x.reshape(S, D),
        A_mem0.reshape(M, D),
        A_Wq.reshape(n, D // n * H, Dh),
        A_Wk.reshape(n, D // n * H, Dh),
        A_Wv.reshape(n, D // n * H, Dh),
        A_Wo.reshape(H * Dh, D),
        B_w_gate.reshape(n, D // n, F),
        B_w_up.reshape(n, D // n, F),
        B_w_down,
    )
    return out.reshape(B, S, D)
```

```python
import functools

import jax
import jax.numpy as jnp
import jax.experimental.pallas as pl
import jax.experimental.pallas.tpu as pltpu

F32 = jnp.float32
BF16 = jnp.bfloat16
WORD = jnp.uint32
LANES = 128
PACK = 16
LN_EPS = 1e-5
MASK_VALUE = -1000000000.0

T4 = (-1.5, -0.5, 0.5, 1.5)
T8 = (-2.75, -1.25, -0.625, -0.125, 0.125, 0.625, 1.25, 2.75)
TQ, TO, TG, TD = 8, 8, 8, 4
TALL_ROWS = 512
BLOCK = 4
NX = 0
QKV_SLOTS, TALL_SLOTS, WIDE_SLOTS = 3, 6, 4
WIDE_ROWS = 128
ROWS = 16
ORDER = None
LONE = None
STAGE_ROWS = 128


def _layernorm(x):
    m = jnp.mean(x, axis=-1, keepdims=True)
    c = x - m
    v = jnp.mean(c * c, axis=-1, keepdims=True)
    return c * jax.lax.rsqrt(v + LN_EPS)


def _sigmoid(x):
    return 0.5 * jnp.tanh(0.5 * x) + 0.5


def _reciprocal(x):
    r = pl.reciprocal(x, approx=True)
    return r * (2.0 - x * r)


def _times(c, x):
    return x if c == 1 else c * x


def _split(x, n):
    w = x.shape[1] // n
    return [x[:, i * w:(i + 1) * w] for i in range(n)]


def _pairs(n):
    return sorted([(i, j) for j in range(n) for i in range(j)],
                  key=lambda p: (p[1] // BLOCK, p[0] // BLOCK, p[1], p[0]))


def _row_operand(t, r, base, both):
    n = len(t)
    if r < 2 * n:
        return base(r)
    (i, j), kind = _pairs(n)[(r - 2 * n) // 3], (r - 2 * n) % 3
    s = base(n + i) + base(n + j)
    if kind == 0 or not both:
        return s
    d = t[j] - t[i]
    return s + _times(d, base(j)) if kind == 1 else s - _times(d, base(i))


def _pack_rows(even, odd):
    bits = lambda x: jax.lax.bitcast_convert_type(x.astype(BF16).astype(F32), WORD)
    return (bits(even) >> 16) | bits(odd)


def _weight_operands(n, w):
    halves = lambda x: [jax.lax.bitcast_convert_type(y, F32)
                        for y in (x << 16, x & WORD(0xFFFF0000))]
    each = lambda op, x, y: [op(a, b) for a, b in zip(x, y)]
    p = [halves(w(i, i)) for i in range(n)]
    q = list(p)
    for k, (i, j) in enumerate(_pairs(n)):
        ij, ji = w(i, j), w(j, i)
        a, b = halves(ij), halves(ji)
        yield 2 * n + 3 * k, _pack_rows(*each(jnp.add, a, b))
        yield 2 * n + 3 * k + 1, ji
        yield 2 * n + 3 * k + 2, ij
        p[i], p[j] = each(jnp.add, p[i], a), each(jnp.add, p[j], b)
        q[i], q[j] = each(jnp.subtract, q[i], b), each(jnp.subtract, q[j], a)
    for i in range(n):
        yield i, _pack_rows(*p[i])
        yield n + i, _pack_rows(*q[i])


def _paired_matmul(t, product, both):
    n = len(t)
    y1, y2 = [None] * n, [None] * n
    acc = lambda a, b: b if a is None else a + b
    todo = [n - 1] * n
    for k, (i, j) in enumerate(_pairs(n)):
        ti, tj = product(2 * n + 3 * k + 1), product(2 * n + 3 * k + 2)
        y2[i], y2[j] = acc(y2[i], ti), acc(y2[j], tj)
        if both:
            u = _times(1.0 / (t[j] - t[i]), ti + tj - product(2 * n + 3 * k))
            y1[i], y1[j] = acc(y1[i], u), (-u if y1[j] is None else y1[j] - u)
        for m in (i, j):
            todo[m] -= 1
            if todo[m] == 0:
                y2[m] = y2[m] + product(n + m)
                if both:
                    y1[m] = y1[m] + product(m)
                    y2[m] = y2[m] + t[m] * y1[m]
    return (y1 if both else None), y2


def _project(t, rows_ref, w_ref, both, c):
    def stored(r):
        return jnp.concatenate([rows_ref[r, k] for k in range(rows_ref.shape[1])], axis=1)

    def product(r):
        rows = stored(r) if r < rows_ref.shape[0] else _row_operand(t, r, stored, both)
        w = pltpu.bitcast(w_ref[c, r], BF16)
        return jax.lax.dot_general(rows, w, (((1,), (0,)), ((), ())),
                                   preferred_element_type=F32)
    return _paired_matmul(t, product, both)


def _store_rows(t, ref, h, rows):
    n, both = len(t), len(h) == 2
    base = ((list(h[0]) + [b - c * a for c, a, b in zip(t, *h)]) if both
            else [None] * n + list(h[0]))
    for r in range(ref.shape[0]):
        if both or (r >= n and (r < 2 * n or (r - 2 * n) % 3)):
            op = _row_operand(t, r, base.__getitem__, both)
            for k, tile in enumerate(_split(op, ref.shape[1])):
                ref[r, k, rows, :] = tile


def _kernel(x_hbm, mem0_hbm, wq_hbm, wk_hbm, wv_hbm, wo_hbm, wg_hbm, wu_hbm, wd_hbm,
            out_hbm,
            x_vm, out_vm, wq, wk, wv, wo, wgu, wd,
            h_ref, o_ref, xb_ref, hb_ref, mem_ref, ra_ref, rb_ref, x2_ref, fill_ref,
            mem0_vm, qkv_stage, tall_stage, wide_stage,
            qkv_sems, tall_sems, wide_sems, x_sem, out_sem, *, seg, n_mem, n_heads):
    S, D = x_vm.shape
    F = wg_hbm.shape[2]
    n_seg = S // seg
    L = n_mem + seg
    tq, to, tg, td = ({4: T4, 8: T8}[k] for k in (TQ, TO, TG, TD))
    n_a, n_b = n_heads // TQ, 2 * F // LANES // TG
    scale = LANES ** -0.5

    class Stream:
        def __init__(self, jobs, stage, sems):
            self.jobs, self.stage, self.sems = jobs, stage, sems
            self.slots = stage.shape[0]

        def copy(self, m, c, slot):
            return [pltpu.make_async_copy(src, dst, self.sems.at[slot])
                    for src, dst in self.jobs[m][1](c, self.stage.at[slot])]

        def begin(self, m, c, slot):
            for cp in self.copy(m, c, slot):
                cp.start()

        def start(self, first=0, last=None):
            for c in range(first, self.slots if last is None else last):
                self.begin(0, c, c)

        def drain(self, m, refill=None):
            count, _, consume = self.jobs[m]
            first = sum(j[0] for j in self.jobs[:m])

            def body(c, carry):
                slot = (first + c) % self.slots
                for cp in self.copy(m, c, slot):
                    cp.wait()
                consume(c, self.stage.at[slot])
                nxt = c + self.slots
                if self.slots < count:
                    pl.when(nxt < count)(lambda: self.begin(m, nxt, slot))
                if m + 1 < len(self.jobs):
                    pl.when(nxt >= count)(lambda: self.begin(m + 1, nxt - count, slot))
                elif refill:
                    for k in range(self.slots):
                        pl.when(nxt == count + k)(functools.partial(refill, k))
                return carry

            jax.lax.fori_loop(0, count, body, 0)

    def put(dst, n, row, g, block):
        rows = pl.ds(pl.multiple_of(row // 2, PACK // 2), PACK // 2)
        for r, op in _weight_operands(n, block):
            dst[g, r, rows, :] = op

    def head_job(src, dst, n):
        kr, gw = STAGE_ROWS // n, n * LANES

        def consume(c, staged):
            for r in range(0, kr, PACK):
                blocks = [_split(pltpu.bitcast(
                    staged[i, pl.ds(r * n_heads, PACK * n_heads), :]
                    .reshape(PACK, n_heads, LANES).reshape(PACK, n_heads * LANES), WORD),
                    n_heads) for i in range(n)]
                for g in range(n_a):
                    put(dst, n, c * kr + r, g, lambda i, j: blocks[i][g * n + j])
        step = kr * n_heads
        return (D // STAGE_ROWS, lambda c, slot: [
            (src.at[:, pl.ds(pl.multiple_of(c * step, step), step), :], slot)], consume)

    def wide_job(srcs, dst, n):
        kr = WIDE_ROWS // n

        def consume(c, staged):
            for r in range(0, kr, PACK):
                for g in range(n_b):
                    put(dst, n, c * kr + r, g, lambda i, j: pltpu.bitcast(staged[
                        j // (n // 2), i, pl.ds(r, PACK),
                        pl.ds((g * (n // 2) + j % (n // 2)) * LANES, LANES)], WORD))
        return D // WIDE_ROWS, lambda c, slot: [
            (src.at[:, pl.ds(pl.multiple_of(c * kr, kr), kr), :], slot.at[m])
            for m, src in enumerate(srcs)], consume

    def tall_job(src, dst, n):
        kr, gw = TALL_ROWS // n, n * LANES

        def consume(c, staged):
            for r in range(0, kr, PACK):
                for g in range(D // gw):
                    put(dst, n, c * kr + r, g, lambda i, j: pltpu.bitcast(staged[
                        pl.ds(i * kr + r, PACK), pl.ds(g * gw + j * LANES, LANES)], WORD))

        def pieces(c, slot):
            first = c * kr // LANES * gw + c * kr % LANES
            return [(src.at[pl.ds(pl.multiple_of(first + i * LANES, kr), kr), :],
                     slot.at[pl.ds(i * kr, kr), :]) for i in range(n)]
        return src.shape[0] // TALL_ROWS, pieces, consume

    qi = jax.lax.broadcasted_iota(jnp.int32, fill_ref.shape, 0)
    ki = jax.lax.broadcasted_iota(jnp.int32, fill_ref.shape, 1)
    same = ((qi >= L) == (ki >= L)) & (ki < 2 * L)
    visible = (jnp.where(qi >= L, qi - L, qi) < n_mem) | (qi >= ki)
    fill_ref[...] = jnp.where(same, jnp.where(visible, 0.0, MASK_VALUE), -jnp.inf)

    BOTH = (0, 1)
    join = lambda blocks: jnp.concatenate(blocks, axis=1)

    def project(t, rows_ref, w_ref, live, c):
        return _project(t, rows_ref, w_ref, len(live) == 2, c)[-len(live):]

    def segment(i, start=0, size=seg):
        return pl.ds(pl.multiple_of(i * seg + start, size), size)

    def segments_in(i, live):
        for r in range(0, seg, ROWS):
            x = [x_vm[segment(jnp.minimum(i, n_seg - 1), r, ROWS), :].astype(F32),
                 x2_ref[pl.ds(r, ROWS), :]]
            if len(live) == 1:
                x = [jnp.where(live[0] == 0, *x)]
            for p, xp in zip(live, x):
                ra_ref[p, pl.ds(r, ROWS), :] = xp
            _store_rows(tq, h_ref, [_split(_layernorm(xp), TQ) for xp in x],
                       rows=pl.ds(n_mem + r, ROWS))

    def memories_in(live):
        _store_rows(tq, h_ref, [_split(mem_ref[p], TQ) for p in live], rows=pl.ds(0, n_mem))

    def heads_of(w, cols, live):
        heads = zip(*project(tq, h_ref, w, live, cols))
        if w is wq:
            return [jnp.concatenate(h, axis=0) for h in heads]
        pad = (jnp.zeros((LANES - len(live) * L, LANES), F32),)
        return [jnp.concatenate(h + pad, axis=0).astype(BF16) for h in heads]

    def softmax(q, k):
        out = []
        for qh, kh in zip(q, k):
            s = jax.lax.dot_general(qh, kh, (((1,), (1,)), ((), ())),
                                    preferred_element_type=F32)
            fill = fill_ref[pl.ds(0, s.shape[0]), :]
            s = jnp.where(fill == 0.0, s * scale, fill)
            p = jnp.exp(s - jnp.max(s, axis=-1, keepdims=True))
            out.append(p * _reciprocal(jnp.sum(p, axis=-1, keepdims=True)))
        return out

    def mix(cols, p, v):
        o = [jax.lax.dot_general(ph, vh, (((1,), (0,)), ((), ())), preferred_element_type=F32)
             for ph, vh in zip(p, v)]
        put_blocks(to, o_ref, cols * TQ, [[a[r:r + L] for a in o]
                                          for r in range(0, o[0].shape[0], L)])

    def put_blocks(t, ref, first, h):
        n = len(t)
        for k, tiles in enumerate(zip(*h)):
            col, i = divmod(first + k, n)
            if len(tiles) == 2:
                ref[i, col] = tiles[0]
            ref[n + i, col] = tiles[1] - t[i] * tiles[0] if len(tiles) == 2 else tiles[0]

    chunk = lambda c: c

    def attention_out(c, i, live):
        for p, y in zip(live, project(to, o_ref, wo, live, c)):
            y, cols = join(y), pl.ds(c * TO * LANES, TO * LANES)
            mem_ref[p, :, cols] = y[:n_mem]
            rb_ref[i & 3, p, :, cols] = ra_ref[p, :, cols] + y[n_mem:]

    def glu_in(i, live):
        for r in range(0, seg, ROWS):
            x = [rb_ref[(i + 3) & 3, p, pl.ds(r, ROWS), :] for p in live]
            _store_rows(tg, xb_ref, [_split(_layernorm(xp), TG) for xp in x], rows=pl.ds(r, ROWS))

    def gate(cols, g, live):
        h = [[_sigmoid(a) * b for a, b in zip(y[:TG // 2], y[TG // 2:])] for y in g]
        if len(live) == 1:
            h = [[jnp.where(live[0] == p, a, 0.0) for a in h[0]] for p in BOTH]
        put_blocks(td, hb_ref, cols * TG // 2, h)

    def glu_out(c, i, live):
        cols = pl.ds(c * TD * LANES, TD * LANES)
        for p, y in zip(live, project(td, hb_ref, wd, live, chunk(c))):
            y = rb_ref[(i + 2) & 3, p, :, cols] + join(y)
            if p == 0:
                x2_ref[:, cols] = y
            else:
                out_vm[segment(jnp.maximum(i - 5, 0)), cols] = y.astype(out_vm.dtype)

    def run(order, i, live):
        val = {what: [] for what in order}
        for what in order:
            c = len(val[what])
            val[what].append({
                'x': lambda: segments_in(i, live),
                'm': lambda: memories_in(live),
                'q': lambda: heads_of(wq, chunk(c), live),
                'k': lambda: heads_of(wk, chunk(c), live),
                'v': lambda: heads_of(wv, chunk(c), live),
                'S': lambda: softmax(val['q'][c], val['k'][c]),
                'P': lambda: mix(chunk(c), val['S'][c], val['v'][c]),
                'W': lambda: attention_out(c, i, live),
                'h': lambda: glu_in(i, live),
                'g': lambda: project(tg, xb_ref, wgu, live, chunk(c)),
                'G': lambda: gate(chunk(c), val['g'][c], live),
                'D': lambda: glu_out(c, i, live),
            }[what]())

    def out_copy(i):
        return pltpu.make_async_copy(out_vm.at[segment(i)], out_hbm.at[segment(i)], out_sem)

    n_d, n_w = D // LANES // TD, D // LANES // TO
    head = pl.ds(0, 4 * seg)
    tail = pl.ds(4 * seg, S - 4 * seg)
    x_head = pltpu.make_async_copy(x_hbm.at[head], x_vm.at[head], x_sem.at[0])
    x_tail = pltpu.make_async_copy(x_hbm.at[tail], x_vm.at[tail], x_sem.at[1])
    mem_copy = pltpu.make_async_copy(mem0_hbm, mem0_vm, x_sem.at[2])

    qkv = Stream([head_job(s, d, TQ) for s, d in
                  ((wq_hbm, wq), (wk_hbm, wk), (wv_hbm, wv))], qkv_stage, qkv_sems)
    proj = Stream([tall_job(wo_hbm, wo, TO)], tall_stage, tall_sems)
    count, pieces, consume = wide_job((wg_hbm, wu_hbm), wgu, TG)
    shift = lambda f: lambda c, slot: f(c + count // 2, slot)
    wide = Stream([(count // 2, pieces, consume),
                   (count // 2, shift(pieces), shift(consume))], wide_stage, wide_sems)
    down = Stream([tall_job(wd_hbm, wd, TD)], tall_stage, tall_sems)

    def refill(stream, calls):
        return lambda k: stream.start(k * stream.slots // calls, (k + 1) * stream.slots // calls)

    qkv.start()
    x_head.start()
    mem_copy.start()
    for m in range(3):
        qkv.drain(m, refill(proj, qkv.slots))
    x_head.wait()
    mem_copy.wait()
    mem_ref[0] = mem_ref[1] = mem0_vm[...].astype(F32)
    x2_ref[...] = rb_ref[0, 1] = rb_ref[1, 1] = rb_ref[2, 1] = jnp.zeros((seg, D), F32)

    attention = 'qkvS' + 'qkvPS' * (n_a - 1)
    glu = 'gG' * n_b

    def full_step(i, carry):
        run(ORDER or 'mxD' + attention + 'D' * (n_d - 1) + 'Ph' + glu + 'W' * n_w, i, BOTH)
        return carry

    def ragged_step(j, carry):
        lone = (jnp.where(j < 4, 0, 1),)
        i = jnp.where(j < 4, jnp.minimum(j, 2), j - 4 + n_seg)
        phase = lambda cond, order, live: pl.when(cond)(lambda: run(order, i, live))
        attends = (j != 3) & (j < 7)
        pl.when(j >= 4)(lambda: out_copy(i - 6).start())
        phase(attends, LONE or 'mx' + attention[:-5] + 'qkPSvP', lone)
        pl.when(j == 0)(lambda: proj.drain(0, refill(wide, proj.slots)))
        pl.when(j == 1)(lambda: wide.drain(0))

        pl.when(j == 2)(lambda: wide.drain(1, lambda k: down.start() if k == 0 else None))
        pl.when(j == 3)(lambda: down.drain(0, lambda k: x_tail.start() if k == 0 else None))
        phase((j >= 3) & (j < 6), 'D' * n_d, BOTH)
        phase(j >= 6, 'D' * n_d, (1,))
        phase(j == 4, 'h' + glu, BOTH)
        pl.when((j > 1) & (j != 4) & (j < 8))(
            lambda: run('h' + glu, jnp.where(j == 2, 1, i), lone))
        phase(attends, 'W' * n_w, lone)

        @pl.when(j == 3)
        def _():
            x_tail.wait()
            jax.lax.fori_loop(3, n_seg, full_step, 0)
            done = pl.ds(0, (n_seg - 6) * seg)
            pltpu.make_async_copy(out_vm.at[done], out_hbm.at[done], out_sem).start()
        return carry

    jax.lax.fori_loop(0, 9, ragged_step, 0)
    out_copy(n_seg - 1).start()
    pltpu.make_async_copy(out_vm, out_hbm, out_sem).wait()


@functools.partial(jax.jit, static_argnames=("A_seg_len",))
def pallas_interleave_layers__memory_aug_recurrent_mem_tr__glu_gated_glu__prompt_kernel(
    A_x: jax.Array,
    A_mem0: jax.Array,
    A_Wq: jax.Array,
    A_Wk: jax.Array,
    A_Wv: jax.Array,
    A_Wo: jax.Array,
    A_seg_len: int,
    B_x: jax.Array,
    B_w_gate: jax.Array,
    B_w_up: jax.Array,
    B_w_down: jax.Array,
):
    del B_x
    B, S, D = A_x.shape
    _, H, Dh = A_Wq.shape
    M = A_mem0.shape[1]
    F = B_w_gate.shape[1]
    seg = int(A_seg_len)
    assert B == 1 and Dh == LANES and S % seg == 0 and S // seg >= 8
    R = lambda n: (3 * n * n + n) // 2
    L = M + seg

    def packed(n, k, cols):
        return pltpu.VMEM((cols // n // LANES, R(n), k // n // 2, LANES), WORD)

    def rows(count, m, k):
        return pltpu.VMEM((count, k // LANES, m, LANES), F32)

    hbm = pl.BlockSpec(memory_space=pl.ANY)
    out = pl.pallas_call(
        functools.partial(_kernel, seg=seg, n_mem=M, n_heads=H),
        out_shape=jax.ShapeDtypeStruct((S, D), A_x.dtype),
        in_specs=[hbm] * 9,
        out_specs=hbm,
        scratch_shapes=[
            pltpu.VMEM((S, D), A_x.dtype),
            pltpu.VMEM((S, D), A_x.dtype),
            packed(TQ, D, H * Dh),
            packed(TQ, D, H * Dh),
            packed(TQ, D, H * Dh),
            packed(TO, H * Dh, D),
            packed(TG, D, 2 * F),
            packed(TD, F, D),
            rows(R(TQ), L, D // TQ),
            rows(2 * TO, L, H * Dh // TO),
            rows(NX or 2 * TG, seg, D // TG),
            rows(2 * TD, seg, F // TD),
            pltpu.VMEM((2, M, D), F32),
            pltpu.VMEM((2, seg, D), F32),
            pltpu.VMEM((4, 2, seg, D), F32),
            pltpu.VMEM((seg, D), F32),
            pltpu.VMEM((2 * L, LANES), F32),
            pltpu.VMEM((M, D), A_mem0.dtype),
            pltpu.VMEM((QKV_SLOTS, TQ, STAGE_ROWS // TQ * H, Dh), BF16),
            pltpu.VMEM((TALL_SLOTS, TALL_ROWS, D), BF16),
            pltpu.VMEM((WIDE_SLOTS, 2, TG, WIDE_ROWS // TG, F), BF16),
            pltpu.SemaphoreType.DMA((QKV_SLOTS,)),
            pltpu.SemaphoreType.DMA((TALL_SLOTS,)),
            pltpu.SemaphoreType.DMA((WIDE_SLOTS,)),
            pltpu.SemaphoreType.DMA((3,)),
            pltpu.SemaphoreType.DMA(()),
        ],
        compiler_params=pltpu.CompilerParams(vmem_limit_bytes=124 * 2**20),
    )(
        A_x.reshape(S, D),
        A_mem0.reshape(M, D),
        A_Wq.reshape(TQ, D // TQ * H, Dh),
        A_Wk.reshape(TQ, D // TQ * H, Dh),
        A_Wv.reshape(TQ, D // TQ * H, Dh),
        A_Wo.reshape(H * Dh, D),
        B_w_gate.reshape(TG, D // TG, F),
        B_w_up.reshape(TG, D // TG, F),
        B_w_down,
    )
    return out.reshape(B, S, D)
```

```python
import functools

import jax
import jax.numpy as jnp
import jax.experimental.pallas as pl
import jax.experimental.pallas.tpu as pltpu

F32 = jnp.float32
BF16 = jnp.bfloat16
WORD = jnp.uint32
LANES = 128
PACK = 16
LN_EPS = 1e-5
MASK_VALUE = -1000000000.0

T8 = (-2.9, -1.4, -0.7, -0.215, 0.215, 0.7, 1.4, 2.9)
T4 = (-1.8, -0.43, 0.43, 1.8)

TALL_ROWS = 512
QKV_SLOTS, TALL_SLOTS, WIDE_SLOTS = 3, 6, 4
ROWS = 16


def _layernorm(x):
    c = x - jnp.mean(x, axis=-1, keepdims=True)
    return c * jax.lax.rsqrt(jnp.mean(c * c, axis=-1, keepdims=True) + LN_EPS)


def _sigmoid(x):
    return 0.5 * jnp.tanh(0.5 * x) + 0.5


def _reciprocal(x):
    r = pl.reciprocal(x, approx=True)
    return r * (2.0 - x * r)


def _dot(a, b, b_axis=0):
    return jax.lax.dot_general(a, b, (((1,), (b_axis,)), ((), ())), preferred_element_type=F32)


def _split(x, n):
    w = x.shape[1] // n
    return [x[:, i * w:(i + 1) * w] for i in range(n)]


def _join(blocks):
    return jnp.concatenate(blocks, axis=1)


def _pairs(n):
    return sorted(((i, j) for j in range(n) for i in range(j)),
                  key=lambda p: (p[1] // 4, p[0] // 4, p[1], p[0]))


def _n_products(n):
    return (3 * n * n + n) // 2


def _weight_operands(n, w):
    def rows(x):
        return [jax.lax.bitcast_convert_type(y, F32) for y in (x << 16, x & WORD(0xFFFF0000))]

    def words(x):
        even, odd = (jax.lax.bitcast_convert_type(y.astype(BF16).astype(F32), WORD) for y in x)
        return (even >> 16) | odd

    add = lambda x, y: [a + b for a, b in zip(x, y)]
    sub = lambda x, y: [a - b for a, b in zip(x, y)]
    p = [rows(w(i, i)) for i in range(n)]
    q = list(p)
    for k, (i, j) in enumerate(_pairs(n)):
        ij, ji = w(i, j), w(j, i)
        a, b = rows(ij), rows(ji)
        yield 2 * n + 3 * k, words(add(a, b))
        yield 2 * n + 3 * k + 1, ji
        yield 2 * n + 3 * k + 2, ij
        p[i], p[j], q[i], q[j] = add(p[i], a), add(p[j], b), sub(q[i], b), sub(q[j], a)
    for i in range(n):
        yield i, words(p[i])
        yield n + i, words(q[i])


def _row_operand(t, r, base, both):
    n = len(t)
    if r < 2 * n:
        return base(r)
    (i, j), kind = _pairs(n)[(r - 2 * n) // 3], (r - 2 * n) % 3
    s = base(n + i) + base(n + j)
    if kind == 0 or not both:
        return s
    return s + (t[j] - t[i]) * base(j) if kind == 1 else s - (t[j] - t[i]) * base(i)


def _store_rows(t, ref, h, rows):
    n, both = len(t), len(h) == 2
    h = [_split(x, n) for x in h]
    base = (h[0] + [b - c * a for c, a, b in zip(t, *h)]) if both else [None] * n + h[0]
    for r in range(ref.shape[0]):
        if both or (r >= n and (r < 2 * n or (r - 2 * n) % 3)):
            op = _row_operand(t, r, base.__getitem__, both)
            for k, tile in enumerate(_split(op, ref.shape[1])):
                ref[r, k, rows, :] = tile


def _store_tiles(t, ref, first, h):
    for x, tiles in enumerate(zip(*h), first):
        k, i = divmod(x, len(t))
        if len(tiles) == 2:
            ref[i, k] = tiles[0]
            ref[len(t) + i, k] = tiles[1] - t[i] * tiles[0]
        else:
            ref[len(t) + i, k] = tiles[0]


def _project(t, rows_ref, w_ref, group, both):
    n = len(t)

    def stored(r):
        return _join([rows_ref[r, k] for k in range(rows_ref.shape[1])])

    def product(r):
        rows = stored(r) if r < rows_ref.shape[0] else _row_operand(t, r, stored, both)
        return _dot(rows, pltpu.bitcast(w_ref[group, r], BF16))

    y1, y2 = [None] * n, [None] * n
    acc = lambda a, b: b if a is None else a + b
    todo = [n - 1] * n
    for k, (i, j) in enumerate(_pairs(n)):
        ti, tj = product(2 * n + 3 * k + 1), product(2 * n + 3 * k + 2)
        y2[i], y2[j] = acc(y2[i], ti), acc(y2[j], tj)
        if both:
            u = (1.0 / (t[j] - t[i])) * (ti + tj - product(2 * n + 3 * k))
            y1[i], y1[j] = acc(y1[i], u), (-u if y1[j] is None else y1[j] - u)
        for m in (i, j):
            todo[m] -= 1
            if todo[m] == 0:
                y2[m] = y2[m] + product(n + m)
                if both:
                    y1[m] = y1[m] + product(m)
                    y2[m] = y2[m] + t[m] * y1[m]
    return (y1, y2) if both else (y2,)


class _Stream:
    def __init__(self, jobs, stage, sems):
        self.jobs, self.stage, self.sems = jobs, stage, sems
        self.slots = stage.shape[0]
        assert all(job[0] >= self.slots for job in jobs)

    def copies(self, m, c, slot):
        return [pltpu.make_async_copy(src, dst, self.sems.at[slot])
                for src, dst in self.jobs[m][1](c, self.stage.at[slot])]

    def fetch(self, m, c, slot):
        for copy in self.copies(m, c, slot):
            copy.start()

    def start(self, part=0, parts=1):
        for c in range(part * self.slots // parts, (part + 1) * self.slots // parts):
            self.fetch(0, c, c)

    def drain(self, m, idle=None):
        count, _, consume = self.jobs[m]
        first = sum(job[0] for job in self.jobs[:m])

        @pl.loop(0, count)
        def _(c):
            slot = (first + c) % self.slots
            for copy in self.copies(m, c, slot):
                copy.wait()
            consume(c, self.stage.at[slot])
            nxt = c + self.slots
            if self.slots < count:
                pl.when(nxt < count)(lambda: self.fetch(m, nxt, slot))
            if m + 1 < len(self.jobs):
                pl.when(nxt >= count)(lambda: self.fetch(m + 1, nxt - count, slot))
            elif idle:
                for k in range(self.slots):
                    pl.when(nxt == count + k)(functools.partial(idle, k))


def _put(dst, n, row, group, block):
    rows = pl.ds(pl.multiple_of(row // 2, PACK // 2), PACK // 2)
    for r, op in _weight_operands(n, block):
        dst[group, r, rows, :] = op


def _head_job(src, dst, n):
    step = PACK * n * dst.shape[0]

    def consume(c, staged):
        heads = [_split(pltpu.bitcast(
            staged[i].reshape(PACK, step // PACK, LANES).reshape(PACK, step // PACK * LANES),
            WORD), step // PACK) for i in range(n)]
        for g in range(dst.shape[0]):
            _put(dst, n, c * PACK, g, lambda i, j: heads[i][g * n + j])

    return (src.shape[1] // step,
            lambda c, slot: [(src.at[:, pl.ds(pl.multiple_of(c * step, step), step), :], slot)],
            consume)


def _wide_job(srcs, dst, n, first, count):
    def consume(c, staged):
        @pl.loop(0, dst.shape[0])
        def _(g):
            lanes = lambda j: pl.ds(pl.multiple_of((g * (n // 2) + j) * LANES, LANES), LANES)
            _put(dst, n, (first + c) * PACK, g, lambda i, j: pltpu.bitcast(
                staged[j // (n // 2), i, :, lanes(j % (n // 2))], WORD))

    def pieces(c, slot):
        rows = pl.ds(pl.multiple_of((first + c) * PACK, PACK), PACK)
        return [(src.at[:, rows, :], slot.at[m]) for m, src in enumerate(srcs)]

    return count, pieces, consume


def _tall_job(src, dst, n):
    kr = TALL_ROWS // n
    step = PACK * 64 // (n * n)

    def consume(c, staged):
        @pl.loop(0, kr, step=step)
        def _(r0):
            for r in range(0, step, PACK):
                for g in range(dst.shape[0]):
                    _put(dst, n, c * kr + r0 + r, g, lambda i, j: pltpu.bitcast(staged[
                        pl.ds(pl.multiple_of(i * kr + r0 + r, PACK), PACK),
                        pl.ds((g * n + j) * LANES, LANES)], WORD))

    def pieces(c, slot):
        first = c * kr // LANES * n * LANES + c * kr % LANES
        return [(src.at[pl.ds(pl.multiple_of(first + i * LANES, kr), kr), :],
                 slot.at[pl.ds(i * kr, kr), :]) for i in range(n)]

    return src.shape[0] // TALL_ROWS, pieces, consume


def _kernel(x_hbm, mem0_hbm, wq_hbm, wk_hbm, wv_hbm, wo_hbm, wg_hbm, wu_hbm, wd_hbm,
            out_hbm,
            x_vm, out_vm, mem0_vm, wq, wk, wv, wo, wgu, wd,
            h_ref, o_ref, xb_ref, hb_ref, mem_ref, ra_ref, rb_ref, x2_ref, fill_ref,
            qkv_stage, tall_stage, wide_stage,
            qkv_sems, tall_sems, wide_sems, in_sems, out_sem):
    S = x_vm.shape[0]
    n_mem, seg = mem_ref.shape[1], x2_ref.shape[0]
    n_seg = S // seg
    L = n_mem + seg
    scale = LANES ** -0.5

    qi = jax.lax.broadcasted_iota(jnp.int32, fill_ref.shape, 0)
    ki = jax.lax.broadcasted_iota(jnp.int32, fill_ref.shape, 1)
    same = ((qi >= L) == (ki >= L)) & (ki < 2 * L)
    visible = (jnp.where(qi >= L, qi - L, qi) < n_mem) | (qi >= ki)
    fill_ref[...] = jnp.where(same, jnp.where(visible, 0.0, MASK_VALUE), -jnp.inf)

    BOTH = (0, 1)

    def segment(i, start=0, size=seg):
        return pl.ds(pl.multiple_of(i * seg + start, size), size)

    def segments_in(i, live):
        for r in range(0, seg, ROWS):
            x = [x_vm[segment(jnp.minimum(i, n_seg - 1), r, ROWS), :].astype(F32),
                 x2_ref[pl.ds(r, ROWS), :]]
            if len(live) == 1:
                x = [jnp.where(live[0] == 0, *x)]
            for p, xp in zip(live, x):
                ra_ref[p, pl.ds(r, ROWS), :] = xp
            _store_rows(T8, h_ref, [_layernorm(xp) for xp in x], pl.ds(n_mem + r, ROWS))

    def memories_in(live):
        _store_rows(T8, h_ref, [mem_ref[p] for p in live], pl.ds(0, n_mem))

    def heads(w, c, live):
        y = zip(*_project(T8, h_ref, w, c, len(live) == 2))
        if w is wq:
            return [jnp.concatenate(h, axis=0) for h in y]
        pad = (jnp.zeros((LANES - len(live) * L, LANES), F32),)
        return [jnp.concatenate(h + pad, axis=0).astype(BF16) for h in y]

    def softmax(q, k):
        out = []
        for qh, kh in zip(q, k):
            s = _dot(qh, kh, 1)
            fill = fill_ref[pl.ds(0, s.shape[0]), :]
            s = jnp.where(fill == 0.0, s * scale, fill)
            p = jnp.exp(s - jnp.max(s, axis=-1, keepdims=True))
            out.append(p * _reciprocal(jnp.sum(p, axis=-1, keepdims=True)))
        return out

    def mix(c, p, v):
        o = [_dot(ph, vh) for ph, vh in zip(p, v)]
        _store_tiles(T8, o_ref, c * len(o),
                     [[a[r:r + L] for a in o] for r in range(0, o[0].shape[0], L)])

    def attention_out(c, i, live):
        for p, y in zip(live, _project(T8, o_ref, wo, c, len(live) == 2)):
            y = _join(y)
            cols = pl.ds(c * y.shape[1], y.shape[1])
            mem_ref[p, :, cols] = y[:n_mem]
            rb_ref[i & 3, p, :, cols] = ra_ref[p, :, cols] + y[n_mem:]

    def glu_in(i, live):
        for r in range(0, seg, ROWS):
            x = [rb_ref[(i + 3) & 3, p, pl.ds(r, ROWS), :] for p in live]
            _store_rows(T8, xb_ref, [_layernorm(xp) for xp in x], pl.ds(r, ROWS))

    def gate(c, live):
        half = len(T8) // 2
        h = [[_sigmoid(g) * u for g, u in zip(y[:half], y[half:])]
             for y in _project(T8, xb_ref, wgu, c, len(live) == 2)]
        if len(live) == 1:
            h = [[jnp.where(live[0] == p, a, 0.0) for a in h[0]] for p in BOTH]
        _store_tiles(T4, hb_ref, c * half, h)

    def glu_out(c, i, live):
        for p, y in zip(live, _project(T4, hb_ref, wd, c, len(live) == 2)):
            y = _join(y)
            cols = pl.ds(c * y.shape[1], y.shape[1])
            y = rb_ref[(i + 2) & 3, p, :, cols] + y
            if p == 0:
                x2_ref[:, cols] = y
            else:
                out_vm[segment(jnp.maximum(i - 5, 0)), cols] = y.astype(out_vm.dtype)

    def run(order, i, live):
        val = {what: [] for what in order}
        for what in order:
            c = len(val[what])
            val[what].append({
                'x': lambda: segments_in(i, live),
                'm': lambda: memories_in(live),
                'q': lambda: heads(wq, c, live),
                'k': lambda: heads(wk, c, live),
                'v': lambda: heads(wv, c, live),
                'S': lambda: softmax(val['q'][c], val['k'][c]),
                'P': lambda: mix(c, val['S'][c], val['v'][c]),
                'W': lambda: attention_out(c, i, live),
                'h': lambda: glu_in(i, live),
                'G': lambda: gate(c, live),
                'D': lambda: glu_out(c, i, live),
            }[what]())

    def out_copy(rows):
        return pltpu.make_async_copy(out_vm.at[rows], out_hbm.at[rows], out_sem)

    head, tail = pl.ds(0, 3 * seg), pl.ds(3 * seg, S - 3 * seg)
    x_head = pltpu.make_async_copy(x_hbm.at[head], x_vm.at[head], in_sems.at[0])
    x_tail = pltpu.make_async_copy(x_hbm.at[tail], x_vm.at[tail], in_sems.at[1])
    mem_copy = pltpu.make_async_copy(mem0_hbm, mem0_vm, in_sems.at[2])
    half = wg_hbm.shape[1] // PACK // 2
    qkv = _Stream([_head_job(s, d, len(T8)) for s, d in
                   ((wq_hbm, wq), (wk_hbm, wk), (wv_hbm, wv))], qkv_stage, qkv_sems)
    proj = _Stream([_tall_job(wo_hbm, wo, len(T8))], tall_stage, tall_sems)
    wide = _Stream([_wide_job((wg_hbm, wu_hbm), wgu, len(T8), first, half)
                    for first in (0, half)], wide_stage, wide_sems)
    down = _Stream([_tall_job(wd_hbm, wd, len(T4))], tall_stage, tall_sems)

    qkv.start()
    x_head.start()
    mem_copy.start()
    for m in range(3):
        qkv.drain(m, lambda k: proj.start(k, qkv.slots))
    x_head.wait()
    mem_copy.wait()
    mem_ref[0] = mem_ref[1] = mem0_vm[...].astype(F32)
    x2_ref[...] = rb_ref[1, 1] = rb_ref[2, 1] = rb_ref[0, 1] = jnp.zeros(x2_ref.shape, F32)

    attention = 'qkvS' + 'qkvPS' * (wq.shape[0] - 1)
    lone_attention = 'mx' + (attention[:-5] + 'qkPSvP' if wq.shape[0] > 1 else 'qkSvP')
    glu, glu_down, attn_out = 'h' + 'G' * wgu.shape[0], 'D' * wd.shape[0], 'W' * wo.shape[0]

    @pl.loop(0, 9)
    def _(j):
        lone = (jnp.where(j < 4, 0, 1),)
        i = jnp.where(j < 4, jnp.minimum(j, 2), j - 4 + n_seg)
        phase = lambda cond, order, live, i=i: pl.when(cond)(lambda: run(order, i, live))
        attends = (j != 3) & (j < 7)

        pl.when(j >= 4)(lambda: out_copy(segment(i - 6)).start())
        phase(attends, lone_attention, lone)
        pl.when(j == 0)(lambda: proj.drain(0, lambda k: wide.start(k, proj.slots)))
        pl.when(j == 1)(lambda: wide.drain(0))
        pl.when(j == 2)(lambda: wide.drain(1, lambda k: down.start() if k == 0 else None))
        pl.when(j == 3)(lambda: down.drain(0, lambda k: x_tail.start() if k == 0 else None))
        phase((j >= 3) & (j < 6), glu_down, BOTH)
        phase(j >= 6, glu_down, (1,))
        phase(j == 4, glu, BOTH)
        phase((j > 1) & (j != 4) & (j < 8), glu, lone, jnp.where(j == 2, 1, i))
        phase(attends, attn_out, lone)

        @pl.when(j == 3)
        def _():
            x_tail.wait()
            pl.loop(3, n_seg)(lambda step: run(
                'mxD' + attention + glu_down[1:] + 'P' + glu + attn_out, step, BOTH))
            out_copy(pl.ds(0, (n_seg - 6) * seg)).start()

    out_copy(segment(n_seg - 1)).start()
    pltpu.make_async_copy(out_vm, out_hbm, out_sem).wait()


@functools.partial(jax.jit, static_argnames=("A_seg_len",))
def pallas_interleave_layers__memory_aug_recurrent_mem_tr__glu_gated_glu__prompt_kernel(
    A_x: jax.Array,
    A_mem0: jax.Array,
    A_Wq: jax.Array,
    A_Wk: jax.Array,
    A_Wv: jax.Array,
    A_Wo: jax.Array,
    A_seg_len: int,
    B_x: jax.Array,
    B_w_gate: jax.Array,
    B_w_up: jax.Array,
    B_w_down: jax.Array,
):
    del B_x
    B, S, D = A_x.shape
    _, H, Dh = A_Wq.shape
    M = A_mem0.shape[1]
    F = B_w_gate.shape[1]
    seg = int(A_seg_len)
    L = M + seg
    n8, n4 = len(T8), len(T4)
    assert B == 1 and Dh == LANES and 2 * L < LANES and S % seg == 0 and S // seg > 6
    assert D % (n8 * LANES) == 0 and H % n8 == 0 and F % (n4 * LANES) == 0

    def weights(n, k, cols):
        return pltpu.VMEM((cols // n // LANES, _n_products(n), k // n // 2, LANES), WORD)

    def rows(count, m, k):
        return pltpu.VMEM((count, k // LANES, m, LANES), F32)

    hbm = pl.BlockSpec(memory_space=pl.ANY)
    out = pl.pallas_call(
        _kernel,
        out_shape=jax.ShapeDtypeStruct((S, D), A_x.dtype),
        in_specs=[hbm] * 9,
        out_specs=hbm,
        scratch_shapes=[
            pltpu.VMEM((S, D), A_x.dtype),
            pltpu.VMEM((S, D), A_x.dtype),
            pltpu.VMEM((M, D), A_mem0.dtype),
            weights(n8, D, H * Dh),
            weights(n8, D, H * Dh),
            weights(n8, D, H * Dh),
            weights(n8, H * Dh, D),
            weights(n8, D, 2 * F),
            weights(n4, F, D),
            rows(_n_products(n8), L, D // n8),
            rows(2 * n8, L, H * Dh // n8),
            rows(2 * n8, seg, D // n8),
            rows(2 * n4, seg, F // n4),
            pltpu.VMEM((2, M, D), F32),
            pltpu.VMEM((2, seg, D), F32),
            pltpu.VMEM((4, 2, seg, D), F32),
            pltpu.VMEM((seg, D), F32),
            pltpu.VMEM((2 * L, LANES), F32),
            pltpu.VMEM((QKV_SLOTS, n8, PACK * H, Dh), BF16),
            pltpu.VMEM((TALL_SLOTS, TALL_ROWS, D), BF16),
            pltpu.VMEM((WIDE_SLOTS, 2, n8, PACK, F), BF16),
            pltpu.SemaphoreType.DMA((QKV_SLOTS,)),
            pltpu.SemaphoreType.DMA((TALL_SLOTS,)),
            pltpu.SemaphoreType.DMA((WIDE_SLOTS,)),
            pltpu.SemaphoreType.DMA((3,)),
            pltpu.SemaphoreType.DMA(()),
        ],
        compiler_params=pltpu.CompilerParams(vmem_limit_bytes=124 * 2**20),
    )(
        A_x.reshape(S, D),
        A_mem0.reshape(M, D),
        A_Wq.reshape(n8, D // n8 * H, Dh),
        A_Wk.reshape(n8, D // n8 * H, Dh),
        A_Wv.reshape(n8, D // n8 * H, Dh),
        A_Wo.reshape(H * Dh, D),
        B_w_gate.reshape(n8, D // n8, F),
        B_w_up.reshape(n8, D // n8, F),
        B_w_down,
    )
    return out.reshape(B, S, D)
```

```python
import functools

import jax
import jax.numpy as jnp
import jax.experimental.pallas as pl
import jax.experimental.pallas.tpu as pltpu

F32 = jnp.float32
BF16 = jnp.bfloat16
WORD = jnp.uint32
LANES = 128
PACK = 16
LN_EPS = 1e-5
MASK_VALUE = -1000000000.0
LOG2_E = 1.4426950408889634

T8 = (-2.9, -1.4, -0.7, -0.215, 0.215, 0.7, 1.4, 2.9)
T4 = (-1.8, -0.43, 0.43, 1.8)

TALL_ROWS = 64
QKV_SLOTS, TALL_SLOTS, WIDE_SLOTS = 3, 6, 4
ROWS = 16


def _layernorm(x):
    c = x - jnp.mean(x, axis=-1, keepdims=True)
    return c * jax.lax.rsqrt(jnp.mean(c * c, axis=-1, keepdims=True) + LN_EPS)


def _sigmoid(x):
    return 0.5 * jnp.tanh(0.5 * x) + 0.5


def _reciprocal(x):
    r = pl.reciprocal(x, approx=True)
    return r * (2.0 - x * r)


def _dot(a, b, b_axis=0):
    return jax.lax.dot_general(a, b, (((1,), (b_axis,)), ((), ())), preferred_element_type=F32)


def _split(x, n):
    w = x.shape[1] // n
    return [x[:, i * w:(i + 1) * w] for i in range(n)]


def _join(blocks):
    return jnp.concatenate(blocks, axis=1)


def _pairs(n):
    return sorted(((i, j) for j in range(n) for i in range(j)),
                  key=lambda p: (p[1] // 4, p[0] // 4, p[1], p[0]))


def _n_products(n):
    return (3 * n * n + n) // 2


def _weight_operands(n, w):
    def rows(x):
        return [jax.lax.bitcast_convert_type(y, F32) for y in (x << 16, x & WORD(0xFFFF0000))]

    def words(x):
        even, odd = (jax.lax.bitcast_convert_type(y.astype(BF16).astype(F32), WORD) for y in x)
        return (even >> 16) | odd

    add = lambda x, y: [a + b for a, b in zip(x, y)]
    sub = lambda x, y: [a - b for a, b in zip(x, y)]
    p = [rows(w(i, i)) for i in range(n)]
    q = list(p)
    for k, (i, j) in enumerate(_pairs(n)):
        ij, ji = w(i, j), w(j, i)
        a, b = rows(ij), rows(ji)
        yield 2 * n + 3 * k, words(add(a, b))
        yield 2 * n + 3 * k + 1, ji
        yield 2 * n + 3 * k + 2, ij
        p[i], p[j], q[i], q[j] = add(p[i], a), add(p[j], b), sub(q[i], b), sub(q[j], a)
    for i in range(n):
        yield i, words(p[i])
        yield n + i, words(q[i])


def _row_operand(t, r, base, both):
    n = len(t)
    if r < 2 * n:
        return base(r)
    (i, j), kind = _pairs(n)[(r - 2 * n) // 3], (r - 2 * n) % 3
    s = base(n + i) + base(n + j)
    if kind == 0 or not both:
        return s
    return s + (t[j] - t[i]) * base(j) if kind == 1 else s - (t[j] - t[i]) * base(i)


def _store_rows(t, ref, h, rows):
    n, both = len(t), len(h) == 2
    h = [_split(x, n) for x in h]
    base = (h[0] + [b - c * a for c, a, b in zip(t, *h)]) if both else [None] * n + h[0]
    for r in range(ref.shape[0]):
        if both or (r >= n and (r < 2 * n or (r - 2 * n) % 3)):
            op = _row_operand(t, r, base.__getitem__, both)
            for k, tile in enumerate(_split(op, ref.shape[1])):
                ref[r, k, rows, :] = tile


def _store_tiles(t, ref, first, h):
    for x, tiles in enumerate(zip(*h), first):
        k, i = divmod(x, len(t))
        if len(tiles) == 2:
            ref[i, k] = tiles[0]
            ref[len(t) + i, k] = tiles[1] - t[i] * tiles[0]
        else:
            ref[len(t) + i, k] = tiles[0]


def _project(t, rows_ref, w_ref, group, both):
    n = len(t)

    def stored(r):
        return _join([rows_ref[r, k] for k in range(rows_ref.shape[1])])

    def product(r):
        rows = stored(r) if r < rows_ref.shape[0] else _row_operand(t, r, stored, both)
        return _dot(rows, pltpu.bitcast(w_ref[group, r], BF16))

    y1, y2 = [None] * n, [None] * n
    acc = lambda a, b: b if a is None else a + b
    todo = [n - 1] * n
    for k, (i, j) in enumerate(_pairs(n)):
        ti, tj = product(2 * n + 3 * k + 1), product(2 * n + 3 * k + 2)
        y2[i], y2[j] = acc(y2[i], ti), acc(y2[j], tj)
        if both:
            u = (1.0 / (t[j] - t[i])) * (ti + tj - product(2 * n + 3 * k))
            y1[i], y1[j] = acc(y1[i], u), (-u if y1[j] is None else y1[j] - u)
        for m in (i, j):
            todo[m] -= 1
            if todo[m] == 0:
                y2[m] = y2[m] + product(n + m)
                if both:
                    y1[m] = y1[m] + product(m)
                    y2[m] = y2[m] + t[m] * y1[m]
    return (y1, y2) if both else (y2,)


class _Stream:
    def __init__(self, jobs, stage, sems):
        self.jobs, self.stage, self.sems = jobs, stage, sems
        self.slots = stage.shape[0]
        assert all(job[0] >= self.slots for job in jobs)

    def copies(self, m, c, slot):
        return [pltpu.make_async_copy(src, dst, self.sems.at[slot])
                for src, dst in self.jobs[m][1](c, self.stage.at[slot])]

    def fetch(self, m, c, slot):
        for copy in self.copies(m, c, slot):
            copy.start()

    def start(self, part=0, parts=1):
        for c in range(part * self.slots // parts, (part + 1) * self.slots // parts):
            self.fetch(0, c, c)

    def drain(self, m, idle=None):
        count, _, consume = self.jobs[m]
        first = sum(job[0] for job in self.jobs[:m])

        @pl.loop(0, count)
        def _(c):
            slot = (first + c) % self.slots
            for copy in self.copies(m, c, slot):
                copy.wait()
            consume(c, self.stage.at[slot])
            nxt = c + self.slots
            if self.slots < count:
                pl.when(nxt < count)(lambda: self.fetch(m, nxt, slot))
            if m + 1 < len(self.jobs):
                pl.when(nxt >= count)(lambda: self.fetch(m + 1, nxt - count, slot))
            elif idle:
                for k in range(self.slots):
                    pl.when(nxt == count + k)(functools.partial(idle, k))


def _put(dst, n, row, group, block):
    rows = pl.ds(pl.multiple_of(row // 2, PACK // 2), PACK // 2)
    for r, op in _weight_operands(n, block):
        dst[group, r, rows, :] = op


def _head_job(src, dst, n):
    step = PACK * n * dst.shape[0]

    def consume(c, staged):
        heads = [_split(pltpu.bitcast(
            staged[i].reshape(PACK, step // PACK, LANES).reshape(PACK, step // PACK * LANES),
            WORD), step // PACK) for i in range(n)]
        for g in range(dst.shape[0]):
            _put(dst, n, c * PACK, g, lambda i, j: heads[i][g * n + j])

    return (src.shape[1] // step,
            lambda c, slot: [(src.at[:, pl.ds(pl.multiple_of(c * step, step), step), :], slot)],
            consume)


def _wide_job(srcs, dst, n, first, count):
    def consume(c, staged):
        @pl.loop(0, dst.shape[0])
        def _(g):
            lanes = lambda j: pl.ds(pl.multiple_of((g * (n // 2) + j) * LANES, LANES), LANES)
            _put(dst, n, (first + c) * PACK, g, lambda i, j: pltpu.bitcast(
                staged[j // (n // 2), i, :, lanes(j % (n // 2))], WORD))

    def pieces(c, slot):
        rows = pl.ds(pl.multiple_of((first + c) * PACK, PACK), PACK)
        return [(src.at[:, rows, :], slot.at[m]) for m, src in enumerate(srcs)]

    return count, pieces, consume


def _tall_job(src, dst, n):
    parts = len(T8) // n
    step = PACK * parts * parts

    def consume(c, staged):
        for part in range(parts):
            @pl.loop(0, TALL_ROWS, step=step)
            def _(r0):
                for r in range(0, step, PACK):
                    for g in range(dst.shape[0]):
                        _put(dst, n, (c * parts + part) * TALL_ROWS + r0 + r, g,
                             lambda i, j: pltpu.bitcast(staged[
                                 part * n + i, pl.ds(pl.multiple_of(r0 + r, PACK), PACK),
                                 pl.ds((g * n + j) * LANES, LANES)], WORD))

    def pieces(c, slot):
        first = [(c * parts + part) * TALL_ROWS for part in range(parts)]
        return [(src.at[row // LANES, :,
                        pl.ds(pl.multiple_of(row % LANES, TALL_ROWS), TALL_ROWS), :],
                 slot.at[pl.ds(part * n, n)]) for part, row in enumerate(first)]

    return src.shape[0] * LANES // TALL_ROWS // parts, pieces, consume


def _kernel(x_hbm, mem0_hbm, wq_hbm, wk_hbm, wv_hbm, wo_hbm, wg_hbm, wu_hbm, wd_hbm,
            out_hbm,
            x_vm, out_vm, mem0_vm, wq, wk, wv, wo, wgu, wd,
            h_ref, o_ref, xb_ref, hb_ref, mem_ref, ra_ref, rb_ref, x2_ref, fill_ref,
            qkv_stage, tall_stage, wide_stage,
            qkv_sems, tall_sems, wide_sems, in_sems, out_sem):
    S = x_vm.shape[0]
    n_mem, seg = mem_ref.shape[1], x2_ref.shape[0]
    n_seg = S // seg
    L = n_mem + seg
    scale = LANES ** -0.5

    qi = jax.lax.broadcasted_iota(jnp.int32, fill_ref.shape, 0)
    ki = jax.lax.broadcasted_iota(jnp.int32, fill_ref.shape, 1)
    same = ((qi >= L) == (ki >= L)) & (ki < 2 * L)
    visible = (jnp.where(qi >= L, qi - L, qi) < n_mem) | (qi >= ki)
    fill_ref[...] = jnp.where(same, jnp.where(visible, 0.0, MASK_VALUE / scale), -jnp.inf)

    BOTH = (0, 1)

    def segment(i, start=0, size=seg):
        return pl.ds(pl.multiple_of(i * seg + start, size), size)

    def segments_in(i, live):
        for r in range(0, seg, ROWS):
            x = [x_vm[segment(jnp.minimum(i, n_seg - 1), r, ROWS), :].astype(F32),
                 x2_ref[pl.ds(r, ROWS), :]]
            if len(live) == 1:
                x = [jnp.where(live[0] == 0, *x)]
            for p, xp in zip(live, x):
                ra_ref[p, pl.ds(r, ROWS), :] = xp
            _store_rows(T8, h_ref, [_layernorm(xp) for xp in x], pl.ds(n_mem + r, ROWS))

    def memories_in(live):
        _store_rows(T8, h_ref, [mem_ref[p] for p in live], pl.ds(0, n_mem))

    def heads(w, c, live):
        y = zip(*_project(T8, h_ref, w, c, len(live) == 2))
        if w is wq:
            return [jnp.concatenate(h, axis=0) for h in y]
        pad = (jnp.zeros((LANES - len(live) * L, LANES), F32),)
        return [jnp.concatenate(h + pad, axis=0).astype(BF16) for h in y]

    def softmax(q, k):
        out = []
        for qh, kh in zip(q, k):
            s = _dot(qh, kh, 1)
            fill = fill_ref[pl.ds(0, s.shape[0]), :]
            s = jnp.where(fill == 0.0, s, fill)
            p = jnp.exp2((s - jnp.max(s, axis=-1, keepdims=True)) * (scale * LOG2_E))
            out.append(p * _reciprocal(jnp.sum(p, axis=-1, keepdims=True)))
        return out

    def mix(c, p, v):
        o = [_dot(ph, vh) for ph, vh in zip(p, v)]
        _store_tiles(T8, o_ref, c * len(o),
                     [[a[r:r + L] for a in o] for r in range(0, o[0].shape[0], L)])

    def attention_out(c, i, live):
        for p, y in zip(live, _project(T8, o_ref, wo, c, len(live) == 2)):
            y = _join(y)
            cols = pl.ds(c * y.shape[1], y.shape[1])
            mem_ref[p, :, cols] = y[:n_mem]
            rb_ref[i & 3, p, :, cols] = ra_ref[p, :, cols] + y[n_mem:]

    def glu_in(i, live):
        for r in range(0, seg, ROWS):
            x = [rb_ref[(i + 3) & 3, p, pl.ds(r, ROWS), :] for p in live]
            _store_rows(T8, xb_ref, [_layernorm(xp) for xp in x], pl.ds(r, ROWS))

    def gate(c, live):
        half = len(T8) // 2
        h = [[_sigmoid(g) * u for g, u in zip(y[:half], y[half:])]
             for y in _project(T8, xb_ref, wgu, c, len(live) == 2)]
        if len(live) == 1:
            h = [[jnp.where(live[0] == p, a, 0.0) for a in h[0]] for p in BOTH]
        _store_tiles(T4, hb_ref, c * half, h)

    def glu_out(c, i, live):
        for p, y in zip(live, _project(T4, hb_ref, wd, c, len(live) == 2)):
            y = _join(y)
            cols = pl.ds(c * y.shape[1], y.shape[1])
            y = rb_ref[(i + 2) & 3, p, :, cols] + y
            if p == 0:
                x2_ref[:, cols] = y
            else:
                out_vm[segment(jnp.maximum(i - 5, 0)), cols] = y.astype(out_vm.dtype)

    def run(order, i, live):
        val = {what: [] for what in order}
        for what in order:
            c = len(val[what])
            val[what].append({
                'x': lambda: segments_in(i, live),
                'm': lambda: memories_in(live),
                'q': lambda: heads(wq, c, live),
                'k': lambda: heads(wk, c, live),
                'v': lambda: heads(wv, c, live),
                'S': lambda: softmax(val['q'][c], val['k'][c]),
                'P': lambda: mix(c, val['S'][c], val['v'][c]),
                'W': lambda: attention_out(c, i, live),
                'h': lambda: glu_in(i, live),
                'G': lambda: gate(c, live),
                'D': lambda: glu_out(c, i, live),
            }[what]())

    def out_copy(rows):
        return pltpu.make_async_copy(out_vm.at[rows], out_hbm.at[rows], out_sem)

    head, tail = pl.ds(0, 3 * seg), pl.ds(3 * seg, S - 3 * seg)
    x_head = pltpu.make_async_copy(x_hbm.at[head], x_vm.at[head], in_sems.at[0])
    x_tail = pltpu.make_async_copy(x_hbm.at[tail], x_vm.at[tail], in_sems.at[1])
    mem_copy = pltpu.make_async_copy(mem0_hbm, mem0_vm, in_sems.at[2])
    half = wg_hbm.shape[1] // PACK // 2
    qkv = _Stream([_head_job(s, d, len(T8)) for s, d in
                   ((wq_hbm, wq), (wk_hbm, wk), (wv_hbm, wv))], qkv_stage, qkv_sems)
    proj = _Stream([_tall_job(wo_hbm, wo, len(T8))], tall_stage, tall_sems)
    wide = _Stream([_wide_job((wg_hbm, wu_hbm), wgu, len(T8), first, half)
                    for first in (0, half)], wide_stage, wide_sems)
    down = _Stream([_tall_job(wd_hbm, wd, len(T4))], tall_stage, tall_sems)

    qkv.start()
    x_head.start()
    mem_copy.start()
    for m in range(3):
        qkv.drain(m, lambda k: proj.start(k, qkv.slots))
    x_head.wait()
    mem_copy.wait()
    mem_ref[0] = mem_ref[1] = mem0_vm[...].astype(F32)
    x2_ref[...] = rb_ref[1, 1] = rb_ref[2, 1] = rb_ref[0, 1] = jnp.zeros(x2_ref.shape, F32)

    attention = 'qkvS' + 'qkvPS' * (wq.shape[0] - 1)
    lone_attention = 'mx' + (attention[:-5] + 'qkPSvP' if wq.shape[0] > 1 else 'qkSvP')
    glu, glu_down, attn_out = 'h' + 'G' * wgu.shape[0], 'D' * wd.shape[0], 'W' * wo.shape[0]

    @pl.loop(0, 9)
    def _(j):
        lone = (jnp.where(j < 4, 0, 1),)
        i = jnp.where(j < 4, jnp.minimum(j, 2), j - 4 + n_seg)
        phase = lambda cond, order, live, i=i: pl.when(cond)(lambda: run(order, i, live))
        attends = (j != 3) & (j < 7)

        pl.when(j >= 4)(lambda: out_copy(segment(i - 6)).start())
        phase(attends, lone_attention, lone)
        pl.when(j == 0)(lambda: proj.drain(0, lambda k: wide.start(k, proj.slots)))
        pl.when(j == 1)(lambda: wide.drain(0))
        pl.when(j == 2)(lambda: wide.drain(1, lambda k: down.start() if k == 0 else None))
        pl.when(j == 3)(lambda: down.drain(0, lambda k: x_tail.start() if k == 0 else None))
        phase((j >= 3) & (j < 6), glu_down, BOTH)
        phase(j >= 6, glu_down, (1,))
        phase(j == 4, glu, BOTH)
        phase((j > 1) & (j != 4) & (j < 8), glu, lone, jnp.where(j == 2, 1, i))
        phase(attends, attn_out, lone)

        @pl.when(j == 3)
        def _():
            x_tail.wait()
            pl.loop(3, n_seg)(lambda step: run(
                'mxD' + attention + glu_down[1:] + 'P' + glu + attn_out, step, BOTH))
            out_copy(pl.ds(0, (n_seg - 6) * seg)).start()

    out_copy(segment(n_seg - 1)).start()
    pltpu.make_async_copy(out_vm, out_hbm, out_sem).wait()


@functools.partial(jax.jit, static_argnames=("A_seg_len",))
def pallas_interleave_layers__memory_aug_recurrent_mem_tr__glu_gated_glu__prompt_kernel(
    A_x: jax.Array,
    A_mem0: jax.Array,
    A_Wq: jax.Array,
    A_Wk: jax.Array,
    A_Wv: jax.Array,
    A_Wo: jax.Array,
    A_seg_len: int,
    B_x: jax.Array,
    B_w_gate: jax.Array,
    B_w_up: jax.Array,
    B_w_down: jax.Array,
):
    del B_x
    B, S, D = A_x.shape
    _, H, Dh = A_Wq.shape
    M = A_mem0.shape[1]
    F = B_w_gate.shape[1]
    seg = int(A_seg_len)
    L = M + seg
    n8, n4 = len(T8), len(T4)
    assert B == 1 and Dh == LANES and 2 * L < LANES and S % seg == 0 and S // seg > 6
    assert D % (n8 * LANES) == 0 and H % n8 == 0 and F % (n4 * LANES) == 0

    def weights(n, k, cols):
        return pltpu.VMEM((cols // n // LANES, _n_products(n), k // n // 2, LANES), WORD)

    def rows(count, m, k):
        return pltpu.VMEM((count, k // LANES, m, LANES), F32)

    hbm = pl.BlockSpec(memory_space=pl.ANY)
    out = pl.pallas_call(
        _kernel,
        out_shape=jax.ShapeDtypeStruct((S, D), A_x.dtype),
        in_specs=[hbm] * 9,
        out_specs=hbm,
        scratch_shapes=[
            pltpu.VMEM((S, D), A_x.dtype),
            pltpu.VMEM((S, D), A_x.dtype),
            pltpu.VMEM((M, D), A_mem0.dtype),
            weights(n8, D, H * Dh),
            weights(n8, D, H * Dh),
            weights(n8, D, H * Dh),
            weights(n8, H * Dh, D),
            weights(n8, D, 2 * F),
            weights(n4, F, D),
            rows(_n_products(n8), L, D // n8),
            rows(2 * n8, L, H * Dh // n8),
            rows(2 * n8, seg, D // n8),
            rows(2 * n4, seg, F // n4),
            pltpu.VMEM((2, M, D), F32),
            pltpu.VMEM((2, seg, D), F32),
            pltpu.VMEM((4, 2, seg, D), F32),
            pltpu.VMEM((seg, D), F32),
            pltpu.VMEM((2 * L, LANES), F32),
            pltpu.VMEM((QKV_SLOTS, n8, PACK * H, Dh), BF16),
            pltpu.VMEM((TALL_SLOTS, n8, TALL_ROWS, D), BF16),
            pltpu.VMEM((WIDE_SLOTS, 2, n8, PACK, F), BF16),
            pltpu.SemaphoreType.DMA((QKV_SLOTS,)),
            pltpu.SemaphoreType.DMA((TALL_SLOTS,)),
            pltpu.SemaphoreType.DMA((WIDE_SLOTS,)),
            pltpu.SemaphoreType.DMA((3,)),
            pltpu.SemaphoreType.DMA(()),
        ],
        compiler_params=pltpu.CompilerParams(vmem_limit_bytes=124 * 2**20),
    )(
        A_x.reshape(S, D),
        A_mem0.reshape(M, D),
        A_Wq.reshape(n8, D // n8 * H, Dh),
        A_Wk.reshape(n8, D // n8 * H, Dh),
        A_Wv.reshape(n8, D // n8 * H, Dh),
        A_Wo.reshape(H // n8, n8, Dh, D),
        B_w_gate.reshape(n8, D // n8, F),
        B_w_up.reshape(n8, D // n8, F),
        B_w_down.reshape(F // LANES // n4, n4, LANES, D),
    )
    return out.reshape(B, S, D)
```

```python
import functools

import jax
import jax.numpy as jnp
import jax.experimental.pallas as pl
import jax.experimental.pallas.tpu as pltpu
import numpy as np

F32 = jnp.float32
BF16 = jnp.bfloat16
WORD = jnp.uint32
LANES = 128
PACK = 16
LN_EPS = 1e-5
MASK_VALUE = -1000000000.0
LOG2_E = 1.4426950408889634
HIGH_HALF = np.uint32(0xFFFF0000)

T8 = (-2.9, -1.4, -0.7, -0.215, 0.215, 0.7, 1.4, 2.9)
T4 = (-1.8, -0.43, 0.43, 1.8)

TALL_ROWS = 64
QKV_SLOTS, TALL_SLOTS, WIDE_SLOTS = 3, 7, 4
ROWS = 16


def _layernorm(x, gain=1.0):
    c = x - jnp.mean(x, axis=-1, keepdims=True)
    return c * (gain * jax.lax.rsqrt(jnp.mean(c * c, axis=-1, keepdims=True) + LN_EPS))


def _reciprocal(x):
    r = pl.reciprocal(x, approx=True)
    return r * (2.0 - x * r)


def _dot(a, b, b_axis=0):
    return jax.lax.dot_general(a, b, (((1,), (b_axis,)), ((), ())), preferred_element_type=F32)


def _split(x, n):
    w = x.shape[1] // n
    return [x[:, i * w:(i + 1) * w] for i in range(n)]


def _join(blocks):
    return jnp.concatenate(blocks, axis=1)


def _pairs(n):
    return sorted(((i, j) for j in range(n) for i in range(j)),
                  key=lambda p: (p[1] // 4, p[0] // 4, p[1], p[0]))


def _n_products(n):
    return (3 * n * n + n) // 2


def _weight_operands(n, w):
    def rows(x):
        return [jax.lax.bitcast_convert_type(y, F32) for y in (x << 16, x & HIGH_HALF)]

    def words(x):
        even, odd = (jax.lax.bitcast_convert_type(y.astype(BF16).astype(F32), WORD) for y in x)
        return (even >> 16) | odd

    add = lambda x, y: [a + b for a, b in zip(x, y)]
    sub = lambda x, y: [a - b for a, b in zip(x, y)]
    p = [rows(w(i, i)) for i in range(n)]
    q = list(p)
    for k, (i, j) in enumerate(_pairs(n)):
        ij, ji = w(i, j), w(j, i)
        a, b = rows(ij), rows(ji)
        yield 2 * n + 3 * k, words(add(a, b))
        yield 2 * n + 3 * k + 1, ji
        yield 2 * n + 3 * k + 2, ij
        p[i], p[j], q[i], q[j] = add(p[i], a), add(p[j], b), sub(q[i], b), sub(q[j], a)
    for i in range(n):
        yield i, words(p[i])
        yield n + i, words(q[i])


def _row_operand(t, r, base, both):
    n = len(t)
    if r < 2 * n:
        return base(r)
    (i, j), kind = _pairs(n)[(r - 2 * n) // 3], (r - 2 * n) % 3
    s = base(n + i) + base(n + j)
    if not both:
        return s
    s = s.astype(BF16).astype(F32)
    if kind == 0:
        return s
    return s + (t[j] - t[i]) * base(j) if kind == 1 else s - (t[j] - t[i]) * base(i)


def _store_rows(t, ref, h, rows):
    n, both = len(t), len(h) == 2
    h = [_split(x, n) for x in h]
    base = (h[0] + [b - c * a for c, a, b in zip(t, *h)]) if both else [None] * n + h[0]
    for r in range(ref.shape[0]):
        if both or (r >= n and (r < 2 * n or (r - 2 * n) % 3)):
            op = _row_operand(t, r, base.__getitem__, both)
            for k, tile in enumerate(_split(op, ref.shape[1])):
                ref[r, k, rows, :] = tile


def _store_tiles(t, ref, first, h):
    for x, tiles in enumerate(zip(*h), first):
        k, i = divmod(x, len(t))
        if len(tiles) == 2:
            ref[i, k] = tiles[0]
            ref[len(t) + i, k] = tiles[1] - t[i] * tiles[0]
        else:
            ref[len(t) + i, k] = tiles[0]


def _project(t, rows_ref, w_ref, group, both):
    n = len(t)

    def stored(r):
        return _join([rows_ref[r, k] for k in range(rows_ref.shape[1])])

    def product(r):
        rows = stored(r) if r < rows_ref.shape[0] else _row_operand(t, r, stored, both)
        return _dot(rows, pltpu.bitcast(w_ref[group, r], BF16))

    y1, y2 = [None] * n, [None] * n
    acc = lambda a, b: b if a is None else a + b
    todo = [n - 1] * n
    for k, (i, j) in enumerate(_pairs(n)):
        ti, tj = product(2 * n + 3 * k + 1), product(2 * n + 3 * k + 2)
        y2[i], y2[j] = acc(y2[i], ti), acc(y2[j], tj)
        if both:
            u = (1.0 / (t[j] - t[i])) * (ti + tj - product(2 * n + 3 * k))
            y1[i], y1[j] = acc(y1[i], u), (-u if y1[j] is None else y1[j] - u)
        for m in (i, j):
            todo[m] -= 1
            if todo[m] == 0:
                y2[m] = y2[m] + product(n + m)
                if both:
                    y1[m] = y1[m] + product(m)
                    y2[m] = y2[m] + t[m] * y1[m]
    return (y1, y2) if both else (y2,)


class _Stream:
    def __init__(self, jobs, stage, sems):
        self.jobs, self.stage, self.sems = jobs, stage, sems
        self.slots = stage.shape[0]
        assert all(job[0] >= self.slots for job in jobs)

    def copies(self, m, c, slot):
        return [pltpu.make_async_copy(src, dst, self.sems.at[slot])
                for src, dst in self.jobs[m][1](c, self.stage.at[slot])]

    def fetch(self, m, c, slot):
        for copy in self.copies(m, c, slot):
            copy.start()

    def start(self, part=0, parts=1):
        for c in range(part * self.slots // parts, (part + 1) * self.slots // parts):
            self.fetch(0, c, c)

    def drain(self, m, idle=None):
        count, _, consume = self.jobs[m]
        first = sum(job[0] for job in self.jobs[:m])

        @pl.loop(0, count)
        def _(c):
            slot = (first + c) % self.slots
            for copy in self.copies(m, c, slot):
                copy.wait()
            consume(c, self.stage.at[slot])
            nxt = c + self.slots
            if self.slots < count:
                pl.when(nxt < count)(lambda: self.fetch(m, nxt, slot))
            if m + 1 < len(self.jobs):
                pl.when(nxt >= count)(lambda: self.fetch(m + 1, nxt - count, slot))
            elif idle:
                for k in range(self.slots):
                    pl.when(nxt == count + k)(functools.partial(idle, k))


def _put(dst, n, row, group, block):
    rows = pl.ds(pl.multiple_of(row // 2, PACK // 2), PACK // 2)
    for r, op in _weight_operands(n, block):
        dst[group, r, rows, :] = op


def _head_job(src, dst, n):
    step = PACK * n * dst.shape[0]

    def consume(c, staged):
        heads = [_split(pltpu.bitcast(
            staged[i].reshape(PACK, step // PACK, LANES).reshape(PACK, step // PACK * LANES),
            WORD), step // PACK) for i in range(n)]
        for g in range(dst.shape[0]):
            _put(dst, n, c * PACK, g, lambda i, j: heads[i][g * n + j])

    return (src.shape[1] // step,
            lambda c, slot: [(src.at[:, pl.ds(pl.multiple_of(c * step, step), step), :], slot)],
            consume)


def _wide_job(srcs, dst, n, first, count):
    def consume(c, staged):
        @pl.loop(0, dst.shape[0])
        def _(g):
            lanes = lambda j: pl.ds(pl.multiple_of((g * (n // 2) + j) * LANES, LANES), LANES)
            _put(dst, n, (first + c) * PACK, g, lambda i, j: pltpu.bitcast(
                staged[j // (n // 2), i, :, lanes(j % (n // 2))], WORD))

    def pieces(c, slot):
        rows = pl.ds(pl.multiple_of((first + c) * PACK, PACK), PACK)
        return [(src.at[:, rows, :], slot.at[m]) for m, src in enumerate(srcs)]

    return count, pieces, consume


def _tall_job(src, dst, n):
    parts = len(T8) // n
    step = PACK * parts * parts

    def consume(c, staged):
        for part in range(parts):
            @pl.loop(0, TALL_ROWS, step=step)
            def _(r0):
                for r in range(0, step, PACK):
                    for g in range(dst.shape[0]):
                        _put(dst, n, (c * parts + part) * TALL_ROWS + r0 + r, g,
                             lambda i, j: pltpu.bitcast(staged[
                                 part * n + i, pl.ds(pl.multiple_of(r0 + r, PACK), PACK),
                                 pl.ds((g * n + j) * LANES, LANES)], WORD))

    def pieces(c, slot):
        first = [(c * parts + part) * TALL_ROWS for part in range(parts)]
        return [(src.at[row // LANES, :,
                        pl.ds(pl.multiple_of(row % LANES, TALL_ROWS), TALL_ROWS), :],
                 slot.at[pl.ds(part * n, n)]) for part, row in enumerate(first)]

    return src.shape[0] * LANES // TALL_ROWS // parts, pieces, consume


def _kernel(x_hbm, mem0_hbm, wq_hbm, wk_hbm, wv_hbm, wo_hbm, wg_hbm, wu_hbm, wd_hbm,
            out_hbm,
            x_vm, out_vm, mem0_vm, wq, wk, wv, wo, wgu, wd,
            h_ref, o_ref, xb_ref, hb_ref, mem_ref, ra_ref, rb_ref, x2_ref, fill_ref,
            qkv_stage, tall_stage, wide_stage,
            qkv_sems, tall_sems, wide_sems, in_sems, out_sem):
    S = x_vm.shape[0]
    n_mem, seg = mem_ref.shape[1], x2_ref.shape[0]
    n_seg = S // seg
    L = n_mem + seg
    scale = LANES ** -0.5

    qi = jax.lax.broadcasted_iota(jnp.int32, fill_ref.shape, 0)
    ki = jax.lax.broadcasted_iota(jnp.int32, fill_ref.shape, 1)
    same = ((qi >= L) == (ki >= L)) & (ki < 2 * L)
    visible = (jnp.where(qi >= L, qi - L, qi) < n_mem) | (qi >= ki)
    fill_ref[...] = jnp.where(same, jnp.where(visible, 0.0, MASK_VALUE / scale), -jnp.inf)

    BOTH = (0, 1)

    def segment(i, start=0, size=seg):
        return pl.ds(pl.multiple_of(i * seg + start, size), size)

    def segments_in(i, live):
        for r in range(0, seg, ROWS):
            x = [x_vm[segment(jnp.minimum(i, n_seg - 1), r, ROWS), :].astype(F32),
                 x2_ref[pl.ds(r, ROWS), :]]
            if len(live) == 1:
                x = [jnp.where(live[0] == 0, *x)]
            for p, xp in zip(live, x):
                ra_ref[p, pl.ds(r, ROWS), :] = xp
            _store_rows(T8, h_ref, [_layernorm(xp) for xp in x], pl.ds(n_mem + r, ROWS))

    def memories_in(live):
        _store_rows(T8, h_ref, [mem_ref[p] for p in live], pl.ds(0, n_mem))

    def heads(w, c, live):
        y = zip(*_project(T8, h_ref, w, c, len(live) == 2))
        if w is wq:
            return [jnp.concatenate(h, axis=0) for h in y]
        pad = (jnp.zeros((LANES - len(live) * L, LANES), F32),)
        return [jnp.concatenate(h + pad, axis=0).astype(BF16) for h in y]

    def softmax(q, k):
        out = []
        for qh, kh in zip(q, k):
            s = _dot(qh, kh, 1)
            fill = fill_ref[pl.ds(0, s.shape[0]), :]
            s = jnp.where(fill == 0.0, s, fill)
            p = jnp.exp2((s - jnp.max(s, axis=-1, keepdims=True)) * (scale * LOG2_E))
            out.append(p * _reciprocal(jnp.sum(p, axis=-1, keepdims=True)))
        return out

    def mix(c, p, v):
        o = [_dot(ph, vh) for ph, vh in zip(p, v)]
        _store_tiles(T8, o_ref, c * len(o),
                     [[a[r:r + L] for a in o] for r in range(0, o[0].shape[0], L)])

    def attention_out(c, i, live):
        for p, y in zip(live, _project(T8, o_ref, wo, c, len(live) == 2)):
            y = _join(y)
            cols = pl.ds(c * y.shape[1], y.shape[1])
            mem_ref[p, :, cols] = y[:n_mem]
            rb_ref[i & 3, p, :, cols] = ra_ref[p, :, cols] + y[n_mem:]

    def glu_in(i, live):
        for r in range(0, seg, ROWS):
            x = [rb_ref[(i + 3) & 3, p, pl.ds(r, ROWS), :] for p in live]
            _store_rows(T8, xb_ref, [_layernorm(xp, 0.5) for xp in x], pl.ds(r, ROWS))

    def gate(c, live):
        half = len(T8) // 2
        h = [[(jnp.tanh(g) + 1.0) * u for g, u in zip(y[:half], y[half:])]
             for y in _project(T8, xb_ref, wgu, c, len(live) == 2)]
        if len(live) == 1:
            h = [[jnp.where(live[0] == p, a, 0.0) for a in h[0]] for p in BOTH]
        _store_tiles(T4, hb_ref, c * half, h)

    def glu_out(c, i, live):
        for p, y in zip(live, _project(T4, hb_ref, wd, c, len(live) == 2)):
            y = _join(y)
            cols = pl.ds(c * y.shape[1], y.shape[1])
            y = rb_ref[(i + 2) & 3, p, :, cols] + y
            if p == 0:
                x2_ref[:, cols] = y
            else:
                out_vm[segment(jnp.maximum(i - 5, 0)), cols] = y.astype(out_vm.dtype)

    def run(order, i, live):
        val = {what: [] for what in order}
        for what in order:
            c = len(val[what])
            val[what].append({
                'x': lambda: segments_in(i, live),
                'm': lambda: memories_in(live),
                'q': lambda: heads(wq, c, live),
                'k': lambda: heads(wk, c, live),
                'v': lambda: heads(wv, c, live),
                'S': lambda: softmax(val['q'][c], val['k'][c]),
                'P': lambda: mix(c, val['S'][c], val['v'][c]),
                'W': lambda: attention_out(c, i, live),
                'h': lambda: glu_in(i, live),
                'G': lambda: gate(c, live),
                'D': lambda: glu_out(c, i, live),
            }[what]())

    def out_copy(rows):
        return pltpu.make_async_copy(out_vm.at[rows], out_hbm.at[rows], out_sem)

    head, tail = pl.ds(0, 3 * seg), pl.ds(3 * seg, S - 3 * seg)
    x_head = pltpu.make_async_copy(x_hbm.at[head], x_vm.at[head], in_sems.at[0])
    x_tail = pltpu.make_async_copy(x_hbm.at[tail], x_vm.at[tail], in_sems.at[1])
    mem_copy = pltpu.make_async_copy(mem0_hbm, mem0_vm, in_sems.at[2])
    half = wg_hbm.shape[1] // PACK // 2
    qkv = _Stream([_head_job(s, d, len(T8)) for s, d in
                   ((wq_hbm, wq), (wk_hbm, wk), (wv_hbm, wv))], qkv_stage, qkv_sems)
    proj = _Stream([_tall_job(wo_hbm, wo, len(T8))], tall_stage, tall_sems)
    wide = _Stream([_wide_job((wg_hbm, wu_hbm), wgu, len(T8), first, half)
                    for first in (0, half)], wide_stage, wide_sems)
    down = _Stream([_tall_job(wd_hbm, wd, len(T4))], tall_stage, tall_sems)

    qkv.start()
    x_head.start()
    mem_copy.start()
    for m in range(3):
        qkv.drain(m, lambda k: proj.start(k, qkv.slots))
    x_head.wait()
    mem_copy.wait()
    mem_ref[0] = mem_ref[1] = mem0_vm[...].astype(F32)
    x2_ref[...] = rb_ref[1, 1] = rb_ref[2, 1] = rb_ref[0, 1] = jnp.zeros(x2_ref.shape, F32)

    attention = 'qkvS' + 'qkvPS' * (wq.shape[0] - 1)
    lone_attention = 'mx' + (attention[:-5] + 'qkPSvP' if wq.shape[0] > 1 else 'qkSvP')
    glu, glu_down, attn_out = 'h' + 'G' * wgu.shape[0], 'D' * wd.shape[0], 'W' * wo.shape[0]

    @pl.loop(0, 9)
    def _(j):
        lone = (jnp.where(j < 4, 0, 1),)
        i = jnp.where(j < 4, jnp.minimum(j, 2), j - 4 + n_seg)
        phase = lambda cond, order, live, i=i: pl.when(cond)(lambda: run(order, i, live))
        attends = (j != 3) & (j < 7)

        pl.when(j >= 4)(lambda: out_copy(segment(i - 6)).start())
        phase(attends, lone_attention, lone)
        pl.when(j == 0)(lambda: proj.drain(0, lambda k: wide.start(k, proj.slots)))
        pl.when(j == 1)(lambda: wide.drain(0))
        pl.when(j == 2)(lambda: wide.drain(1, lambda k: down.start() if k == 0 else None))
        pl.when(j == 3)(lambda: down.drain(0, lambda k: x_tail.start() if k == 0 else None))
        phase((j >= 3) & (j < 6), glu_down, BOTH)
        phase(j >= 6, glu_down, (1,))
        phase(j == 4, glu, BOTH)
        phase((j > 1) & (j != 4) & (j < 8), glu, lone, jnp.where(j == 2, 1, i))
        phase(attends, attn_out, lone)

        @pl.when(j == 3)
        def _():
            x_tail.wait()
            pl.loop(3, n_seg)(lambda step: run(
                'mxD' + attention + glu_down[1:] + 'P' + glu + attn_out, step, BOTH))
            out_copy(pl.ds(0, (n_seg - 6) * seg)).start()

    out_copy(segment(n_seg - 1)).start()
    pltpu.make_async_copy(out_vm, out_hbm, out_sem).wait()


@functools.partial(jax.jit, static_argnames=("A_seg_len",))
def pallas_interleave_layers__memory_aug_recurrent_mem_tr__glu_gated_glu__prompt_kernel(
    A_x: jax.Array,
    A_mem0: jax.Array,
    A_Wq: jax.Array,
    A_Wk: jax.Array,
    A_Wv: jax.Array,
    A_Wo: jax.Array,
    A_seg_len: int,
    B_x: jax.Array,
    B_w_gate: jax.Array,
    B_w_up: jax.Array,
    B_w_down: jax.Array,
):
    del B_x
    B, S, D = A_x.shape
    _, H, Dh = A_Wq.shape
    M = A_mem0.shape[1]
    F = B_w_gate.shape[1]
    seg = int(A_seg_len)
    L = M + seg
    n8, n4 = len(T8), len(T4)
    assert B == 1 and Dh == LANES and 2 * L < LANES and S % seg == 0 and S // seg > 6
    assert D % (n8 * LANES) == 0 and H % n8 == 0 and F % (n4 * LANES) == 0

    def weights(n, k, cols):
        return pltpu.VMEM((cols // n // LANES, _n_products(n), k // n // 2, LANES), WORD)

    def rows(count, m, k):
        return pltpu.VMEM((count, k // LANES, m, LANES), F32)

    hbm = pl.BlockSpec(memory_space=pl.ANY)
    out = pl.pallas_call(
        _kernel,
        out_shape=jax.ShapeDtypeStruct((S, D), A_x.dtype),
        in_specs=[hbm] * 9,
        out_specs=hbm,
        scratch_shapes=[
            pltpu.VMEM((S, D), A_x.dtype),
            pltpu.VMEM((S, D), A_x.dtype),
            pltpu.VMEM((M, D), A_mem0.dtype),
            weights(n8, D, H * Dh),
            weights(n8, D, H * Dh),
            weights(n8, D, H * Dh),
            weights(n8, H * Dh, D),
            weights(n8, D, 2 * F),
            weights(n4, F, D),
            rows(_n_products(n8), L, D // n8),
            rows(2 * n8, L, H * Dh // n8),
            rows(2 * n8, seg, D // n8),
            rows(2 * n4, seg, F // n4),
            pltpu.VMEM((2, M, D), F32),
            pltpu.VMEM((2, seg, D), F32),
            pltpu.VMEM((4, 2, seg, D), F32),
            pltpu.VMEM((seg, D), F32),
            pltpu.VMEM((2 * L, LANES), F32),
            pltpu.VMEM((QKV_SLOTS, n8, PACK * H, Dh), BF16),
            pltpu.VMEM((TALL_SLOTS, n8, TALL_ROWS, D), BF16),
            pltpu.VMEM((WIDE_SLOTS, 2, n8, PACK, F), BF16),
            pltpu.SemaphoreType.DMA((QKV_SLOTS,)),
            pltpu.SemaphoreType.DMA((TALL_SLOTS,)),
            pltpu.SemaphoreType.DMA((WIDE_SLOTS,)),
            pltpu.SemaphoreType.DMA((3,)),
            pltpu.SemaphoreType.DMA(()),
        ],
        compiler_params=pltpu.CompilerParams(vmem_limit_bytes=124 * 2**20),
    )(
        A_x.reshape(S, D),
        A_mem0.reshape(M, D),
        A_Wq.reshape(n8, D // n8 * H, Dh),
        A_Wk.reshape(n8, D // n8 * H, Dh),
        A_Wv.reshape(n8, D // n8 * H, Dh),
        A_Wo.reshape(H // n8, n8, Dh, D),
        B_w_gate.reshape(n8, D // n8, F),
        B_w_up.reshape(n8, D // n8, F),
        B_w_down.reshape(F // LANES // n4, n4, LANES, D),
    )
    return out.reshape(B, S, D)
```
